```python
import jax
import jax.numpy as jnp

def _softmax(x, axis=-1):
    return jax.nn.softmax(x, axis=axis)

def _gelu(x):
    return jax.nn.gelu(x, approximate=True)

def _silu(x):
    return jax.nn.silu(x)

def _sigmoid(x):
    return jax.nn.sigmoid(x)

def _layernorm(x, axis=-1, eps=1e-05):
    m = jnp.mean(x, axis=axis, keepdims=True)
    v = jnp.var(x, axis=axis, keepdims=True)
    return (x - m) / jnp.sqrt(v + eps)

def _scatter_add(tgt, idx, src, axis=0):
    return tgt.at[idx].add(src)

def _segment_sum(src, seg, n):
    return jax.ops.segment_sum(src, seg, n)

class _Rng:

    def __init__(self, key):
        self._k = key

    def _next(self):
        self._k, sub = jax.random.split(self._k)
        return sub

    def normal(self, shape):
        return jax.random.normal(self._next(), shape, dtype=jnp.bfloat16)

    def randint(self, lo, hi, shape):
        return jax.random.randint(self._next(), shape, lo, hi, dtype=jnp.int32)

    def uniform(self, shape, lo=0.0, hi=1.0):
        return jax.random.uniform(self._next(), shape, jnp.bfloat16, lo, hi)

    def permutation(self, n):
        return jax.random.permutation(self._next(), n)
kernel_name = 'standalone__conformer_family_conformer__speech'

def setup_inputs():
    _rng = _Rng(jax.random.key(int.from_bytes(__import__("os").urandom(4), "little")))
    _w = lambda a: (lambda t: t.astype(jnp.bfloat16) if jnp.issubdtype(t.dtype, jnp.floating) else t)(jnp.asarray(a))
    B, T, D, K = (2, 4000, 512, 15)
    F = 4 * D
    s = D ** (-0.5)
    sf = F ** (-0.5)
    return {'x': _w((lambda *s: _rng.normal(s) * 0.05)(B, T, D)), 'w_ff1_a': _w((lambda *s: _rng.normal(s) * 0.05)(D, F) * s), 'w_ff1_b': _w((lambda *s: _rng.normal(s) * 0.05)(F, D) * sf), 'w_q': _w((lambda *s: _rng.normal(s) * 0.05)(D, D) * s), 'w_k': _w((lambda *s: _rng.normal(s) * 0.05)(D, D) * s), 'w_v': _w((lambda *s: _rng.normal(s) * 0.05)(D, D) * s), 'w_o': _w((lambda *s: _rng.normal(s) * 0.05)(D, D) * s), 'w_pw1': _w((lambda *s: _rng.normal(s) * 0.05)(D, 2 * D) * s), 'dw': _w((lambda *s: _rng.normal(s) * 0.05)(K, D) * K ** (-0.5)), 'w_pw2': _w((lambda *s: _rng.normal(s) * 0.05)(D, D) * s), 'w_ff2_a': _w((lambda *s: _rng.normal(s) * 0.05)(D, F) * s), 'w_ff2_b': _w((lambda *s: _rng.normal(s) * 0.05)(F, D) * sf)}

def reference(x, w_ff1_a, w_ff1_b, w_q, w_k, w_v, w_o, w_pw1, dw, w_pw2, w_ff2_a, w_ff2_b):
    B, T, D = x.shape
    K = dw.shape[0]
    scale = D ** (-0.5)
    h = _layernorm(x, axis=-1)
    h = _silu(h @ w_ff1_a) @ w_ff1_b
    x1 = x + 0.5 * h
    h = _layernorm(x1, axis=-1)
    q = h @ w_q
    k = h @ w_k
    v = h @ w_v
    scores = jnp.einsum('btd,bsd->bts', q, k) * scale
    p = _softmax(scores, axis=-1)
    attn = jnp.einsum('bts,bsd->btd', p, v) @ w_o
    x2 = x1 + attn
    h = _layernorm(x2, axis=-1)
    h = h @ w_pw1
    a = h[..., :D].copy()
    b = h[..., D:].copy()
    h = a * _sigmoid(b)
    pad = K // 2
    hp = jnp.pad(h, ((0, 0), (pad, K - 1 - pad), (0, 0)))
    dc = jnp.zeros_like(h)
    for i in range(K):
        dc = dc + hp[:, i:i + T, :] * dw[i][None, None, :]
    flat = dc.reshape(-1, D)
    mu = flat.mean(0)
    var = ((flat - mu) ** 2).mean(0)
    dc = (dc - mu[None, None, :]) / jnp.sqrt(var[None, None, :] + 1e-05)
    h = _silu(dc) @ w_pw2
    x3 = x2 + h
    h = _layernorm(x3, axis=-1)
    h = _silu(h @ w_ff2_a) @ w_ff2_b
    x4 = x3 + 0.5 * h
    return _layernorm(x4, axis=-1)
```

```python
import functools
import math

import jax
import jax.numpy as jnp
import jax.experimental.pallas as pl
import jax.experimental.pallas.tpu as pltpu

_LN_EPS = 1e-05
_BN_EPS = 1e-05
_LOG2E = 1.4426950408889634

R = 400
FC = 512
KC = 512
HALO = 8

_NT = (((1,), (1,)), ((), ()))
_F32 = jnp.float32
_BF16 = jnp.bfloat16


def _ln(x, scale=None):
    m = jnp.mean(x, axis=-1, keepdims=True)
    xc = x - m
    v = jnp.mean(xc * xc, axis=-1, keepdims=True)
    r = jax.lax.rsqrt(v + _LN_EPS)
    if scale is not None:
        r = r * scale
    return xc * r


def _ff(hb, wa_ref, wb_ref):
    F = wa_ref.shape[1]
    acc = None
    for c in range(F // FC):
        u = jnp.dot(hb, wa_ref[:, c * FC:(c + 1) * FC], preferred_element_type=_F32)
        a = (u + u * jnp.tanh(u)).astype(_BF16)
        d = jnp.dot(a, wb_ref[c * FC:(c + 1) * FC, :], preferred_element_type=_F32)
        acc = d if acc is None else acc + d
    return acc


def _kernel(x_hbm, wa1_h, wb1_h, wq_h, wk_h, wv_h, wo_h, wp1_h, dw_h, wp2_h, wa2_h, wb2_h,
            o_hbm,
            wa1, wb1, wq, wk, wv, wo, wp1, dwv, wp2, wa2, wb2, wm, wvo,
            xbuf, x1, hh, g, dc, sbuf, pbuf, obuf, wsem, xsem, osem,
            *, B, T, D, K):
    N = B * T
    NT = N // R
    TPB = T // R
    TP = hh.shape[1]
    scale = D ** -0.5

    w_pairs = [(wa1_h, wa1), (wb1_h, wb1), (wq_h, wq), (wk_h, wk), (wv_h, wv), (wo_h, wo),
               (wp1_h, wp1), (dw_h, dwv), (wp2_h, wp2), (wa2_h, wa2), (wb2_h, wb2)]
    w_copies = [pltpu.make_async_copy(s, d, wsem.at[i]) for i, (s, d) in enumerate(w_pairs)]

    def x_copy(i, slot):
        return pltpu.make_async_copy(x_hbm.at[pl.ds(pl.multiple_of(i * R, R), R), :],
                                     xbuf.at[slot], xsem.at[slot])

    def o_copy(i, slot):
        return pltpu.make_async_copy(obuf.at[slot],
                                     o_hbm.at[pl.ds(pl.multiple_of(i * R, R), R), :],
                                     osem.at[slot])

    x_copy(0, 0).start()
    for c in w_copies:
        c.start()

    for b in range(B):
        hh[b, T:TP, :] = jnp.zeros((TP - T, D), _BF16)
        for j in range(D // 128):
            g[b, j, 0:HALO, :] = jnp.zeros((HALO, 128), _F32)
            g[b, j, HALO + T:HALO + T + HALO, :] = jnp.zeros((HALO, 128), _F32)

    w_copies[0].wait()
    w_copies[1].wait()

    def phase_a(i, carry):
        slot = i % 2
        x_copy(i, slot).wait()

        @pl.when(i + 1 < NT)
        def _():
            x_copy(i + 1, 1 - slot).start()

        b = i // TPB
        r0 = pl.multiple_of((i - b * TPB) * R, 16)
        xt = xbuf[slot].astype(_F32)
        hb = _ln(xt, 0.5).astype(_BF16)
        f = _ff(hb, wa1, wb1)
        xr = xt + 0.5 * f
        x1[b, pl.ds(r0, R), :] = xr
        hh[b, pl.ds(r0, R), :] = _ln(xr).astype(_BF16)
        return carry

    jax.lax.fori_loop(0, NT, phase_a, 0)

    for c in w_copies[2:]:
        c.wait()
    wm[...] = (jax.lax.dot_general(wq[...], wk[...], _NT, preferred_element_type=_F32)
               * (scale * _LOG2E)).astype(_BF16)
    wvo[...] = jnp.dot(wv[...], wo[...], preferred_element_type=_F32).astype(_BF16)

    def phase_b(i, carry):
        b = i // TPB
        r0 = pl.multiple_of((i - b * TPB) * R, 16)
        q = jnp.dot(hh[b, pl.ds(r0, R), :], wm[...], preferred_element_type=_F32).astype(_BF16)
        m = None
        NC = TP // KC
        for c in range(NC):
            s = jax.lax.dot_general(q, hh[b, c * KC:(c + 1) * KC, :], _NT,
                                    preferred_element_type=_F32)
            if (c + 1) * KC > T:
                col = jax.lax.broadcasted_iota(jnp.int32, s.shape, 1) + c * KC
                s = jnp.where(col < T, s, -1e30)
            sbuf[:, c * KC:(c + 1) * KC] = s
            mc = jnp.max(s, axis=-1, keepdims=True)
            m = mc if m is None else jnp.maximum(m, mc)
        l = None
        acc = None
        for c in range(NC):
            p = jnp.exp2(sbuf[:, c * KC:(c + 1) * KC] - m)
            lc = jnp.sum(p, axis=-1, keepdims=True)
            l = lc if l is None else l + lc
            d = jnp.dot(p.astype(_BF16), hh[b, c * KC:(c + 1) * KC, :], preferred_element_type=_F32)
            acc = d if acc is None else acc + d
        o = (acc * (1.0 / l)).astype(_BF16)
        x2 = x1[b, pl.ds(r0, R), :] + jnp.dot(o, wvo[...], preferred_element_type=_F32)
        x1[b, pl.ds(r0, R), :] = x2
        hb = _ln(x2).astype(_BF16)
        ab = jnp.dot(hb, wp1[...], preferred_element_type=_F32)
        a = ab[:, :D] * 0.5
        gl = a + a * jnp.tanh(ab[:, D:] * 0.5)
        for j in range(D // 128):
            g[b, j, pl.ds(r0 + HALO, R), :] = gl[:, j * 128:(j + 1) * 128]
        return carry

    jax.lax.fori_loop(0, NT, phase_b, 0)

    CR = 80
    pad = K // 2

    def conv_body(i, ssum):
        b = i // (T // CR)
        r0 = pl.multiple_of((i - b * (T // CR)) * CR, 8)
        cols = []
        for j in range(D // 128):
            acc = None
            for k in range(K):
                t = (g[b, j, pl.ds(r0 + HALO - pad + k, CR), :]
                     * dwv[k:k + 1, j * 128:(j + 1) * 128].astype(_F32))
                acc = t if acc is None else acc + t
            cols.append(acc)
        acc = jnp.concatenate(cols, axis=1)
        dc[b, pl.ds(r0, CR), :] = acc
        return ssum + jnp.sum(acc, axis=0, keepdims=True)

    ssum = jax.lax.fori_loop(0, N // CR, conv_body, jnp.zeros((1, D), _F32))
    mu = ssum * (1.0 / N)

    def var_body(i, vsum):
        b = i // (T // CR)
        r0 = pl.multiple_of((i - b * (T // CR)) * CR, 8)
        dd = dc[b, pl.ds(r0, CR), :] - mu
        return vsum + jnp.sum(dd * dd, axis=0, keepdims=True)

    vsum = jax.lax.fori_loop(0, N // CR, var_body, jnp.zeros((1, D), _F32))
    rstd = jax.lax.rsqrt(vsum * (1.0 / N) + _BN_EPS) * 0.5

    def phase_d(i, carry):
        slot = i % 2
        b = i // TPB
        r0 = pl.multiple_of((i - b * TPB) * R, 16)
        u = (dc[b, pl.ds(r0, R), :] - mu) * rstd
        a = (u + u * jnp.tanh(u)).astype(_BF16)
        x3 = x1[b, pl.ds(r0, R), :] + jnp.dot(a, wp2[...], preferred_element_type=_F32)
        hb = _ln(x3, 0.5).astype(_BF16)
        f = _ff(hb, wa2, wb2)
        x4 = x3 + 0.5 * f
        y = _ln(x4).astype(_BF16)

        @pl.when(i >= 2)
        def _():
            o_copy(i - 2, slot).wait()

        obuf[slot] = y
        o_copy(i, slot).start()
        return carry

    jax.lax.fori_loop(0, NT, phase_d, 0)
    o_copy(NT - 2, 0).wait()
    o_copy(NT - 1, 1).wait()


@jax.jit
def pallas_standalone__conformer_family_conformer__speech_kernel(
    x: jax.Array,
    w_ff1_a: jax.Array,
    w_ff1_b: jax.Array,
    w_q: jax.Array,
    w_k: jax.Array,
    w_v: jax.Array,
    w_o: jax.Array,
    w_pw1: jax.Array,
    dw: jax.Array,
    w_pw2: jax.Array,
    w_ff2_a: jax.Array,
    w_ff2_b: jax.Array,
):
    B, T, D = x.shape
    K = dw.shape[0]
    F = w_ff1_a.shape[1]
    N = B * T
    TP = -(-T // KC) * KC
    assert T % R == 0 and K // 2 <= HALO and K - 1 - K // 2 <= HALO

    weights = (w_ff1_a, w_ff1_b, w_q, w_k, w_v, w_o, w_pw1, dw, w_pw2, w_ff2_a, w_ff2_b)
    scratch = [pltpu.VMEM(w.shape, w.dtype) for w in weights]
    scratch += [
        pltpu.VMEM((D, D), _BF16),
        pltpu.VMEM((D, D), _BF16),
        pltpu.VMEM((2, R, D), x.dtype),
        pltpu.VMEM((B, T, D), _F32),
        pltpu.VMEM((B, TP, D), _BF16),
        pltpu.VMEM((B, D // 128, T + 2 * HALO, 128), _F32),
        pltpu.VMEM((B, T, D), _F32),
        pltpu.VMEM((R, TP), _F32),
        pltpu.VMEM((R, TP), _BF16),
        pltpu.VMEM((2, R, D), x.dtype),
        pltpu.SemaphoreType.DMA((len(weights),)),
        pltpu.SemaphoreType.DMA((2,)),
        pltpu.SemaphoreType.DMA((2,)),
    ]
    out = pl.pallas_call(
        functools.partial(_kernel, B=B, T=T, D=D, K=K),
        out_shape=jax.ShapeDtypeStruct((N, D), x.dtype),
        in_specs=[pl.BlockSpec(memory_space=pl.ANY)] * (1 + len(weights)),
        out_specs=pl.BlockSpec(memory_space=pl.ANY),
        scratch_shapes=scratch,
        compiler_params=pltpu.CompilerParams(vmem_limit_bytes=120 * 2**20),
        name="conformer",
    )(x.reshape(N, D), *weights)
    return out.reshape(B, T, D)
```

```python
import functools

import jax
import jax.numpy as jnp
import numpy as np
import jax.experimental.pallas as pl
import jax.experimental.pallas.tpu as pltpu

_EPS = 1e-05
_LOG2E = 1.4426950408889634

R = 400
FC = 512
HALO = 8
L = 128

CFG = dict(CP=40, cstart=1, cevery=1, lsum='tile', lnp=10, lstart=52, levery=1,
           egn=2, egr=25, fin=70)

_NT = (((1,), (1,)), ((), ()))
_F32 = jnp.float32
_BF16 = jnp.bfloat16
_U32 = jnp.uint32


def _cat(xs, axis=1):
    return jnp.concatenate(xs, axis=axis)


def _bf(x):
    return pltpu.bitcast(x, _BF16)


def _ln(x, scale=None):
    d = x.shape[-1]
    m = jnp.sum(x, axis=-1, keepdims=True) * (1.0 / d)
    xc = x - m
    v = jnp.sum(xc * xc, axis=-1, keepdims=True) * (1.0 / d)
    r = jax.lax.rsqrt(v + _EPS)
    if scale is not None:
        r = r * scale
    return xc * r


def _kernel(zero_ref,
            x_hbm, wa1_h, wb1_h, wq_h, wk_h, wv_h, wo_h, wp1_h, dw_h, wp2_h, wa2_h, wb2_h,
            o_hbm,
            wa1, wb1, wq, wk, wv, wo, wp1, dwv, wp2, wa2, wb2, wm, wvo,
            xall, x1, hh, g, dc, sbuf, hb, acc, oacc, qbuf, o16, h3b, lbuf, mbuf, dwf, tmean,
            wsem, xsem,
            *, B, T, D, K):
    N = B * T
    NT = N // R
    TPB = T // R
    TP = hh.shape[2]
    F = wa1.shape[1]
    NK = TP // L
    ND = D // L
    scale = D ** -0.5
    pad = K // 2
    cfg = CFG
    hh32 = hh.bitcast(_U32)

    def w_copy(src, dst, k):
        return pltpu.make_async_copy(src, dst, wsem.at[k])

    def col_copies(src, dst, k0):
        return [pltpu.make_async_copy(src.at[:, pl.ds(n * L, L)], dst.at[n], wsem.at[k0 + n])
                for n in range(dst.shape[0])]

    c_wa1, c_wb1 = w_copy(wa1_h, wa1, 0), w_copy(wb1_h, wb1, 1)
    c_rest = [w_copy(wq_h, wq, 2), w_copy(wk_h, wk, 3), w_copy(wv_h, wv, 4), w_copy(wo_h, wo, 5),
              w_copy(dw_h, dwv, 6), w_copy(wp2_h, wp2, 7), w_copy(wa2_h, wa2, 8),
              w_copy(wb2_h, wb2, 9)] + col_copies(wp1_h, wp1, 10)

    def rows(i):
        return i * R if isinstance(i, int) else pl.multiple_of(i * R, 16)

    def x_copy(i):
        return pltpu.make_async_copy(x_hbm.at[pl.ds(rows(i), R), :], xall.at[pl.ds(rows(i), R), :],
                                     xsem.at[i])

    def o_copy(i):
        return pltpu.make_async_copy(xall.at[pl.ds(rows(i), R), :], o_hbm.at[pl.ds(rows(i), R), :],
                                     xsem.at[i])

    def tile(i):
        if isinstance(i, int):
            return i // TPB, (i % TPB) * R
        b = i // TPB
        return b, pl.multiple_of((i - b * TPB) * R, 16)

    def ld_x(i):
        b, r0 = tile(i)
        return _cat([x1[b, n, pl.ds(r0, R), :] for n in range(ND)])

    def st_cols(ref, i, v):
        b, r0 = tile(i)
        for n in range(ND):
            ref[b, n, pl.ds(r0, R), :] = v[:, n * L:(n + 1) * L]

    x_copy(0).start()
    c_wa1.start()
    c_wb1.start()
    for t in range(1, NT):
        x_copy(t).start()
    for c in c_rest:
        c.start()

    for b in range(B):
        for n in range(ND):
            hh[b, n, T:TP, :] = jnp.zeros((TP - T, L), _BF16)
            g[b, n, 0:2 * HALO, :] = jnp.zeros((2 * HALO, L), _F32)
            g[b, n, 2 * HALO + T:, :] = jnp.zeros((2 * HALO, L), _F32)
        dc[b, 0:HALO, :] = jnp.zeros((HALO, D), _F32)

    def ff(wa, wb, mid=None):
        NF = F // FC
        hid = {}

        def up(c):
            u = jnp.dot(hb[...], wa[:, c * FC:(c + 1) * FC], preferred_element_type=_F32)
            hid[c] = (u + u * jnp.tanh(u)).astype(_BF16)

        def down(c):
            d = jnp.dot(hid.pop(c), wb[c * FC:(c + 1) * FC, :], preferred_element_type=_F32)
            if c == 0:
                acc[...] = d
            else:
                acc[...] += d

        up(0)
        for c in range(NF):
            if c + 1 < NF:
                up(c + 1)
            if c == NF - 2 and mid is not None:
                mid()
            down(c)

    def ln1(i):
        hb[...] = _ln(xall[pl.ds(rows(i), R), :].astype(_F32), 0.5).astype(_BF16)

    def post_a(i):
        xr = xall[pl.ds(rows(i), R), :].astype(_F32) + 0.5 * acc[...]
        st_cols(x1, i, xr)
        st_cols(hh, i, _ln(xr).astype(_BF16))

    x_copy(0).wait()
    ln1(0)
    c_wa1.wait()
    c_wb1.wait()
    ff(wa1, wb1)
    x_copy(1).wait()
    ln1(1)

    def phase_a(i, carry):
        x_copy(i + 1).wait()
        post_a(i - 1)
        ff(wa1, wb1)
        ln1(i + 1)
        return carry

    jax.lax.fori_loop(1, NT - 1, phase_a, 0)
    post_a(NT - 2)
    ff(wa1, wb1)
    post_a(NT - 1)

    for c in c_rest:
        c.wait()
    for n in range(ND):
        wm[n] = (jax.lax.dot_general(wq[...], wk[n * L:(n + 1) * L, :], _NT,
                                     preferred_element_type=_F32)
                 * (scale * _LOG2E)).astype(_BF16)
        wvo[n] = jnp.dot(wv[...], wo[:, n * L:(n + 1) * L],
                         preferred_element_type=_F32).astype(_BF16)
    dwf[...] = dwv[...].astype(_F32)

    CP = cfg['CP']
    CW = R + HALO
    piece_rows = [(p * CP, CP) for p in range(R // CP)] + [(R, HALO)]

    def q_proj(i, after_pass=lambda d: None):
        b, r0 = tile(i)
        r = r0 // 2 if isinstance(r0, int) else pl.multiple_of(r0 // 2, 8)
        h = _cat([_bf(hh32[b, j, pl.ds(r, R // 2), :]) for j in range(ND)])
        for n in range(ND):
            d = jnp.dot(h, wm[n], preferred_element_type=_F32)
            qbuf[n] = d.astype(_BF16)
            after_pass(d)

    def step_b(i, stats, cur=True, prev=True, conv=True, nxt=True):
        z0 = zero_ref[0]
        nz = [0]

        def fresh(ref):
            nz[0] += 1
            z = pl.multiple_of(z0 * nz[0], 8)
            r32 = ref.bitcast(_U32)
            return _cat([_bf(r32[j, pl.ds(z, R // 2), :]) for j in range(ND)])

        st = dict(psum=None, stats=stats)
        k = i - 2

        def conv_valid(w0, n):
            _, r0 = tile(k)
            row = jax.lax.broadcasted_iota(jnp.int32, (n, 1), 0) + (r0 + (w0 - HALO))
            ok = row >= 0
            if w0 + n > R:
                ok = jnp.logical_and(ok, jnp.logical_or(row < r0 + R - HALO, r0 == T - R))
            return ok

        def conv_piece(p):
            b, r0 = tile(k)
            w0, n = piece_rows[p]
            cols = []
            for j in range(ND):
                a = None
                for t in range(K):
                    v = (g[b, j, pl.ds(r0 + w0 + HALO - pad + t, n), :]
                         * dwf[t:t + 1, j * L:(j + 1) * L])
                    a = v if a is None else a + v
                cols.append(a)
            a = _cat(cols)
            dc[b, pl.ds(r0 + w0, n), :] = a
            if w0 == 0 or w0 + n > R:
                a = jnp.where(conv_valid(w0, n), a, 0.0)
            ps = jnp.sum(a.reshape(n // 8, 8, D), axis=0)
            st['psum'] = ps if st['psum'] is None else st['psum'] + ps

        def conv_finish():
            b, r0 = tile(k)
            psum = st['psum']
            cnt = (R - HALO * jnp.asarray(r0 == 0, jnp.int32)
                   + HALO * jnp.asarray(r0 == T - R, jnp.int32)).astype(_F32)
            mu = jnp.sum(psum, axis=0, keepdims=True) / cnt
            dd = dc[b, pl.ds(r0, CW), :] - mu
            dd = jnp.where(conv_valid(0, CW), dd * dd, 0.0)
            tmean[pl.ds(k, 1), :] = mu
            s = st['stats']
            st['stats'] = (s[0] + psum, s[1] + jnp.sum(dd.reshape(CW // 8, 8, D), axis=0))

        def ln3_part(part):
            b, r0 = tile(i - 1)
            rs = R // cfg['lnp']
            x2 = _cat([x1[b, n, pl.ds(pl.multiple_of(r0 + part * rs + z0, 8), rs), :]
                       for n in range(ND)])
            h = _ln(x2, 0.5).astype(_BF16)
            for n in range(ND):
                h3b[n, part * rs:(part + 1) * rs, :] = h[:, n * L:(n + 1) * L]

        def exp_chunk(c):
            ps = []
            lc = None
            for n in range(ND * c, ND * c + ND):
                p = jnp.exp2(sbuf[n] - st['m'])
                ps.append(p.astype(_BF16))
                if cfg['lsum'] == 'tile':
                    if n == 0:
                        lbuf[...] = p
                    else:
                        lbuf[...] += p
                else:
                    lc = p if lc is None else lc + p
            if cfg['lsum'] != 'tile':
                if c == 0:
                    lbuf[...] = lc
                else:
                    lbuf[...] += lc
            return _cat(ps)

        def gate_g(d):
            g[z0, 0, pl.ds(T + 3 * HALO, 8), :] = d[0:8, :]

        def gate_x(d):
            x1[z0, 0, pl.ds(T, 8), :] = d[0:8, :]

        def gate_s(d):
            r = cfg['egr'] * 8
            sbuf[z0 + NK, 0:8, :] = d[r:r + 8, :]

        def gate_dc(d):
            dc[z0, pl.ds(T + HALO, 8), 0:L] = d[0:8, :]

        jobs = {}

        def add(t, gate, fn):
            jobs.setdefault(t, []).append((gate, fn))

        if conv:
            for p in range(len(piece_rows)):
                add(cfg['cstart'] + p * cfg['cevery'], gate_g, functools.partial(conv_piece, p))
            add(cfg['fin'], gate_dc, conv_finish)
        if prev:
            for p in range(cfg['lnp']):
                add(cfg['lstart'] + p * cfg['levery'], gate_x, functools.partial(ln3_part, p))

        def after_pass(t, d):
            for gate, fn in jobs.pop(t, []):
                gate(d)
                fn()

        def flush(lo, hi):
            for t in range(lo, hi):
                for _, fn in jobs.pop(t, []):
                    fn()

        T_S, T_W, T_O, T_Q, T_P = 0, NK, NK + ND, 2 * NK + ND, 2 * NK + 2 * ND
        b, _ = tile(i) if cur else (None, None)
        if cur:
            for n in range(NK):
                keys = _cat([_bf(hh32[b, j, pl.ds(n * L // 2, L // 2), :]) for j in range(ND)])
                s = jax.lax.dot_general(fresh(qbuf), keys, _NT, preferred_element_type=_F32)
                if (n + 1) * L > T:
                    col = jax.lax.broadcasted_iota(jnp.int32, (1, L), 1) + n * L
                    s = jnp.where(col < T, s, -1e30)
                sbuf[n] = s
                if n == 0:
                    mbuf[...] = s
                else:
                    mbuf[...] = jnp.maximum(mbuf[...], s)
                after_pass(T_S + n, s)
            st['m'] = jnp.max(mbuf[...], axis=-1, keepdims=True)
        else:
            flush(T_S, T_W)
        if prev:
            b1, r1 = tile(i - 1)
            for n in range(ND):
                d = jnp.dot(fresh(o16), wvo[n], preferred_element_type=_F32)
                x1[b1, n, pl.ds(r1, R), :] += d
                after_pass(T_W + n, d)
        else:
            flush(T_W, T_O)
        if cur:
            NC = NK // ND
            p = exp_chunk(0)
            for c in range(NC):
                pn = None
                for n in range(ND):
                    v = _bf(hh32[b, n, pl.ds(c * ND * L // 2, ND * L // 2), :])
                    d = jnp.dot(p, v, preferred_element_type=_F32)
                    if c == 0:
                        oacc[n] = d
                    else:
                        oacc[n] += d
                    if n == cfg['egn'] and c + 1 < NC:
                        gate_s(d)
                        pn = exp_chunk(c + 1)
                    after_pass(T_O + c * ND + n, d)
                p = pn
            r = 1.0 / jnp.sum(lbuf[...], axis=-1, keepdims=True)
            for n in range(ND):
                o16[n] = (oacc[n] * r).astype(_BF16)
        else:
            flush(T_O, T_Q)
        if nxt:
            cnt = [T_Q]

            def ap(d):
                after_pass(cnt[0], d)
                cnt[0] += 1
            q_proj(i + 1, ap)
        else:
            flush(T_Q, T_P)
        if prev:
            for n in range(ND):
                a = jnp.dot(fresh(h3b), wp1[n], preferred_element_type=_F32)
                after_pass(T_P + 2 * n, a)
                bb = jnp.dot(fresh(h3b), wp1[ND + n], preferred_element_type=_F32)
                g[b1, n, pl.ds(r1 + 2 * HALO, R), :] = a + a * jnp.tanh(bb)
                after_pass(T_P + 2 * n + 1, bb)
        flush(0, T_P + 2 * ND)
        return st['stats']

    stats = (jnp.zeros((8, D), _F32), jnp.zeros((8, D), _F32))
    q_proj(0)
    stats = step_b(0, stats, prev=False, conv=False)
    stats = step_b(1, stats, conv=False)
    stats = jax.lax.fori_loop(2, NT - 1, step_b, stats)
    stats = step_b(NT - 1, stats, nxt=False)
    stats = step_b(NT, stats, cur=False, nxt=False)
    stats = step_b(NT + 1, stats, cur=False, prev=False, nxt=False)

    mu = jnp.sum(stats[0], axis=0, keepdims=True) * (1.0 / N)
    dm = tmean[...] - mu
    trow = jax.lax.broadcasted_iota(jnp.int32, (NT, 1), 0) % TPB
    tcnt = (R - HALO * (trow == 0).astype(jnp.int32)
            + HALO * (trow == TPB - 1).astype(jnp.int32)).astype(_F32)
    var = (jnp.sum(stats[1], axis=0, keepdims=True)
           + jnp.sum(dm * dm * tcnt, axis=0, keepdims=True)) * (1.0 / N)
    rstd = jax.lax.rsqrt(var + _EPS) * 0.5

    def pw2(i):
        b, r0 = tile(i)
        u = (dc[b, pl.ds(r0 + HALO, R), :] - mu) * rstd
        a = (u + u * jnp.tanh(u)).astype(_BF16)
        st_cols(x1, i, ld_x(i) + jnp.dot(a, wp2[...], preferred_element_type=_F32))

    def ln4(i):
        hb[...] = _ln(ld_x(i), 0.5).astype(_BF16)

    def post_d(i):
        xall[pl.ds(rows(i), R), :] = _ln(ld_x(i) + 0.5 * acc[...]).astype(_BF16)
        o_copy(i).start()

    pw2(0)
    ln4(0)
    ff(wa2, wb2, mid=lambda: pw2(1))
    ln4(1)

    def phase_d(i, carry):
        post_d(i - 1)
        ff(wa2, wb2, mid=lambda: pw2(i + 1))
        ln4(i + 1)
        return carry

    jax.lax.fori_loop(1, NT - 1, phase_d, 0)
    post_d(NT - 2)
    ff(wa2, wb2)
    post_d(NT - 1)
    for t in range(NT):
        o_copy(t).wait()


@jax.jit
def pallas_standalone__conformer_family_conformer__speech_kernel(
    x: jax.Array,
    w_ff1_a: jax.Array,
    w_ff1_b: jax.Array,
    w_q: jax.Array,
    w_k: jax.Array,
    w_v: jax.Array,
    w_o: jax.Array,
    w_pw1: jax.Array,
    dw: jax.Array,
    w_pw2: jax.Array,
    w_ff2_a: jax.Array,
    w_ff2_b: jax.Array,
):
    B, T, D = x.shape
    K = dw.shape[0]
    N = B * T
    TP = -(-T // D) * D
    ND = D // L
    assert T % R == 0 and K // 2 <= HALO and K - 1 - K // 2 <= HALO and D % L == 0

    weights = (w_ff1_a, w_ff1_b, w_q, w_k, w_v, w_o, w_pw1, dw, w_pw2, w_ff2_a, w_ff2_b)
    V = pltpu.VMEM
    scratch = [V(w.shape, w.dtype) for w in weights[:6]]
    scratch += [V((2 * ND, D, L), _BF16)]
    scratch += [V(w.shape, w.dtype) for w in weights[7:]]
    scratch += [
        V((ND, D, L), _BF16),
        V((ND, D, L), _BF16),
        V((N, D), x.dtype),
        V((B, ND, T + 8, L), _F32),
        V((B, ND, TP, L), _BF16),
        V((B, ND, T + 4 * HALO, L), _F32),
        V((B, T + 2 * HALO, D), _F32),
        V((TP // L + 1, R, L), _F32),
        V((R, D), _BF16),
        V((R, D), _F32),
        V((ND, R, L), _F32),
        V((ND, R, L), _BF16),
        V((ND, R, L), _BF16),
        V((ND, R, L), _BF16),
        V((R, L), _F32),
        V((R, L), _F32),
        V((K, D), _F32),
        V((N // R, D), _F32),
        pltpu.SemaphoreType.DMA((10 + 2 * ND,)),
        pltpu.SemaphoreType.DMA((N // R,)),
    ]
    out = pl.pallas_call(
        functools.partial(_kernel, B=B, T=T, D=D, K=K),
        out_shape=jax.ShapeDtypeStruct((N, D), x.dtype),
        in_specs=([pl.BlockSpec(memory_space=pltpu.SMEM)]
                  + [pl.BlockSpec(memory_space=pl.ANY)] * (1 + len(weights))),
        out_specs=pl.BlockSpec(memory_space=pl.ANY),
        scratch_shapes=scratch,
        compiler_params=pltpu.CompilerParams(
            vmem_limit_bytes=120 * 2**20,
            flags={"XLA_TPU_EVENLY_DISTRIBUTE_CRITICAL_NODES": True},
        ),
        name="conformer",
    )(np.zeros((1,), np.int32), x.reshape(N, D), *weights)
    return out.reshape(B, T, D)
```

```python
import functools

import jax
import jax.numpy as jnp
import numpy as np
import jax.experimental.pallas as pl
import jax.experimental.pallas.tpu as pltpu

_EPS = 1e-05
_LOG2E = 1.4426950408889634

R = 400
FC = 512
HALO = 8
L = 128

CFG = dict(CP=40, cstart=2, cevery=1, lsum='tile', lnp=10, lstart=37, levery=2,
           egn=3, egr=10, fin=66, nfin=3, fevery=2, cgate='mem')

_NT = (((1,), (1,)), ((), ()))
_F32 = jnp.float32
_BF16 = jnp.bfloat16
_U32 = jnp.uint32


def _cat(xs, axis=1):
    return jnp.concatenate(xs, axis=axis)


def _bf(x):
    return pltpu.bitcast(x, _BF16)


def _ln(x, scale=None):
    d = x.shape[-1]
    m = jnp.sum(x, axis=-1, keepdims=True) * (1.0 / d)
    xc = x - m
    v = jnp.sum(xc * xc, axis=-1, keepdims=True) * (1.0 / d)
    r = jax.lax.rsqrt(v + _EPS)
    if scale is not None:
        r = r * scale
    return xc * r


def _kernel(zero_ref, kbias,
            x_hbm, wa1_h, wb1_h, wq_h, wk_h, wv_h, wo_h, wp1_h, dw_h, wp2_h, wa2_h, wb2_h,
            o_hbm,
            wa1, wb1, wq, wk, wv, wo, wp1, dwv, wp2, wa2, wb2, wm, wvo,
            xall, x1, hh, g, dc, sbuf, hb, acc, qbuf, o16, h3b, rbuf, dwf, tmean,
            wsem, xsem,
            *, B, T, D, K):
    N = B * T
    NT = N // R
    TPB = T // R
    TP = hh.shape[2]
    F = wa1.shape[1]
    NK = TP // L
    ND = D // L
    scale = D ** -0.5
    pad = K // 2
    cfg = CFG
    hh32 = hh.bitcast(_U32)

    def w_copy(src, dst, k):
        return pltpu.make_async_copy(src, dst, wsem.at[k])

    def col_copies(src, dst, k0):
        return [pltpu.make_async_copy(src.at[:, pl.ds(n * L, L)], dst.at[n], wsem.at[k0 + n])
                for n in range(dst.shape[0])]

    c_wa1, c_wb1 = w_copy(wa1_h, wa1, 0), w_copy(wb1_h, wb1, 1)
    c_rest = [w_copy(wq_h, wq, 2), w_copy(wk_h, wk, 3), w_copy(wv_h, wv, 4), w_copy(wo_h, wo, 5),
              w_copy(dw_h, dwv, 6), w_copy(wp2_h, wp2, 7), w_copy(wa2_h, wa2, 8),
              w_copy(wb2_h, wb2, 9)] + col_copies(wp1_h, wp1, 10)

    def rows(i):
        return i * R if isinstance(i, int) else pl.multiple_of(i * R, 16)

    def x_copy(i):
        return pltpu.make_async_copy(x_hbm.at[pl.ds(rows(i), R), :], xall.at[pl.ds(rows(i), R), :],
                                     xsem.at[i])

    def o_copy(i):
        return pltpu.make_async_copy(xall.at[pl.ds(rows(i), R), :], o_hbm.at[pl.ds(rows(i), R), :],
                                     xsem.at[i])

    def tile(i):
        if isinstance(i, int):
            return i // TPB, (i % TPB) * R
        b = i // TPB
        return b, pl.multiple_of((i - b * TPB) * R, 16)

    def ld_x(i):
        b, r0 = tile(i)
        return _cat([x1[b, n, pl.ds(r0, R), :] for n in range(ND)])

    def st_cols(ref, i, v):
        b, r0 = tile(i)
        for n in range(ND):
            ref[b, n, pl.ds(r0, R), :] = v[:, n * L:(n + 1) * L]

    x_copy(0).start()
    c_wa1.start()
    c_wb1.start()
    for t in range(1, NT):
        x_copy(t).start()
    for c in c_rest:
        c.start()

    for b in range(B):
        for n in range(ND):
            hh[b, n, T:TP, :] = jnp.zeros((TP - T, L), _BF16)
            g[b, n, 0:2 * HALO, :] = jnp.zeros((2 * HALO, L), _F32)
            g[b, n, 2 * HALO + T:, :] = jnp.zeros((2 * HALO, L), _F32)
        dc[b, 0:HALO, :] = jnp.zeros((HALO, D), _F32)

    def ff(wa, wb, mid=None):
        NF = F // FC
        hid = {}

        def up(c):
            u = jnp.dot(hb[...], wa[:, c * FC:(c + 1) * FC], preferred_element_type=_F32)
            hid[c] = (u + u * jnp.tanh(u)).astype(_BF16)

        def down(c):
            d = jnp.dot(hid.pop(c), wb[c * FC:(c + 1) * FC, :], preferred_element_type=_F32)
            if c == 0:
                acc[...] = d
            else:
                acc[...] += d

        up(0)
        for c in range(NF):
            if c + 1 < NF:
                up(c + 1)
            if c == NF - 2 and mid is not None:
                mid()
            down(c)

    def ln1(i):
        hb[...] = _ln(xall[pl.ds(rows(i), R), :].astype(_F32), 0.5).astype(_BF16)

    def post_a(i):
        xr = xall[pl.ds(rows(i), R), :].astype(_F32) + 0.5 * acc[...]
        st_cols(x1, i, xr)
        st_cols(hh, i, _ln(xr).astype(_BF16))

    x_copy(0).wait()
    ln1(0)
    c_wa1.wait()
    c_wb1.wait()
    ff(wa1, wb1)
    x_copy(1).wait()
    ln1(1)

    def phase_a(i, carry):
        x_copy(i + 1).wait()
        post_a(i - 1)
        ff(wa1, wb1)
        ln1(i + 1)
        return carry

    jax.lax.fori_loop(1, NT - 1, phase_a, 0)
    post_a(NT - 2)
    ff(wa1, wb1)
    post_a(NT - 1)

    for c in c_rest:
        c.wait()
    for n in range(ND):
        wm[n] = (jax.lax.dot_general(wq[...], wk[n * L:(n + 1) * L, :], _NT,
                                     preferred_element_type=_F32)
                 * (scale * _LOG2E)).astype(_BF16)
        wvo[n] = jnp.dot(wv[...], wo[:, n * L:(n + 1) * L],
                         preferred_element_type=_F32).astype(_BF16)
    dwf[...] = dwv[...].astype(_F32)

    CP = cfg['CP']
    CW = R + HALO
    piece_rows = [(p * CP, CP) for p in range(R // CP)] + [(R, HALO)]

    def q_proj(i, after_pass=lambda d: None):
        b, r0 = tile(i)
        r = r0 // 2 if isinstance(r0, int) else pl.multiple_of(r0 // 2, 8)
        h = _cat([_bf(hh32[b, j, pl.ds(r, R // 2), :]) for j in range(ND)])
        for n in range(ND):
            d = jnp.dot(h, wm[n], preferred_element_type=_F32)
            qbuf[n] = d.astype(_BF16)
            after_pass(d)

    def step_b(i, stats, cur=True, prev=True, conv=True, nxt=True):
        z0 = zero_ref[0]
        nz = [0]

        def fresh(ref):
            nz[0] += 1
            z = pl.multiple_of(z0 * nz[0], 8)
            r32 = ref.bitcast(_U32)
            return _cat([_bf(r32[j, pl.ds(z, R // 2), :]) for j in range(ND)])

        st = dict(psum=None, stats=stats)
        k = i - 2

        def edge_mask(w0, a):
            _, r0 = tile(k)
            n = a.shape[0]
            parts = [a]
            if w0 == 0:
                parts = [jnp.where(r0 > 0, a[:HALO], 0.0), a[HALO:]]
            if w0 + n > R:
                h = parts[-1]
                cut = h.shape[0] - HALO
                parts[-1:] = [h[:cut], jnp.where(r0 == T - R, h[cut:], 0.0)]
            parts = [q for q in parts if q.shape[0]]
            return parts[0] if len(parts) == 1 else _cat(parts, 0)

        def conv_piece(p):
            b, r0 = tile(k)
            w0, n = piece_rows[p]
            cols = []
            for j in range(ND):
                win = g[b, j, pl.ds(r0 + w0, n + 2 * HALO), :]
                a = None
                if cfg['cgate'] == 'data':
                    win = jnp.where(never, jnp.broadcast_to(st['tok'], win.shape), win) \
                        if cfg.get('cg', 0) == 0 else win
                for t in range(K):
                    o = HALO - pad + t
                    v = win[o:o + n, :] * dwf[t:t + 1, j * L:(j + 1) * L]
                    a = v if a is None else a + v
                cols.append(a)
            a = _cat(cols)
            dc[b, pl.ds(r0 + w0, n), :] = a
            ps = jnp.sum(edge_mask(w0, a).reshape(n // 8, 8, D), axis=0)
            st['psum'] = ps if st['psum'] is None else st['psum'] + ps

        def conv_finish(part):
            b, r0 = tile(k)
            nparts = cfg['nfin']
            if part == 0:
                cnt = (R - HALO * jnp.asarray(r0 == 0, jnp.int32)
                       + HALO * jnp.asarray(r0 == T - R, jnp.int32)).astype(_F32)
                st['mu'] = jnp.sum(st['psum'], axis=0, keepdims=True) / cnt
                tmean[pl.ds(k, 1), :] = st['mu']
            lo = (CW // 8 * part // nparts) * 8
            hi = (CW // 8 * (part + 1) // nparts) * 8
            dd = dc[b, pl.ds(r0 + lo, hi - lo), :] - st['mu']
            m2 = jnp.sum(edge_mask(lo, dd * dd).reshape((hi - lo) // 8, 8, D), axis=0)
            s = st['stats']
            st['stats'] = (s[0] + st['psum'] if part == 0 else s[0], s[1] + m2)

        def ln3_part(part):
            b, r0 = tile(i - 1)
            rs = R // cfg['lnp']
            x2 = _cat([x1[b, n, pl.ds(pl.multiple_of(r0 + part * rs + z0, 8), rs), :]
                       for n in range(ND)])
            h = _ln(x2, 0.5).astype(_BF16)
            for n in range(ND):
                h3b[n, part * rs:(part + 1) * rs, :] = h[:, n * L:(n + 1) * L]

        def exp_chunk(c):
            ps = []
            for n in range(ND * c, ND * c + ND):
                p = jnp.exp2(sbuf[n] - st['m'])
                ps.append(p.astype(_BF16))
                st['l'] = p if n == 0 else st['l'] + p
            return _cat(ps)

        never = z0 > 0

        def gate_g(d):
            if cfg['cgate'] == 'data':
                st['tok'] = d[0:1, 0:1]
            else:
                g[z0, 0, pl.ds(T + 3 * HALO, 8), :] = d[0:8, :]

        def gate_x(d):
            x1[z0, 0, pl.ds(T, 8), :] = d[0:8, :]

        def gate_s(d):
            r = cfg['egr'] * 8
            sbuf[z0 + NK, 0:8, :] = d[r:r + 8, :]

        def gate_dc(d):
            dc[z0, pl.ds(T + HALO, 8), 0:L] = d[0:8, :]

        jobs = {}

        def add(t, gate, fn):
            jobs.setdefault(t, []).append((gate, fn))

        if conv:
            for p in range(len(piece_rows)):
                add(cfg['cstart'] + p * cfg['cevery'], gate_g, functools.partial(conv_piece, p))
            for p in range(cfg['nfin']):
                add(cfg['fin'] + p * cfg['fevery'], gate_dc, functools.partial(conv_finish, p))
        if prev:
            for p in range(cfg['lnp']):
                add(cfg['lstart'] + p * cfg['levery'], gate_x, functools.partial(ln3_part, p))

        def after_pass(t, d):
            for gate, fn in jobs.pop(t, []):
                gate(d)
                fn()

        def flush(lo, hi):
            for t in range(lo, hi):
                for _, fn in jobs.pop(t, []):
                    fn()

        T_S, T_W, T_O, T_Q, T_P = 0, NK, NK + ND, 2 * NK + ND, 2 * NK + 2 * ND
        b, _ = tile(i) if cur else (None, None)
        if cur:
            for n in range(NK):
                keys = _cat([_bf(hh32[b, j, pl.ds(n * L // 2, L // 2), :]) for j in range(ND)])
                s = jax.lax.dot_general(fresh(qbuf), keys, _NT, preferred_element_type=_F32)
                if (n + 1) * L > T:
                    if isinstance(i, int):
                        s = s + kbias[n - T // L]
                    else:
                        col = jax.lax.broadcasted_iota(jnp.int32, (1, L), 1) + n * L
                        s = jnp.where(col < T, s, -1e30)
                sbuf[n] = s
                m = s if n == 0 else jnp.maximum(m, s)
                after_pass(T_S + n, s)
            st['m'] = jnp.max(m, axis=-1, keepdims=True)
        else:
            flush(T_S, T_W)
        if prev:
            b1, r1 = tile(i - 1)
            for n in range(ND):
                d = jnp.dot(fresh(o16), wvo[n], preferred_element_type=_F32)
                x1[b1, n, pl.ds(r1, R), :] += d * rbuf[...]
                after_pass(T_W + n, d)
        else:
            flush(T_W, T_O)
        if cur:
            NC = NK // ND
            p = exp_chunk(0)
            o = [None] * ND
            for c in range(NC):
                pn = None
                for n in range(ND):
                    v = _bf(hh32[b, n, pl.ds(c * ND * L // 2, ND * L // 2), :])
                    d = jnp.dot(p, v, preferred_element_type=_F32)
                    o[n] = d if c == 0 else o[n] + d
                    if c + 1 == NC:
                        o16[n] = o[n].astype(_BF16)
                    if n == cfg['egn'] and c + 1 < NC:
                        gate_s(d)
                        pn = exp_chunk(c + 1)
                    after_pass(T_O + c * ND + n, d)
                p = pn
            rbuf[...] = jnp.broadcast_to(1.0 / jnp.sum(st['l'], axis=-1, keepdims=True), (R, L))
        else:
            flush(T_O, T_Q)
        if nxt:
            cnt = [T_Q]

            def ap(d):
                after_pass(cnt[0], d)
                cnt[0] += 1
            q_proj(i + 1, ap)
        else:
            flush(T_Q, T_P)
        if prev:
            for n in range(ND):
                a = jnp.dot(fresh(h3b), wp1[n], preferred_element_type=_F32)
                after_pass(T_P + 2 * n, a)
                bb = jnp.dot(fresh(h3b), wp1[ND + n], preferred_element_type=_F32)
                g[b1, n, pl.ds(r1 + 2 * HALO, R), :] = a + a * jnp.tanh(bb)
                after_pass(T_P + 2 * n + 1, bb)
        flush(0, T_P + 2 * ND)
        return st['stats']

    stats = (jnp.zeros((8, D), _F32), jnp.zeros((8, D), _F32))
    q_proj(0)
    stats = step_b(0, stats, prev=False, conv=False)
    stats = step_b(1, stats, conv=False)
    stats = jax.lax.fori_loop(2, NT - 1, step_b, stats)
    stats = step_b(NT - 1, stats, nxt=False)
    stats = step_b(NT, stats, cur=False, nxt=False)
    stats = step_b(NT + 1, stats, cur=False, prev=False, nxt=False)

    mu = jnp.sum(stats[0], axis=0, keepdims=True) * (1.0 / N)
    dm = tmean[...] - mu
    trow = jax.lax.broadcasted_iota(jnp.int32, (NT, 1), 0) % TPB
    tcnt = (R - HALO * (trow == 0).astype(jnp.int32)
            + HALO * (trow == TPB - 1).astype(jnp.int32)).astype(_F32)
    var = (jnp.sum(stats[1], axis=0, keepdims=True)
           + jnp.sum(dm * dm * tcnt, axis=0, keepdims=True)) * (1.0 / N)
    rstd = jax.lax.rsqrt(var + _EPS) * 0.5

    def pw2(i):
        b, r0 = tile(i)
        u = (dc[b, pl.ds(r0 + HALO, R), :] - mu) * rstd
        a = (u + u * jnp.tanh(u)).astype(_BF16)
        st_cols(x1, i, ld_x(i) + jnp.dot(a, wp2[...], preferred_element_type=_F32))

    def ln4(i):
        hb[...] = _ln(ld_x(i), 0.5).astype(_BF16)

    def post_d(i):
        xall[pl.ds(rows(i), R), :] = _ln(ld_x(i) + 0.5 * acc[...]).astype(_BF16)
        o_copy(i).start()

    pw2(0)
    ln4(0)
    ff(wa2, wb2, mid=lambda: pw2(1))
    ln4(1)

    def phase_d(i, carry):
        post_d(i - 1)
        ff(wa2, wb2, mid=lambda: pw2(i + 1))
        ln4(i + 1)
        return carry

    jax.lax.fori_loop(1, NT - 1, phase_d, 0)
    post_d(NT - 2)
    ff(wa2, wb2)
    post_d(NT - 1)
    for t in range(NT):
        o_copy(t).wait()


@jax.jit
def pallas_standalone__conformer_family_conformer__speech_kernel(
    x: jax.Array,
    w_ff1_a: jax.Array,
    w_ff1_b: jax.Array,
    w_q: jax.Array,
    w_k: jax.Array,
    w_v: jax.Array,
    w_o: jax.Array,
    w_pw1: jax.Array,
    dw: jax.Array,
    w_pw2: jax.Array,
    w_ff2_a: jax.Array,
    w_ff2_b: jax.Array,
):
    B, T, D = x.shape
    K = dw.shape[0]
    N = B * T
    TP = -(-T // D) * D
    ND = D // L
    assert T % R == 0 and K // 2 <= HALO and K - 1 - K // 2 <= HALO and D % L == 0

    weights = (w_ff1_a, w_ff1_b, w_q, w_k, w_v, w_o, w_pw1, dw, w_pw2, w_ff2_a, w_ff2_b)
    V = pltpu.VMEM
    scratch = [V(w.shape, w.dtype) for w in weights[:6]]
    scratch += [V((2 * ND, D, L), _BF16)]
    scratch += [V(w.shape, w.dtype) for w in weights[7:]]
    scratch += [
        V((ND, D, L), _BF16),
        V((ND, D, L), _BF16),
        V((N, D), x.dtype),
        V((B, ND, T + 8, L), _F32),
        V((B, ND, TP, L), _BF16),
        V((B, ND, T + 4 * HALO, L), _F32),
        V((B, T + 2 * HALO, D), _F32),
        V((TP // L + 1, R, L), _F32),
        V((R, D), _BF16),
        V((R, D), _F32),
        V((ND, R, L), _BF16),
        V((ND, R, L), _BF16),
        V((ND, R, L), _BF16),
        V((R, L), _F32),
        V((K, D), _F32),
        V((N // R, D), _F32),
        pltpu.SemaphoreType.DMA((10 + 2 * ND,)),
        pltpu.SemaphoreType.DMA((N // R,)),
    ]
    col = np.arange(T // L * L, TP).reshape(-1, 1, L)
    kbias = np.where(col < T, 0.0, -1e30).astype(np.float32)
    out = pl.pallas_call(
        functools.partial(_kernel, B=B, T=T, D=D, K=K),
        out_shape=jax.ShapeDtypeStruct((N, D), x.dtype),
        in_specs=([pl.BlockSpec(memory_space=pltpu.SMEM), pl.BlockSpec(memory_space=pltpu.VMEM)]
                  + [pl.BlockSpec(memory_space=pl.ANY)] * (1 + len(weights))),
        out_specs=pl.BlockSpec(memory_space=pl.ANY),
        scratch_shapes=scratch,
        compiler_params=pltpu.CompilerParams(
            vmem_limit_bytes=120 * 2**20,
            flags={"XLA_TPU_EVENLY_DISTRIBUTE_CRITICAL_NODES": True},
        ),
        name="conformer",
    )(np.zeros((1,), np.int32), kbias, x.reshape(N, D), *weights)
    return out.reshape(B, T, D)
```

```python
import functools

import jax
import jax.numpy as jnp
import numpy as np
import jax.experimental.pallas as pl
import jax.experimental.pallas.tpu as pltpu

_EPS = 1e-05
_LOG2E = 1.4426950408889634

R = 400
FC = 512
HALO = 8
L = 128

CFG = dict(order='WAPBOQ', ssplit=8, CP=40, cseg='B', cstart=2, cevery=1, lseg='A', lnp=5, lstart=0, levery=1,
           egn=1, egr=10, fseg='B', fin=13, nfin=2, fevery=1, TP=24)

_NT = (((1,), (1,)), ((), ()))
_F32 = jnp.float32
_BF16 = jnp.bfloat16
_U32 = jnp.uint32


def _cat(xs, axis=1):
    return jnp.concatenate(xs, axis=axis)


def _bf(x):
    return pltpu.bitcast(x, _BF16)


def _ln(x, scale=None):
    d = x.shape[-1]
    m = jnp.sum(x, axis=-1, keepdims=True) * (1.0 / d)
    xc = x - m
    v = jnp.sum(xc * xc, axis=-1, keepdims=True) * (1.0 / d)
    r = jax.lax.rsqrt(v + _EPS)
    if scale is not None:
        r = r * scale
    return xc * r


def _kernel(zero_ref, kbias,
            x_hbm, wa1_h, wb1_h, wq_h, wk_h, wv_h, wo_h, wp1_h, dw_h, wp2_h, wa2_h, wb2_h,
            o_hbm,
            wa1, wb1, wq, wk, wv, wo, wp1, dwv, wp2, wa2, wb2, wm, wvo,
            xall, x1, hh, g, dc, sbuf, hb, acc, qbuf, o16, h3b, rbuf, dwf, tmean,
            wsem, xsem,
            *, B, T, D, K):
    N = B * T
    NT = N // R
    TPB = T // R
    TP = hh.shape[2]
    F = wa1.shape[1]
    NK = TP // L
    ND = D // L
    scale = D ** -0.5
    pad = K // 2
    cfg = CFG
    hh32 = hh.bitcast(_U32)

    def w_copy(src, dst, k):
        return pltpu.make_async_copy(src, dst, wsem.at[k])

    def col_copies(src, dst, k0):
        return [pltpu.make_async_copy(src.at[:, pl.ds(n * L, L)], dst.at[n], wsem.at[k0 + n])
                for n in range(dst.shape[0])]

    NF = F // FC
    c_wa1 = [w_copy(wa1_h.at[:, pl.ds(c * FC, FC)], wa1.at[:, pl.ds(c * FC, FC)], c) for c in range(NF)]
    c_wb1 = [w_copy(wb1_h.at[pl.ds(c * FC, FC), :], wb1.at[pl.ds(c * FC, FC), :], NF + c)
             for c in range(NF)]
    k0 = 2 * NF
    c_rest = [w_copy(src, dst, k0 + n) for n, (src, dst) in enumerate(
        [(wq_h, wq), (wk_h, wk), (wv_h, wv), (wo_h, wo), (dw_h, dwv), (wp2_h, wp2),
         (wa2_h, wa2), (wb2_h, wb2)])] + col_copies(wp1_h, wp1, k0 + 8)

    def rows(i):
        return i * R if isinstance(i, int) else pl.multiple_of(i * R, 16)

    def x_copy(i):
        return pltpu.make_async_copy(x_hbm.at[pl.ds(rows(i), R), :], xall.at[pl.ds(rows(i), R), :],
                                     xsem.at[i])

    def o_copy(i):
        return pltpu.make_async_copy(xall.at[pl.ds(rows(i), R), :], o_hbm.at[pl.ds(rows(i), R), :],
                                     xsem.at[i])

    def tile(i):
        if isinstance(i, int):
            return i // TPB, (i % TPB) * R
        b = i // TPB
        return b, pl.multiple_of((i - b * TPB) * R, 16)

    def ld_x(i):
        b, r0 = tile(i)
        return _cat([x1[b, n, pl.ds(r0, R), :] for n in range(ND)])

    def st_cols(ref, i, v):
        b, r0 = tile(i)
        for n in range(ND):
            ref[b, n, pl.ds(r0, R), :] = v[:, n * L:(n + 1) * L]

    x_copy(0).start()
    c_wa1[0].start()
    for c in range(NF):
        if c + 1 < NF:
            c_wa1[c + 1].start()
        c_wb1[c].start()
        if c == 0:
            x_copy(1).start()
    for t in range(2, NT):
        x_copy(t).start()
    for c in c_rest:
        c.start()

    for b in range(B):
        for n in range(ND):
            hh[b, n, T:TP, :] = jnp.zeros((TP - T, L), _BF16)
            g[b, n, 0:2 * HALO, :] = jnp.zeros((2 * HALO, L), _F32)
            g[b, n, 2 * HALO + T:, :] = jnp.zeros((2 * HALO, L), _F32)
        dc[b, 0:HALO, :] = jnp.zeros((HALO, D), _F32)

    def ff(wa, wb, mid=None, first=False):
        hid = {}

        def up(c):
            if first and c < 2:
                c_wa1[c].wait()
            if first and c == 1:
                c_wb1[0].wait()
            if first and c == 2:
                for w in c_wa1[2:] + c_wb1[1:]:
                    w.wait()
            u = jnp.dot(hb[...], wa[:, c * FC:(c + 1) * FC], preferred_element_type=_F32)
            hid[c] = (u + u * jnp.tanh(u)).astype(_BF16)

        def down(c):
            d = jnp.dot(hid.pop(c), wb[c * FC:(c + 1) * FC, :], preferred_element_type=_F32)
            if c == 0:
                acc[...] = d
            else:
                acc[...] += d

        up(0)
        for c in range(NF):
            if c + 1 < NF:
                up(c + 1)
            if c == NF - 2 and mid is not None:
                mid()
            down(c)

    def ln1(i):
        hb[...] = _ln(xall[pl.ds(rows(i), R), :].astype(_F32), 0.5).astype(_BF16)

    def post_a(i):
        xr = xall[pl.ds(rows(i), R), :].astype(_F32) + 0.5 * acc[...]
        st_cols(x1, i, xr)
        st_cols(hh, i, _ln(xr).astype(_BF16))

    x_copy(0).wait()
    ln1(0)
    x_copy(1).wait()
    ff(wa1, wb1, first=True)
    ln1(1)

    def phase_a(i, carry):
        x_copy(i + 1).wait()
        post_a(i - 1)
        ff(wa1, wb1)
        ln1(i + 1)
        return carry

    jax.lax.fori_loop(1, NT - 1, phase_a, 0)
    for c in c_rest:
        c.wait()
    post_a(NT - 2)
    ff(wa1, wb1)
    for n in range(ND):
        wm[n] = (jax.lax.dot_general(wq[...], wk[n * L:(n + 1) * L, :], _NT,
                                     preferred_element_type=_F32)
                 * (scale * _LOG2E)).astype(_BF16)
        wvo[n] = jnp.dot(wv[...], wo[:, n * L:(n + 1) * L],
                         preferred_element_type=_F32).astype(_BF16)
    dwf[...] = dwv[...].astype(_F32)
    post_a(NT - 1)

    CP = cfg['CP']
    CW = R + HALO
    piece_rows = [(p * CP, CP) for p in range(R // CP)] + [(R, HALO)]

    def q_proj(i, after_pass=lambda d: None):
        b, r0 = tile(i)
        r = r0 // 2 if isinstance(r0, int) else pl.multiple_of(r0 // 2, 8)
        h = _cat([_bf(hh32[b, j, pl.ds(r, R // 2), :]) for j in range(ND)])
        for n in range(ND):
            d = jnp.dot(h, wm[n], preferred_element_type=_F32)
            qbuf[n] = d.astype(_BF16)
            after_pass(d)

    def step_b(i, stats, prev=True, conv=True):
        z0 = zero_ref[0]
        nz = [0]

        def fresh(ref):
            nz[0] += 1
            z = pl.multiple_of(z0 * nz[0], 8)
            r32 = ref.bitcast(_U32)
            return _cat([ref[j] for j in range(ND)])

        st = dict(psum=None, stats=stats)
        k = i - 1

        def edge_mask(w0, a):
            _, r0 = tile(k)
            n = a.shape[0]
            parts = [a]
            if w0 == 0:
                parts = [jnp.where(r0 > 0, a[:HALO], 0.0), a[HALO:]]
            if w0 + n > R:
                h = parts[-1]
                cut = h.shape[0] - HALO
                parts[-1:] = [h[:cut], jnp.where(r0 == T - R, h[cut:], 0.0)]
            parts = [q for q in parts if q.shape[0]]
            return parts[0] if len(parts) == 1 else _cat(parts, 0)

        def conv_piece(p):
            b, r0 = tile(k)
            w0, n = piece_rows[p]
            cols = []
            for j in range(ND):
                win = g[b, j, pl.ds(r0 + w0, n + 2 * HALO), :]
                a = None
                for t in range(K):
                    o = HALO - pad + t
                    v = win[o:o + n, :] * dwf[t:t + 1, j * L:(j + 1) * L]
                    a = v if a is None else a + v
                cols.append(a)
            a = _cat(cols)
            dc[b, pl.ds(r0 + w0, n), :] = a
            ps = jnp.sum(edge_mask(w0, a).reshape(n // 8, 8, D), axis=0)
            st['psum'] = ps if st['psum'] is None else st['psum'] + ps

        def conv_finish(part):
            b, r0 = tile(k)
            nparts = cfg['nfin']
            if part == 0:
                cnt = (R - HALO * jnp.asarray(r0 == 0, jnp.int32)
                       + HALO * jnp.asarray(r0 == T - R, jnp.int32)).astype(_F32)
                st['mu'] = jnp.sum(st['psum'], axis=0, keepdims=True) / cnt
                tmean[pl.ds(k, 1), :] = st['mu']
            lo = (CW // 8 * part // nparts) * 8
            hi = (CW // 8 * (part + 1) // nparts) * 8
            dd = dc[b, pl.ds(r0 + lo, hi - lo), :] - st['mu']
            m2 = jnp.sum(edge_mask(lo, dd * dd).reshape((hi - lo) // 8, 8, D), axis=0)
            s = st['stats']
            st['stats'] = (s[0] + st['psum'] if part == 0 else s[0], s[1] + m2)

        def ln3_part(part):
            b, r0 = tile(i - 1)
            rs = R // cfg['lnp']
            x2 = _cat([x1[b, n, pl.ds(pl.multiple_of(r0 + part * rs + z0, 8), rs), :]
                       for n in range(ND)])
            h = _ln(x2, 0.5).astype(_BF16)
            for n in range(ND):
                h3b[n, part * rs:(part + 1) * rs, :] = h[:, n * L:(n + 1) * L]

        def exp_chunk(c):
            ps = []
            for n in range(ND * c, ND * c + ND):
                p = jnp.exp2(sbuf[n] - st['m'])
                ps.append(p.astype(_BF16))
                st['l'] = p if n == 0 else st['l'] + p
            return _cat(ps)

        def gate_g(d):
            g[z0, 0, pl.ds(T + 3 * HALO, 8), :] = d[0:8, :]

        def gate_x(d):
            x1[z0, 0, pl.ds(T, 8), :] = d[0:8, :]

        def gate_s(d):
            r = cfg['egr'] * 8
            sbuf[z0 + NK, 0:8, :] = d[r:r + 8, :]

        def gate_dc(d):
            dc[z0, pl.ds(T + HALO, 8), 0:L] = d[0:8, :]

        order = cfg['order']
        size = dict(S=NK, A=cfg['ssplit'], B=NK - cfg['ssplit'], W=ND, O=NK, Q=ND, P=2 * ND)
        start = {}
        for name in order:
            start[name] = sum(size[o] for o in order[:order.index(name)])
        jobs = {}

        def add(seg, t, gate, fn):
            jobs.setdefault(start[seg] + t, []).append((gate, fn))

        if conv:
            for p in range(len(piece_rows)):
                add(cfg['cseg'], cfg['cstart'] + p * cfg['cevery'], gate_g,
                    functools.partial(conv_piece, p))
            for p in range(cfg['nfin']):
                add(cfg['fseg'], cfg['fin'] + p * cfg['fevery'], gate_dc,
                    functools.partial(conv_finish, p))
        if prev:
            for p in range(cfg['lnp']):
                add(cfg['lseg'], cfg['lstart'] + p * cfg['levery'], gate_x,
                    functools.partial(ln3_part, p))

        def after_pass(t, d):
            for gate, fn in jobs.pop(t, []):
                gate(d)
                fn()

        b, _ = tile(i)

        def seg_s(lo, hi, t0):
            for n in range(lo, hi):
                keys = _cat([_bf(hh32[b, j, pl.ds(n * L // 2, L // 2), :]) for j in range(ND)])
                s = jax.lax.dot_general(fresh(qbuf), keys, _NT, preferred_element_type=_F32)
                if (n + 1) * L > T:
                    if isinstance(i, int):
                        s = s + kbias[n - T // L]
                    else:
                        col = jax.lax.broadcasted_iota(jnp.int32, (1, L), 1) + n * L
                        s = jnp.where(col < T, s, -1e30)
                sbuf[n] = s
                st['mm'] = s if n == 0 else jnp.maximum(st['mm'], s)
                after_pass(t0 + n - lo, s)
            if hi == NK:
                st['m'] = jnp.max(st['mm'], axis=-1, keepdims=True)

        def seg_w(t0):
            b1, r1 = tile(i - 1)
            for n in range(ND):
                d = jnp.dot(fresh(o16), wvo[n], preferred_element_type=_F32)
                x1[b1, n, pl.ds(r1, R), :] += d * rbuf[...]
                after_pass(t0 + n, d)

        def seg_o(t0):
            NC = NK // ND
            p = exp_chunk(0)
            o = [None] * ND
            for c in range(NC):
                pn = None
                for n in range(ND):
                    v = _bf(hh32[b, n, pl.ds(c * ND * L // 2, ND * L // 2), :])
                    d = jnp.dot(p, v, preferred_element_type=_F32)
                    o[n] = d if c == 0 else o[n] + d
                    if c + 1 == NC:
                        o16[n] = o[n].astype(_BF16)
                    if n == cfg['egn'] and c + 1 < NC:
                        gate_s(d)
                        pn = exp_chunk(c + 1)
                    after_pass(t0 + c * ND + n, d)
                p = pn
            rbuf[...] = jnp.broadcast_to(1.0 / jnp.sum(st['l'], axis=-1, keepdims=True), (R, L))

        def seg_q(t0):
            cnt = [t0]

            def ap(d):
                after_pass(cnt[0], d)
                cnt[0] += 1
            q_proj(i + 1 if isinstance(i, int) else jnp.minimum(i + 1, NT - 1), ap)

        def seg_p(t0):
            b1, r1 = tile(i - 1)
            for n in range(ND):
                a = jnp.dot(fresh(h3b), wp1[n], preferred_element_type=_F32)
                after_pass(t0 + 2 * n, a)
                bb = jnp.dot(fresh(h3b), wp1[ND + n], preferred_element_type=_F32)
                g[b1, n, pl.ds(r1 + 2 * HALO, R), :] = a + a * jnp.tanh(bb)
                after_pass(t0 + 2 * n + 1, bb)

        segs = dict(S=(True, functools.partial(seg_s, 0, NK)),
                    A=(True, functools.partial(seg_s, 0, cfg['ssplit'])),
                    B=(True, functools.partial(seg_s, cfg['ssplit'], NK)), W=(prev, seg_w), O=(True, seg_o), Q=(True, seg_q),
                    P=(prev, seg_p))
        for name in order:
            on, fn = segs[name]
            if on:
                fn(start[name])
            for t in range(start[name], start[name] + size[name]):
                for _, job in jobs.pop(t, []):
                    job()
        assert not jobs
        return st['stats']

    stats = (jnp.zeros((8, D), _F32), jnp.zeros((8, D), _F32))
    q_proj(0)
    stats = step_b(0, stats, prev=False, conv=False)
    stats = jax.lax.fori_loop(1, NT, step_b, stats)

    last = NT - 1
    b1, r1 = tile(last)
    RH = (R // 32) * 16
    for lo, hi in ((0, RH), (RH, R)):
        o = _cat([o16[c, lo:hi, :] for c in range(ND)])
        for n in range(ND):
            d = jnp.dot(o, wvo[n], preferred_element_type=_F32)
            x1[b1, n, r1 + lo:r1 + hi, :] += d * rbuf[lo:hi, :]
    for lo, hi in ((0, RH), (RH, R)):
        h = _ln(_cat([x1[b1, n, r1 + lo:r1 + hi, :] for n in range(ND)]), 0.5).astype(_BF16)
        for j in range(ND):
            a = jnp.dot(h, wp1[j], preferred_element_type=_F32)
            bb = jnp.dot(h, wp1[ND + j], preferred_element_type=_F32)
            g[b1, j, r1 + 2 * HALO + lo:r1 + 2 * HALO + hi, :] = a + a * jnp.tanh(bb)

    TPR = cfg['TP']
    shift = tmean[last - 1:last, :]

    def tail_conv(p, carry):
        w0 = pl.multiple_of(p * TPR, 8)
        c1, c2 = [], []
        for j in range(ND):
            a = None
            for t in range(K):
                v = (g[b1, j, pl.ds(r1 + w0 + HALO - pad + t, TPR), :]
                     * dwf[t:t + 1, j * L:(j + 1) * L])
                a = v if a is None else a + v
            dc[b1, pl.ds(r1 + w0, TPR), j * L:(j + 1) * L] = a
            dd = (a - shift[:, j * L:(j + 1) * L]).reshape(TPR // 8, 8, L)
            c1.append(jnp.sum(dd, axis=0))
            c2.append(jnp.sum(dd * dd, axis=0))
        return carry[0] + _cat(c1), carry[1] + _cat(c2)

    t1, t2 = jax.lax.fori_loop(0, CW // TPR, tail_conv,
                               (jnp.zeros((8, D), _F32), jnp.zeros((8, D), _F32)))
    t1 = jnp.sum(t1, axis=0, keepdims=True)
    t2 = jnp.sum(t2, axis=0, keepdims=True)
    tmean[last:NT, :] = shift + t1 * (1.0 / CW)

    trow = jax.lax.broadcasted_iota(jnp.int32, (NT, 1), 0) % TPB
    tcnt = (R - HALO * (trow == 0).astype(jnp.int32)
            + HALO * (trow == TPB - 1).astype(jnp.int32)).astype(_F32)
    mu = (jnp.sum(stats[0], axis=0, keepdims=True) + (t1 + CW * shift)) * (1.0 / N)
    dm = tmean[...] - mu
    var = (jnp.sum(stats[1], axis=0, keepdims=True) + (t2 - t1 * t1 * (1.0 / CW))
           + jnp.sum(dm * dm * tcnt, axis=0, keepdims=True)) * (1.0 / N)
    rstd = jax.lax.rsqrt(var + _EPS) * 0.5

    def pw2(i):
        b, r0 = tile(i)
        u = (dc[b, pl.ds(r0 + HALO, R), :] - mu) * rstd
        a = (u + u * jnp.tanh(u)).astype(_BF16)
        st_cols(x1, i, ld_x(i) + jnp.dot(a, wp2[...], preferred_element_type=_F32))

    def ln4(i):
        hb[...] = _ln(ld_x(i), 0.5).astype(_BF16)

    def post_d(i):
        xall[pl.ds(rows(i), R), :] = _ln(ld_x(i) + 0.5 * acc[...]).astype(_BF16)
        o_copy(i).start()

    pw2(0)
    pw2(1)
    ln4(0)
    ff(wa2, wb2, mid=lambda: pw2(2))
    ln4(1)

    def phase_d(i, carry):
        post_d(i - 1)
        ff(wa2, wb2, mid=lambda: pw2(i + 2))
        ln4(i + 1)
        return carry

    jax.lax.fori_loop(1, NT - 2, phase_d, 0)
    post_d(NT - 3)
    ff(wa2, wb2)
    ln4(NT - 1)
    post_d(NT - 2)
    ff(wa2, wb2)
    post_d(NT - 1)
    for t in range(NT):
        o_copy(t).wait()


@jax.jit
def pallas_standalone__conformer_family_conformer__speech_kernel(
    x: jax.Array,
    w_ff1_a: jax.Array,
    w_ff1_b: jax.Array,
    w_q: jax.Array,
    w_k: jax.Array,
    w_v: jax.Array,
    w_o: jax.Array,
    w_pw1: jax.Array,
    dw: jax.Array,
    w_pw2: jax.Array,
    w_ff2_a: jax.Array,
    w_ff2_b: jax.Array,
):
    B, T, D = x.shape
    K = dw.shape[0]
    N = B * T
    TP = -(-T // D) * D
    ND = D // L
    assert T % R == 0 and K // 2 <= HALO and K - 1 - K // 2 <= HALO and D % L == 0

    weights = (w_ff1_a, w_ff1_b, w_q, w_k, w_v, w_o, w_pw1, dw, w_pw2, w_ff2_a, w_ff2_b)
    V = pltpu.VMEM
    scratch = [V(w.shape, w.dtype) for w in weights[:6]]
    scratch += [V((2 * ND, D, L), _BF16)]
    scratch += [V(w.shape, w.dtype) for w in weights[7:]]
    scratch += [
        V((ND, D, L), _BF16),
        V((ND, D, L), _BF16),
        V((N, D), x.dtype),
        V((B, ND, T + 8, L), _F32),
        V((B, ND, TP, L), _BF16),
        V((B, ND, T + 4 * HALO, L), _F32),
        V((B, T + 2 * HALO, D), _F32),
        V((TP // L + 1, R, L), _F32),
        V((R, D), _BF16),
        V((R, D), _F32),
        V((ND, R, L), _BF16),
        V((ND, R, L), _BF16),
        V((ND, R, L), _BF16),
        V((R, L), _F32),
        V((K, D), _F32),
        V((N // R, D), _F32),
        pltpu.SemaphoreType.DMA((8 + 2 * (w_ff1_a.shape[1] // FC) + 2 * ND,)),
        pltpu.SemaphoreType.DMA((N // R,)),
    ]
    col = np.arange(T // L * L, TP).reshape(-1, 1, L)
    kbias = np.where(col < T, 0.0, -1e30).astype(np.float32)
    out = pl.pallas_call(
        functools.partial(_kernel, B=B, T=T, D=D, K=K),
        out_shape=jax.ShapeDtypeStruct((N, D), x.dtype),
        in_specs=([pl.BlockSpec(memory_space=pltpu.SMEM), pl.BlockSpec(memory_space=pltpu.VMEM)]
                  + [pl.BlockSpec(memory_space=pl.ANY)] * (1 + len(weights))),
        out_specs=pl.BlockSpec(memory_space=pl.ANY),
        scratch_shapes=scratch,
        compiler_params=pltpu.CompilerParams(
            vmem_limit_bytes=120 * 2**20,
            flags={"XLA_TPU_EVENLY_DISTRIBUTE_CRITICAL_NODES": True},
        ),
        name="conformer",
    )(np.zeros((1,), np.int32), kbias, x.reshape(N, D), *weights)
    return out.reshape(B, T, D)
```

```python
import functools

import jax
import jax.numpy as jnp
import numpy as np
import jax.experimental.pallas as pl
import jax.experimental.pallas.tpu as pltpu

_EPS = 1e-05
_LOG2E = 1.4426950408889634

R = 400
FC = 512
HALO = 8
L = 128

CFG = dict(order='WAPBOQ', ssplit=8, CP=40, cseg='B', cstart=2, cevery=1, lseg='A', lnp=5, lstart=0, levery=1,
           egn=1, egr=10, fseg='B', fin=13, nfin=2, fevery=1, TP=24)

_NT = (((1,), (1,)), ((), ()))
_F32 = jnp.float32
_BF16 = jnp.bfloat16
_U32 = jnp.uint32


def _cat(xs, axis=1):
    return jnp.concatenate(xs, axis=axis)


def _bf(x):
    return pltpu.bitcast(x, _BF16)


def _ln(x, scale=None):
    d = x.shape[-1]
    m = jnp.sum(x, axis=-1, keepdims=True) * (1.0 / d)
    xc = x - m
    v = jnp.sum(xc * xc, axis=-1, keepdims=True) * (1.0 / d)
    r = jax.lax.rsqrt(v + _EPS)
    if scale is not None:
        r = r * scale
    return xc * r


def _kernel(zero_ref, kbias,
            x_hbm, wa1_h, wb1_h, wq_h, wk_h, wv_h, wo_h, wp1_h, dw_h, wp2_h, wa2_h, wb2_h,
            o_hbm,
            wa1, wb1, wq, wk, wv, wo, wp1, dwv, wp2, wa2, wb2, wm, wvo,
            xall, x1, hh, g, dc, sbuf, hb, acc, qbuf, o16, h3b, rbuf, dwf, tmean,
            wsem, xsem,
            *, B, T, D, K):
    N = B * T
    NT = N // R
    TPB = T // R
    TP = hh.shape[2]
    F = wa1.shape[1]
    NK = TP // L
    ND = D // L
    scale = D ** -0.5
    pad = K // 2
    cfg = CFG
    hh32 = hh.bitcast(_U32)

    def w_copy(src, dst, k):
        return pltpu.make_async_copy(src, dst, wsem.at[k])

    def col_copies(src, dst, k0):
        return [pltpu.make_async_copy(src.at[:, pl.ds(n * L, L)], dst.at[n], wsem.at[k0 + n])
                for n in range(dst.shape[0])]

    NF = F // FC
    c_wa1 = [w_copy(wa1_h.at[:, pl.ds(c * FC, FC)], wa1.at[:, pl.ds(c * FC, FC)], c) for c in range(NF)]
    c_wb1 = [w_copy(wb1_h.at[pl.ds(c * FC, FC), :], wb1.at[pl.ds(c * FC, FC), :], NF + c)
             for c in range(NF)]
    k0 = 2 * NF
    c_rest = [w_copy(src, dst, k0 + n) for n, (src, dst) in enumerate(
        [(wq_h, wq), (wk_h, wk), (wv_h, wv), (wo_h, wo), (dw_h, dwv), (wp2_h, wp2),
         (wa2_h, wa2), (wb2_h, wb2)])] + col_copies(wp1_h, wp1, k0 + 8)

    def rows(i):
        return i * R if isinstance(i, int) else pl.multiple_of(i * R, 16)

    def x_copy(i):
        return pltpu.make_async_copy(x_hbm.at[pl.ds(rows(i), R), :], xall.at[pl.ds(rows(i), R), :],
                                     xsem.at[i])

    def o_copy(i):
        return pltpu.make_async_copy(xall.at[pl.ds(rows(i), R), :], o_hbm.at[pl.ds(rows(i), R), :],
                                     xsem.at[i])

    def tile(i):
        if isinstance(i, int):
            return i // TPB, (i % TPB) * R
        b = i // TPB
        return b, pl.multiple_of((i - b * TPB) * R, 16)

    def ld_x(i):
        b, r0 = tile(i)
        return _cat([x1[b, n, pl.ds(r0, R), :] for n in range(ND)])

    def st_cols(ref, i, v):
        b, r0 = tile(i)
        for n in range(ND):
            ref[b, n, pl.ds(r0, R), :] = v[:, n * L:(n + 1) * L]

    x_copy(0).start()
    c_wa1[0].start()
    for c in range(NF):
        if c + 1 < NF:
            c_wa1[c + 1].start()
        c_wb1[c].start()
    for t in range(1, NT):
        x_copy(t).start()
    for c in c_rest:
        c.start()

    for b in range(B):
        for n in range(ND):
            hh[b, n, T:TP, :] = jnp.zeros((TP - T, L), _BF16)
            g[b, n, 0:2 * HALO, :] = jnp.zeros((2 * HALO, L), _F32)
            g[b, n, 2 * HALO + T:, :] = jnp.zeros((2 * HALO, L), _F32)
        dc[b, 0:HALO, :] = jnp.zeros((HALO, D), _F32)

    def ff(wa, wb, mid=None, first=False):
        hid = {}

        def up(c):
            if first and c < 3:
                for w in ([c_wa1[0]], [c_wa1[1], c_wb1[0]], c_wa1[2:] + [c_wb1[1]])[c]:
                    w.wait()
            u = jnp.dot(hb[...], wa[:, c * FC:(c + 1) * FC], preferred_element_type=_F32)
            hid[c] = (u + u * jnp.tanh(u)).astype(_BF16)

        def down(c):
            if first and c == 2:
                for w in c_wb1[2:] + [x_copy(1)]:
                    w.wait()
            d = jnp.dot(hid.pop(c), wb[c * FC:(c + 1) * FC, :], preferred_element_type=_F32)
            if c == 0:
                acc[...] = d
            else:
                acc[...] += d

        up(0)
        for c in range(NF):
            if c + 1 < NF:
                up(c + 1)
            if c == NF - 2 and mid is not None:
                mid()
            down(c)

    def ln1(i):
        hb[...] = _ln(xall[pl.ds(rows(i), R), :].astype(_F32), 0.5).astype(_BF16)

    def post_a(i):
        xr = xall[pl.ds(rows(i), R), :].astype(_F32) + 0.5 * acc[...]
        st_cols(x1, i, xr)
        st_cols(hh, i, _ln(xr).astype(_BF16))

    x_copy(0).wait()
    ln1(0)
    ff(wa1, wb1, first=True)
    ln1(1)

    def phase_a(i, carry):
        x_copy(i + 1).wait()
        post_a(i - 1)
        ff(wa1, wb1)
        ln1(i + 1)
        return carry

    jax.lax.fori_loop(1, NT - 1, phase_a, 0)
    for c in c_rest:
        c.wait()
    post_a(NT - 2)
    ff(wa1, wb1)
    for n in range(ND):
        wm[n] = (jax.lax.dot_general(wq[...], wk[n * L:(n + 1) * L, :], _NT,
                                     preferred_element_type=_F32)
                 * (scale * _LOG2E)).astype(_BF16)
        wvo[n] = jnp.dot(wv[...], wo[:, n * L:(n + 1) * L],
                         preferred_element_type=_F32).astype(_BF16)
    dwf[...] = dwv[...].astype(_F32)
    post_a(NT - 1)

    CP = cfg['CP']
    CW = R + HALO
    piece_rows = [(p * CP, CP) for p in range(R // CP)] + [(R, HALO)]

    def q_proj(i, after_pass=lambda d: None):
        b, r0 = tile(i)
        r = r0 // 2 if isinstance(r0, int) else pl.multiple_of(r0 // 2, 8)
        h = _cat([_bf(hh32[b, j, pl.ds(r, R // 2), :]) for j in range(ND)])
        for n in range(ND):
            d = jnp.dot(h, wm[n], preferred_element_type=_F32)
            qbuf[n] = d.astype(_BF16)
            after_pass(d)

    def step_b(i, stats, prev=True, conv=True):
        z0 = zero_ref[0]
        nz = [0]

        def fresh(ref):
            nz[0] += 1
            z = pl.multiple_of(z0 * nz[0], 8)
            r32 = ref.bitcast(_U32)
            return _cat([ref[j] for j in range(ND)])

        st = dict(psum=None, stats=stats)
        k = i - 1

        def edge_mask(w0, a):
            _, r0 = tile(k)
            n = a.shape[0]
            parts = [a]
            if w0 == 0:
                parts = [jnp.where(r0 > 0, a[:HALO], 0.0), a[HALO:]]
            if w0 + n > R:
                h = parts[-1]
                cut = h.shape[0] - HALO
                parts[-1:] = [h[:cut], jnp.where(r0 == T - R, h[cut:], 0.0)]
            parts = [q for q in parts if q.shape[0]]
            return parts[0] if len(parts) == 1 else _cat(parts, 0)

        def conv_piece(p):
            b, r0 = tile(k)
            w0, n = piece_rows[p]
            cols = []
            for j in range(ND):
                win = g[b, j, pl.ds(r0 + w0, n + 2 * HALO), :]
                a = None
                for t in range(K):
                    o = HALO - pad + t
                    v = win[o:o + n, :] * dwf[t:t + 1, j * L:(j + 1) * L]
                    a = v if a is None else a + v
                cols.append(a)
            a = _cat(cols)
            dc[b, pl.ds(r0 + w0, n), :] = a
            ps = jnp.sum(edge_mask(w0, a).reshape(n // 8, 8, D), axis=0)
            st['psum'] = ps if st['psum'] is None else st['psum'] + ps

        def conv_finish(part):
            b, r0 = tile(k)
            nparts = cfg['nfin']
            if part == 0:
                cnt = (R - HALO * jnp.asarray(r0 == 0, jnp.int32)
                       + HALO * jnp.asarray(r0 == T - R, jnp.int32)).astype(_F32)
                st['mu'] = jnp.sum(st['psum'], axis=0, keepdims=True) / cnt
                tmean[pl.ds(k, 1), :] = st['mu']
            lo = (CW // 8 * part // nparts) * 8
            hi = (CW // 8 * (part + 1) // nparts) * 8
            dd = dc[b, pl.ds(r0 + lo, hi - lo), :] - st['mu']
            m2 = jnp.sum(edge_mask(lo, dd * dd).reshape((hi - lo) // 8, 8, D), axis=0)
            s = st['stats']
            st['stats'] = (s[0] + st['psum'] if part == 0 else s[0], s[1] + m2)

        def ln3_part(part):
            b, r0 = tile(i - 1)
            rs = R // cfg['lnp']
            x2 = _cat([x1[b, n, pl.ds(pl.multiple_of(r0 + part * rs + z0, 8), rs), :]
                       for n in range(ND)])
            h = _ln(x2, 0.5).astype(_BF16)
            for n in range(ND):
                h3b[n, part * rs:(part + 1) * rs, :] = h[:, n * L:(n + 1) * L]

        def exp_chunk(c):
            ps = []
            for n in range(ND * c, ND * c + ND):
                p = jnp.exp2(sbuf[n] - st['m'])
                ps.append(p.astype(_BF16))
                st['l'] = p if n == 0 else st['l'] + p
            return _cat(ps)

        def gate_g(d):
            g[z0, 0, pl.ds(T + 3 * HALO, 8), :] = d[0:8, :]

        def gate_x(d):
            x1[z0, 0, pl.ds(T, 8), :] = d[0:8, :]

        def gate_s(d):
            r = cfg['egr'] * 8
            sbuf[z0 + NK, 0:8, :] = d[r:r + 8, :]

        def gate_dc(d):
            dc[z0, pl.ds(T + HALO, 8), 0:L] = d[0:8, :]

        order = cfg['order']
        size = dict(S=NK, A=cfg['ssplit'], B=NK - cfg['ssplit'], W=ND, O=NK, Q=ND, P=2 * ND)
        start = {}
        for name in order:
            start[name] = sum(size[o] for o in order[:order.index(name)])
        jobs = {}

        def add(seg, t, gate, fn):
            jobs.setdefault(start[seg] + t, []).append((gate, fn))

        if conv:
            for p in range(len(piece_rows)):
                add(cfg['cseg'], cfg['cstart'] + p * cfg['cevery'], gate_g,
                    functools.partial(conv_piece, p))
            for p in range(cfg['nfin']):
                add(cfg['fseg'], cfg['fin'] + p * cfg['fevery'], gate_dc,
                    functools.partial(conv_finish, p))
        if prev:
            for p in range(cfg['lnp']):
                add(cfg['lseg'], cfg['lstart'] + p * cfg['levery'], gate_x,
                    functools.partial(ln3_part, p))

        def after_pass(t, d):
            for gate, fn in jobs.pop(t, []):
                gate(d)
                fn()

        b, _ = tile(i)

        def seg_s(lo, hi, t0):
            for n in range(lo, hi):
                keys = _cat([_bf(hh32[b, j, pl.ds(n * L // 2, L // 2), :]) for j in range(ND)])
                s = jax.lax.dot_general(fresh(qbuf), keys, _NT, preferred_element_type=_F32)
                if (n + 1) * L > T:
                    if isinstance(i, int):
                        s = s + kbias[n - T // L]
                    else:
                        col = jax.lax.broadcasted_iota(jnp.int32, (1, L), 1) + n * L
                        s = jnp.where(col < T, s, -1e30)
                sbuf[n] = s
                st['mm'] = s if n == 0 else jnp.maximum(st['mm'], s)
                after_pass(t0 + n - lo, s)
            if hi == NK:
                st['m'] = jnp.max(st['mm'], axis=-1, keepdims=True)

        def seg_w(t0):
            b1, r1 = tile(i - 1)
            for n in range(ND):
                d = jnp.dot(fresh(o16), wvo[n], preferred_element_type=_F32)
                x1[b1, n, pl.ds(r1, R), :] += d * rbuf[...]
                after_pass(t0 + n, d)

        def seg_o(t0):
            NC = NK // ND
            p = exp_chunk(0)
            o = [None] * ND
            for c in range(NC):
                pn = None
                for n in range(ND):
                    v = _bf(hh32[b, n, pl.ds(c * ND * L // 2, ND * L // 2), :])
                    d = jnp.dot(p, v, preferred_element_type=_F32)
                    o[n] = d if c == 0 else o[n] + d
                    if c + 1 == NC:
                        o16[n] = o[n].astype(_BF16)
                    if n == cfg['egn'] and c + 1 < NC:
                        gate_s(d)
                        pn = exp_chunk(c + 1)
                    after_pass(t0 + c * ND + n, d)
                p = pn
            rbuf[...] = jnp.broadcast_to(1.0 / jnp.sum(st['l'], axis=-1, keepdims=True), (R, L))

        def seg_q(t0):
            cnt = [t0]

            def ap(d):
                after_pass(cnt[0], d)
                cnt[0] += 1
            q_proj(i + 1 if isinstance(i, int) else jnp.minimum(i + 1, NT - 1), ap)

        def seg_p(t0):
            b1, r1 = tile(i - 1)
            for n in range(ND):
                a = jnp.dot(fresh(h3b), wp1[n], preferred_element_type=_F32)
                after_pass(t0 + 2 * n, a)
                bb = jnp.dot(fresh(h3b), wp1[ND + n], preferred_element_type=_F32)
                g[b1, n, pl.ds(r1 + 2 * HALO, R), :] = a + a * jnp.tanh(bb)
                after_pass(t0 + 2 * n + 1, bb)

        segs = dict(S=(True, functools.partial(seg_s, 0, NK)),
                    A=(True, functools.partial(seg_s, 0, cfg['ssplit'])),
                    B=(True, functools.partial(seg_s, cfg['ssplit'], NK)), W=(prev, seg_w), O=(True, seg_o), Q=(True, seg_q),
                    P=(prev, seg_p))
        for name in order:
            on, fn = segs[name]
            if on:
                fn(start[name])
            for t in range(start[name], start[name] + size[name]):
                for _, job in jobs.pop(t, []):
                    job()
        assert not jobs
        return st['stats']

    stats = (jnp.zeros((8, D), _F32), jnp.zeros((8, D), _F32))
    q_proj(0)
    stats = step_b(0, stats, prev=False, conv=False)
    stats = jax.lax.fori_loop(1, NT, step_b, stats)

    last = NT - 1
    b1, r1 = tile(last)
    RH = (R // 32) * 16
    for lo, hi in ((0, RH), (RH, R)):
        o = _cat([o16[c, lo:hi, :] for c in range(ND)])
        for n in range(ND):
            d = jnp.dot(o, wvo[n], preferred_element_type=_F32)
            x1[b1, n, r1 + lo:r1 + hi, :] += d * rbuf[lo:hi, :]
    for lo, hi in ((0, RH), (RH, R)):
        h = _ln(_cat([x1[b1, n, r1 + lo:r1 + hi, :] for n in range(ND)]), 0.5).astype(_BF16)
        for j in range(ND):
            a = jnp.dot(h, wp1[j], preferred_element_type=_F32)
            bb = jnp.dot(h, wp1[ND + j], preferred_element_type=_F32)
            g[b1, j, r1 + 2 * HALO + lo:r1 + 2 * HALO + hi, :] = a + a * jnp.tanh(bb)

    TPR = cfg['TP']
    shift = tmean[last - 1:last, :]

    def tail_conv(p, carry):
        w0 = pl.multiple_of(p * TPR, 8)
        c1, c2 = [], []
        for j in range(ND):
            a = None
            for t in range(K):
                v = (g[b1, j, pl.ds(r1 + w0 + HALO - pad + t, TPR), :]
                     * dwf[t:t + 1, j * L:(j + 1) * L])
                a = v if a is None else a + v
            dc[b1, pl.ds(r1 + w0, TPR), j * L:(j + 1) * L] = a
            dd = (a - shift[:, j * L:(j + 1) * L]).reshape(TPR // 8, 8, L)
            c1.append(jnp.sum(dd, axis=0))
            c2.append(jnp.sum(dd * dd, axis=0))
        return carry[0] + _cat(c1), carry[1] + _cat(c2)

    t1, t2 = jax.lax.fori_loop(0, CW // TPR, tail_conv,
                               (jnp.zeros((8, D), _F32), jnp.zeros((8, D), _F32)))
    t1 = jnp.sum(t1, axis=0, keepdims=True)
    t2 = jnp.sum(t2, axis=0, keepdims=True)
    tmean[last:NT, :] = shift + t1 * (1.0 / CW)

    trow = jax.lax.broadcasted_iota(jnp.int32, (NT, 1), 0) % TPB
    tcnt = (R - HALO * (trow == 0).astype(jnp.int32)
            + HALO * (trow == TPB - 1).astype(jnp.int32)).astype(_F32)
    mu = (jnp.sum(stats[0], axis=0, keepdims=True) + (t1 + CW * shift)) * (1.0 / N)
    dm = tmean[...] - mu
    var = (jnp.sum(stats[1], axis=0, keepdims=True) + (t2 - t1 * t1 * (1.0 / CW))
           + jnp.sum(dm * dm * tcnt, axis=0, keepdims=True)) * (1.0 / N)
    rstd = jax.lax.rsqrt(var + _EPS) * 0.5

    def pw2(i):
        b, r0 = tile(i)
        u = (dc[b, pl.ds(r0 + HALO, R), :] - mu) * rstd
        a = (u + u * jnp.tanh(u)).astype(_BF16)
        st_cols(x1, i, ld_x(i) + jnp.dot(a, wp2[...], preferred_element_type=_F32))

    def ln4(i):
        hb[...] = _ln(ld_x(i), 0.5).astype(_BF16)

    def post_d(i):
        xall[pl.ds(rows(i), R), :] = _ln(ld_x(i) + 0.5 * acc[...]).astype(_BF16)
        o_copy(i).start()

    pw2(0)
    pw2(1)
    ln4(0)
    ff(wa2, wb2)
    ln4(1)

    def phase_d(i, carry):
        post_d(i - 1)
        ff(wa2, wb2, mid=lambda: pw2(i + 1))
        ln4(i + 1)
        return carry

    jax.lax.fori_loop(1, NT - 1, phase_d, 0)
    post_d(NT - 2)
    ff(wa2, wb2)
    post_d(NT - 1)
    for t in range(NT):
        o_copy(t).wait()


@jax.jit
def pallas_standalone__conformer_family_conformer__speech_kernel(
    x: jax.Array,
    w_ff1_a: jax.Array,
    w_ff1_b: jax.Array,
    w_q: jax.Array,
    w_k: jax.Array,
    w_v: jax.Array,
    w_o: jax.Array,
    w_pw1: jax.Array,
    dw: jax.Array,
    w_pw2: jax.Array,
    w_ff2_a: jax.Array,
    w_ff2_b: jax.Array,
):
    B, T, D = x.shape
    K = dw.shape[0]
    N = B * T
    TP = -(-T // D) * D
    ND = D // L
    assert T % R == 0 and K // 2 <= HALO and K - 1 - K // 2 <= HALO and D % L == 0

    weights = (w_ff1_a, w_ff1_b, w_q, w_k, w_v, w_o, w_pw1, dw, w_pw2, w_ff2_a, w_ff2_b)
    V = pltpu.VMEM
    scratch = [V(w.shape, w.dtype) for w in weights[:6]]
    scratch += [V((2 * ND, D, L), _BF16)]
    scratch += [V(w.shape, w.dtype) for w in weights[7:]]
    scratch += [
        V((ND, D, L), _BF16),
        V((ND, D, L), _BF16),
        V((N, D), x.dtype),
        V((B, ND, T + 8, L), _F32),
        V((B, ND, TP, L), _BF16),
        V((B, ND, T + 4 * HALO, L), _F32),
        V((B, T + 2 * HALO, D), _F32),
        V((TP // L + 1, R, L), _F32),
        V((R, D), _BF16),
        V((R, D), _F32),
        V((ND, R, L), _BF16),
        V((ND, R, L), _BF16),
        V((ND, R, L), _BF16),
        V((R, L), _F32),
        V((K, D), _F32),
        V((N // R, D), _F32),
        pltpu.SemaphoreType.DMA((8 + 2 * (w_ff1_a.shape[1] // FC) + 2 * ND,)),
        pltpu.SemaphoreType.DMA((N // R,)),
    ]
    col = np.arange(T // L * L, TP).reshape(-1, 1, L)
    kbias = np.where(col < T, 0.0, -1e30).astype(np.float32)
    out = pl.pallas_call(
        functools.partial(_kernel, B=B, T=T, D=D, K=K),
        out_shape=jax.ShapeDtypeStruct((N, D), x.dtype),
        in_specs=([pl.BlockSpec(memory_space=pltpu.SMEM), pl.BlockSpec(memory_space=pltpu.VMEM)]
                  + [pl.BlockSpec(memory_space=pl.ANY)] * (1 + len(weights))),
        out_specs=pl.BlockSpec(memory_space=pl.ANY),
        scratch_shapes=scratch,
        compiler_params=pltpu.CompilerParams(
            vmem_limit_bytes=120 * 2**20,
            flags={"XLA_TPU_EVENLY_DISTRIBUTE_CRITICAL_NODES": True},
        ),
        name="conformer",
    )(np.zeros((1,), np.int32), kbias, x.reshape(N, D), *weights)
    return out.reshape(B, T, D)
```

```python
import functools

import jax
import jax.numpy as jnp
import numpy as np
import jax.experimental.pallas as pl
import jax.experimental.pallas.tpu as pltpu

_EPS = 1e-05
_LOG2E = 1.4426950408889634

R = 400
FC = 512
HALO = 8
L = 128

CFG = dict(order='WAPBQOR', ssplit=8, qsplit=2, CP=40, cseg='B', cstart=0, cevery=1, lseg='A', lnp=5, lstart=1, levery=1,
           egn=2, egr=10, fseg='B', fin=14, nfin=2, fevery=1, TP=24, rseg='R', rpos=1)

_NT = (((1,), (1,)), ((), ()))
_F32 = jnp.float32
_BF16 = jnp.bfloat16
_U32 = jnp.uint32


def _cat(xs, axis=1):
    return jnp.concatenate(xs, axis=axis)


def _bf(x):
    return pltpu.bitcast(x, _BF16)


def _ln(x, scale=None):
    d = x.shape[-1]
    m = jnp.sum(x, axis=-1, keepdims=True) * (1.0 / d)
    xc = x - m
    v = jnp.sum(xc * xc, axis=-1, keepdims=True) * (1.0 / d)
    r = jax.lax.rsqrt(v + _EPS)
    if scale is not None:
        r = r * scale
    return xc * r


def _kernel(zero_ref, kbias,
            x_hbm, wa1_h, wb1_h, wq_h, wk_h, wv_h, wo_h, wp1_h, dw_h, wp2_h, wa2_h, wb2_h,
            o_hbm,
            wa1, wb1, wq, wk, wv, wo, wp1, dwv, wp2, wa2, wb2, wm, wvo,
            xall, x1, hh, g, dc, sbuf, hb, acc, qbuf, o16, h3b, rbuf, lbuf, dwf, tmean,
            wsem, xsem,
            *, B, T, D, K):
    N = B * T
    NT = N // R
    TPB = T // R
    TP = hh.shape[2]
    F = wa1.shape[1]
    NK = TP // L
    ND = D // L
    scale = D ** -0.5
    pad = K // 2
    cfg = CFG
    hh32 = hh.bitcast(_U32)

    def w_copy(src, dst, k):
        return pltpu.make_async_copy(src, dst, wsem.at[k])

    def col_copies(src, dst, k0):
        return [pltpu.make_async_copy(src.at[:, pl.ds(n * L, L)], dst.at[n], wsem.at[k0 + n])
                for n in range(dst.shape[0])]

    NF = F // FC
    c_wa1 = [w_copy(wa1_h.at[:, pl.ds(c * FC, FC)], wa1.at[:, pl.ds(c * FC, FC)], c) for c in range(NF)]
    c_wb1 = [w_copy(wb1_h.at[pl.ds(c * FC, FC), :], wb1.at[pl.ds(c * FC, FC), :], NF + c)
             for c in range(NF)]
    k0 = 2 * NF
    c_rest = [w_copy(src, dst, k0 + n) for n, (src, dst) in enumerate(
        [(wq_h, wq), (wk_h, wk), (wv_h, wv), (wo_h, wo), (dw_h, dwv), (wp2_h, wp2),
         (wa2_h, wa2), (wb2_h, wb2)])] + col_copies(wp1_h, wp1, k0 + 8)

    def rows(i):
        return i * R if isinstance(i, int) else pl.multiple_of(i * R, 16)

    def x_copy(i):
        return pltpu.make_async_copy(x_hbm.at[pl.ds(rows(i), R), :], xall.at[pl.ds(rows(i), R), :],
                                     xsem.at[i])

    def o_copy(i):
        return pltpu.make_async_copy(xall.at[pl.ds(rows(i), R), :], o_hbm.at[pl.ds(rows(i), R), :],
                                     xsem.at[i])

    def tile(i):
        if isinstance(i, int):
            return i // TPB, (i % TPB) * R
        b = i // TPB
        return b, pl.multiple_of((i - b * TPB) * R, 16)

    def ld_x(i):
        b, r0 = tile(i)
        return _cat([x1[b, n, pl.ds(r0, R), :] for n in range(ND)])

    def st_cols(ref, i, v):
        b, r0 = tile(i)
        for n in range(ND):
            ref[b, n, pl.ds(r0, R), :] = v[:, n * L:(n + 1) * L]

    x_copy(0).start()
    c_wa1[0].start()
    for c in range(NF):
        if c + 1 < NF:
            c_wa1[c + 1].start()
        c_wb1[c].start()
    for t in range(1, NT):
        x_copy(t).start()
    for c in c_rest:
        c.start()

    for b in range(B):
        for n in range(ND):
            hh[b, n, T:TP, :] = jnp.zeros((TP - T, L), _BF16)
            g[b, n, 0:2 * HALO, :] = jnp.zeros((2 * HALO, L), _F32)
            g[b, n, 2 * HALO + T:, :] = jnp.zeros((2 * HALO, L), _F32)
        dc[b, 0:HALO, :] = jnp.zeros((HALO, D), _F32)

    def ff(wa, wb, mid=None, first=False):
        hid = {}

        def up(c):
            if first and c < 3:
                for w in ([c_wa1[0]], [c_wa1[1], c_wb1[0]], c_wa1[2:] + [c_wb1[1]])[c]:
                    w.wait()
            u = jnp.dot(hb[...], wa[:, c * FC:(c + 1) * FC], preferred_element_type=_F32)
            hid[c] = (u + u * jnp.tanh(u)).astype(_BF16)

        def down(c):
            if first and c == 2:
                for w in c_wb1[2:] + [x_copy(1)]:
                    w.wait()
            d = jnp.dot(hid.pop(c), wb[c * FC:(c + 1) * FC, :], preferred_element_type=_F32)
            if c == 0:
                acc[...] = d
            else:
                acc[...] += d

        up(0)
        for c in range(NF):
            if c + 1 < NF:
                up(c + 1)
            if c == NF - 2 and mid is not None:
                mid()
            down(c)

    def ln1(i):
        hb[...] = _ln(xall[pl.ds(rows(i), R), :].astype(_F32), 0.5).astype(_BF16)

    def post_a(i):
        xr = xall[pl.ds(rows(i), R), :].astype(_F32) + 0.5 * acc[...]
        st_cols(x1, i, xr)
        st_cols(hh, i, _ln(xr).astype(_BF16))

    x_copy(0).wait()
    ln1(0)
    ff(wa1, wb1, first=True)
    ln1(1)

    def phase_a(i, carry):
        x_copy(i + 1).wait()
        post_a(i - 1)
        ff(wa1, wb1)
        ln1(i + 1)
        return carry

    jax.lax.fori_loop(1, NT - 1, phase_a, 0)
    for c in c_rest:
        c.wait()
    post_a(NT - 2)
    ff(wa1, wb1)
    for n in range(ND):
        wm[n] = (jax.lax.dot_general(wq[...], wk[n * L:(n + 1) * L, :], _NT,
                                     preferred_element_type=_F32)
                 * (scale * _LOG2E)).astype(_BF16)
        wvo[n] = jnp.dot(wv[...], wo[:, n * L:(n + 1) * L],
                         preferred_element_type=_F32).astype(_BF16)
    dwf[...] = dwv[...].astype(_F32)
    post_a(NT - 1)

    CP = cfg['CP']
    CW = R + HALO
    piece_rows = [(p * CP, CP) for p in range(R // CP)] + [(R, HALO)]

    def q_proj(i, lo=0, hi=ND, after_pass=lambda d: None):
        b, r0 = tile(i)
        r = r0 // 2 if isinstance(r0, int) else pl.multiple_of(r0 // 2, 8)
        h = _cat([_bf(hh32[b, j, pl.ds(r, R // 2), :]) for j in range(ND)])
        for n in range(lo, hi):
            d = jnp.dot(h, wm[n], preferred_element_type=_F32)
            qbuf[n] = d.astype(_BF16)
            after_pass(d)

    def step_b(i, stats, prev=True, conv=True):
        z0 = zero_ref[0]
        nz = [0]

        def fresh(ref):
            nz[0] += 1
            z = pl.multiple_of(z0 * nz[0], 8)
            r32 = ref.bitcast(_U32)
            return _cat([ref[j] for j in range(ND)])

        st = dict(psum=None, stats=stats)
        k = i - 1

        def edge_mask(w0, a):
            _, r0 = tile(k)
            n = a.shape[0]
            parts = [a]
            if w0 == 0:
                parts = [jnp.where(r0 > 0, a[:HALO], 0.0), a[HALO:]]
            if w0 + n > R:
                h = parts[-1]
                cut = h.shape[0] - HALO
                parts[-1:] = [h[:cut], jnp.where(r0 == T - R, h[cut:], 0.0)]
            parts = [q for q in parts if q.shape[0]]
            return parts[0] if len(parts) == 1 else _cat(parts, 0)

        def conv_piece(p):
            b, r0 = tile(k)
            w0, n = piece_rows[p]
            cols = []
            for j in range(ND):
                win = g[b, j, pl.ds(r0 + w0, n + 2 * HALO), :]
                a = None
                for t in range(K):
                    o = HALO - pad + t
                    v = win[o:o + n, :] * dwf[t:t + 1, j * L:(j + 1) * L]
                    a = v if a is None else a + v
                cols.append(a)
            a = _cat(cols)
            dc[b, pl.ds(r0 + w0, n), :] = a
            ps = jnp.sum(edge_mask(w0, a).reshape(n // 8, 8, D), axis=0)
            st['psum'] = ps if st['psum'] is None else st['psum'] + ps

        def conv_finish(part):
            b, r0 = tile(k)
            nparts = cfg['nfin']
            if part == 0:
                cnt = (R - HALO * jnp.asarray(r0 == 0, jnp.int32)
                       + HALO * jnp.asarray(r0 == T - R, jnp.int32)).astype(_F32)
                st['mu'] = jnp.sum(st['psum'], axis=0, keepdims=True) / cnt
                tmean[pl.ds(k, 1), :] = st['mu']
            lo = (CW // 8 * part // nparts) * 8
            hi = (CW // 8 * (part + 1) // nparts) * 8
            dd = dc[b, pl.ds(r0 + lo, hi - lo), :] - st['mu']
            m2 = jnp.sum(edge_mask(lo, dd * dd).reshape((hi - lo) // 8, 8, D), axis=0)
            s = st['stats']
            st['stats'] = (s[0] + st['psum'] if part == 0 else s[0], s[1] + m2)

        def ln3_part(part):
            b, r0 = tile(i - 1)
            rs = R // cfg['lnp']
            x2 = _cat([x1[b, n, pl.ds(pl.multiple_of(r0 + part * rs + z0, 8), rs), :]
                       for n in range(ND)])
            h = _ln(x2, 0.5).astype(_BF16)
            for n in range(ND):
                h3b[n, part * rs:(part + 1) * rs, :] = h[:, n * L:(n + 1) * L]

        def exp_chunk(c):
            ps = []
            for n in range(ND * c, ND * c + ND):
                p = jnp.exp2(sbuf[n] - st['m'])
                ps.append(p.astype(_BF16))
                st['l'] = p if n == 0 else st['l'] + p
            return _cat(ps)

        def gate_g(d):
            g[z0, 0, pl.ds(T + 3 * HALO, 8), :] = d[0:8, :]

        def gate_x(d):
            x1[z0, 0, pl.ds(T, 8), :] = d[0:8, :]

        def gate_s(d):
            r = cfg['egr'] * 8
            sbuf[z0 + NK, 0:8, :] = d[r:r + 8, :]

        def gate_l(d):
            lbuf[pl.ds(pl.multiple_of(R + z0, 8), 8), :] = d[0:8, :]

        def inv_l():
            rbuf[...] = jnp.broadcast_to(1.0 / jnp.sum(lbuf[0:R, :], axis=-1, keepdims=True), (R, L))

        def gate_dc(d):
            dc[z0, pl.ds(T + HALO, 8), 0:L] = d[0:8, :]

        order = cfg['order']
        size = dict(S=NK, A=cfg['ssplit'], B=NK - cfg['ssplit'], W=ND, O=NK, P=2 * ND,
                    Q=cfg['qsplit'], R=ND - cfg['qsplit'])
        start = {}
        for name in order:
            start[name] = sum(size[o] for o in order[:order.index(name)])
        jobs = {}

        def add(seg, t, gate, fn):
            jobs.setdefault(start[seg] + t, []).append((gate, fn))

        if conv:
            for p in range(len(piece_rows)):
                add(cfg['cseg'], cfg['cstart'] + p * cfg['cevery'], gate_g,
                    functools.partial(conv_piece, p))
            for p in range(cfg['nfin']):
                add(cfg['fseg'], cfg['fin'] + p * cfg['fevery'], gate_dc,
                    functools.partial(conv_finish, p))
        if cfg['rseg']:
            add(cfg['rseg'], cfg['rpos'], gate_l, inv_l)
        if prev:
            for p in range(cfg['lnp']):
                add(cfg['lseg'], cfg['lstart'] + p * cfg['levery'], gate_x,
                    functools.partial(ln3_part, p))

        def after_pass(t, d):
            for gate, fn in jobs.pop(t, []):
                gate(d)
                fn()

        b, _ = tile(i)

        def seg_s(lo, hi, t0):
            for n in range(lo, hi):
                keys = _cat([_bf(hh32[b, j, pl.ds(n * L // 2, L // 2), :]) for j in range(ND)])
                s = jax.lax.dot_general(fresh(qbuf), keys, _NT, preferred_element_type=_F32)
                if (n + 1) * L > T:
                    if isinstance(i, int):
                        s = s + kbias[n - T // L]
                    else:
                        col = jax.lax.broadcasted_iota(jnp.int32, (1, L), 1) + n * L
                        s = jnp.where(col < T, s, -1e30)
                sbuf[n] = s
                st['mm'] = s if n == 0 else jnp.maximum(st['mm'], s)
                after_pass(t0 + n - lo, s)
            if hi == NK:
                st['m'] = jnp.max(st['mm'], axis=-1, keepdims=True)

        def seg_w(t0):
            b1, r1 = tile(i - 1)
            for n in range(ND):
                d = jnp.dot(fresh(o16), wvo[n], preferred_element_type=_F32)
                x1[b1, n, pl.ds(r1, R), :] += d * rbuf[...]
                after_pass(t0 + n, d)

        def seg_o(t0):
            NC = NK // ND
            p = exp_chunk(0)
            o = [None] * ND
            for c in range(NC):
                pn = None
                for n in range(ND):
                    v = _bf(hh32[b, n, pl.ds(c * ND * L // 2, ND * L // 2), :])
                    d = jnp.dot(p, v, preferred_element_type=_F32)
                    o[n] = d if c == 0 else o[n] + d
                    if c + 1 == NC:
                        o16[n] = o[n].astype(_BF16)
                    if n == cfg['egn'] and c + 1 < NC:
                        gate_s(d)
                        pn = exp_chunk(c + 1)
                    after_pass(t0 + c * ND + n, d)
                p = pn
            if cfg['rseg']:
                lbuf[0:R, :] = st['l']
            else:
                rbuf[...] = jnp.broadcast_to(1.0 / jnp.sum(st['l'], axis=-1, keepdims=True), (R, L))

        def seg_q(lo, hi, t0):
            cnt = [t0]

            def ap(d):
                after_pass(cnt[0], d)
                cnt[0] += 1
            q_proj(i + 1 if isinstance(i, int) else jnp.minimum(i + 1, NT - 1), lo, hi, ap)

        def seg_p(t0):
            b1, r1 = tile(i - 1)
            for n in range(ND):
                a = jnp.dot(fresh(h3b), wp1[n], preferred_element_type=_F32)
                after_pass(t0 + 2 * n, a)
                bb = jnp.dot(fresh(h3b), wp1[ND + n], preferred_element_type=_F32)
                g[b1, n, pl.ds(r1 + 2 * HALO, R), :] = a + a * jnp.tanh(bb)
                after_pass(t0 + 2 * n + 1, bb)

        segs = dict(S=(True, functools.partial(seg_s, 0, NK)),
                    A=(True, functools.partial(seg_s, 0, cfg['ssplit'])),
                    B=(True, functools.partial(seg_s, cfg['ssplit'], NK)), W=(prev, seg_w), O=(True, seg_o), Q=(True, functools.partial(seg_q, 0, cfg['qsplit'])),
                    R=(True, functools.partial(seg_q, cfg['qsplit'], ND)),
                    P=(prev, seg_p))
        for name in order:
            on, fn = segs[name]
            if on:
                fn(start[name])
            for t in range(start[name], start[name] + size[name]):
                for _, job in jobs.pop(t, []):
                    job()
        assert not jobs
        return st['stats']

    stats = (jnp.zeros((8, D), _F32), jnp.zeros((8, D), _F32))
    q_proj(0)
    stats = step_b(0, stats, prev=False, conv=False)
    stats = jax.lax.fori_loop(1, NT, step_b, stats)

    last = NT - 1
    b1, r1 = tile(last)
    RH = (R // 32) * 16
    for lo, hi in ((0, RH), (RH, R)):
        o = _cat([o16[c, lo:hi, :] for c in range(ND)])
        for n in range(ND):
            d = jnp.dot(o, wvo[n], preferred_element_type=_F32)
            x1[b1, n, r1 + lo:r1 + hi, :] += d * rbuf[lo:hi, :]
    for lo, hi in ((0, RH), (RH, R)):
        h = _ln(_cat([x1[b1, n, r1 + lo:r1 + hi, :] for n in range(ND)]), 0.5).astype(_BF16)
        for j in range(ND):
            a = jnp.dot(h, wp1[j], preferred_element_type=_F32)
            bb = jnp.dot(h, wp1[ND + j], preferred_element_type=_F32)
            g[b1, j, r1 + 2 * HALO + lo:r1 + 2 * HALO + hi, :] = a + a * jnp.tanh(bb)

    TPR = cfg['TP']
    shift = tmean[last - 1:last, :]

    def tail_conv(p, carry):
        w0 = pl.multiple_of(p * TPR, 8)
        c1, c2 = [], []
        for j in range(ND):
            a = None
            for t in range(K):
                v = (g[b1, j, pl.ds(r1 + w0 + HALO - pad + t, TPR), :]
                     * dwf[t:t + 1, j * L:(j + 1) * L])
                a = v if a is None else a + v
            dc[b1, pl.ds(r1 + w0, TPR), j * L:(j + 1) * L] = a
            dd = (a - shift[:, j * L:(j + 1) * L]).reshape(TPR // 8, 8, L)
            c1.append(jnp.sum(dd, axis=0))
            c2.append(jnp.sum(dd * dd, axis=0))
        return carry[0] + _cat(c1), carry[1] + _cat(c2)

    t1, t2 = jax.lax.fori_loop(0, CW // TPR, tail_conv,
                               (jnp.zeros((8, D), _F32), jnp.zeros((8, D), _F32)))
    t1 = jnp.sum(t1, axis=0, keepdims=True)
    t2 = jnp.sum(t2, axis=0, keepdims=True)
    tmean[last:NT, :] = shift + t1 * (1.0 / CW)

    trow = jax.lax.broadcasted_iota(jnp.int32, (NT, 1), 0) % TPB
    tcnt = (R - HALO * (trow == 0).astype(jnp.int32)
            + HALO * (trow == TPB - 1).astype(jnp.int32)).astype(_F32)
    mu = (jnp.sum(stats[0], axis=0, keepdims=True) + (t1 + CW * shift)) * (1.0 / N)
    dm = tmean[...] - mu
    var = (jnp.sum(stats[1], axis=0, keepdims=True) + (t2 - t1 * t1 * (1.0 / CW))
           + jnp.sum(dm * dm * tcnt, axis=0, keepdims=True)) * (1.0 / N)
    rstd = jax.lax.rsqrt(var + _EPS) * 0.5

    def pw2(i):
        b, r0 = tile(i)
        u = (dc[b, pl.ds(r0 + HALO, R), :] - mu) * rstd
        a = (u + u * jnp.tanh(u)).astype(_BF16)
        st_cols(x1, i, ld_x(i) + jnp.dot(a, wp2[...], preferred_element_type=_F32))

    def ln4(i):
        hb[...] = _ln(ld_x(i), 0.5).astype(_BF16)

    def post_d(i):
        xall[pl.ds(rows(i), R), :] = _ln(ld_x(i) + 0.5 * acc[...]).astype(_BF16)
        o_copy(i).start()

    pw2(0)
    pw2(1)
    ln4(0)
    ff(wa2, wb2)
    ln4(1)

    def phase_d(i, carry):
        post_d(i - 1)
        ff(wa2, wb2, mid=lambda: pw2(i + 1))
        ln4(i + 1)
        return carry

    jax.lax.fori_loop(1, NT - 1, phase_d, 0)
    post_d(NT - 2)
    ff(wa2, wb2)
    post_d(NT - 1)
    for t in range(NT):
        o_copy(t).wait()


@jax.jit
def pallas_standalone__conformer_family_conformer__speech_kernel(
    x: jax.Array,
    w_ff1_a: jax.Array,
    w_ff1_b: jax.Array,
    w_q: jax.Array,
    w_k: jax.Array,
    w_v: jax.Array,
    w_o: jax.Array,
    w_pw1: jax.Array,
    dw: jax.Array,
    w_pw2: jax.Array,
    w_ff2_a: jax.Array,
    w_ff2_b: jax.Array,
):
    B, T, D = x.shape
    K = dw.shape[0]
    N = B * T
    TP = -(-T // D) * D
    ND = D // L
    assert T % R == 0 and K // 2 <= HALO and K - 1 - K // 2 <= HALO and D % L == 0

    weights = (w_ff1_a, w_ff1_b, w_q, w_k, w_v, w_o, w_pw1, dw, w_pw2, w_ff2_a, w_ff2_b)
    V = pltpu.VMEM
    scratch = [V(w.shape, w.dtype) for w in weights[:6]]
    scratch += [V((2 * ND, D, L), _BF16)]
    scratch += [V(w.shape, w.dtype) for w in weights[7:]]
    scratch += [
        V((ND, D, L), _BF16),
        V((ND, D, L), _BF16),
        V((N, D), x.dtype),
        V((B, ND, T + 8, L), _F32),
        V((B, ND, TP, L), _BF16),
        V((B, ND, T + 4 * HALO, L), _F32),
        V((B, T + 2 * HALO, D), _F32),
        V((TP // L + 1, R, L), _F32),
        V((R, D), _BF16),
        V((R, D), _F32),
        V((ND, R, L), _BF16),
        V((ND, R, L), _BF16),
        V((ND, R, L), _BF16),
        V((R, L), _F32),
        V((R + 8, L), _F32),
        V((K, D), _F32),
        V((N // R, D), _F32),
        pltpu.SemaphoreType.DMA((8 + 2 * (w_ff1_a.shape[1] // FC) + 2 * ND,)),
        pltpu.SemaphoreType.DMA((N // R,)),
    ]
    col = np.arange(T // L * L, TP).reshape(-1, 1, L)
    kbias = np.where(col < T, 0.0, -1e30).astype(np.float32)
    out = pl.pallas_call(
        functools.partial(_kernel, B=B, T=T, D=D, K=K),
        out_shape=jax.ShapeDtypeStruct((N, D), x.dtype),
        in_specs=([pl.BlockSpec(memory_space=pltpu.SMEM), pl.BlockSpec(memory_space=pltpu.VMEM)]
                  + [pl.BlockSpec(memory_space=pl.ANY)] * (1 + len(weights))),
        out_specs=pl.BlockSpec(memory_space=pl.ANY),
        scratch_shapes=scratch,
        compiler_params=pltpu.CompilerParams(
            vmem_limit_bytes=120 * 2**20,
            flags={"XLA_TPU_EVENLY_DISTRIBUTE_CRITICAL_NODES": True},
        ),
        name="conformer",
    )(np.zeros((1,), np.int32), kbias, x.reshape(N, D), *weights)
    return out.reshape(B, T, D)
```

```python
import functools

import jax
import jax.numpy as jnp
import numpy as np
import jax.experimental.pallas as pl
import jax.experimental.pallas.tpu as pltpu

_EPS = 1e-05
_LOG2E = 1.4426950408889634

R = 400
FC = 512
HALO = 8
L = 128

CFG = dict(order='WAPBQOR', ssplit=8, qsplit=2, CP=40, cseg='B', cstart=0, cevery=1, lseg='A', lnp=5, lstart=1, levery=1,
           egn=2, egr=10, fseg='B', fin=14, nfin=2, fevery=1, TP=24, rseg='R', rpos=1, oparts=5)

_NT = (((1,), (1,)), ((), ()))
_F32 = jnp.float32
_BF16 = jnp.bfloat16
_U32 = jnp.uint32


def _cat(xs, axis=1):
    return jnp.concatenate(xs, axis=axis)


def _bf(x):
    return pltpu.bitcast(x, _BF16)


def _ln(x, scale=None):
    d = x.shape[-1]
    m = jnp.sum(x, axis=-1, keepdims=True) * (1.0 / d)
    xc = x - m
    v = jnp.sum(xc * xc, axis=-1, keepdims=True) * (1.0 / d)
    r = jax.lax.rsqrt(v + _EPS)
    if scale is not None:
        r = r * scale
    return xc * r


def _kernel(zero_ref, kbias,
            x_hbm, wa1_h, wb1_h, wq_h, wk_h, wv_h, wo_h, wp1_h, dw_h, wp2_h, wa2_h, wb2_h,
            o_hbm,
            wa1, wb1, wq, wk, wv, wo, wp1, dwv, wp2, wa2, wb2, wm, wvo,
            xall, x1, hh, g, dc, sbuf, hb, acc, qbuf, o16, h3b, rbuf, lbuf, dwf, tmean,
            wsem, xsem,
            *, B, T, D, K):
    N = B * T
    NT = N // R
    TPB = T // R
    TP = hh.shape[2]
    F = wa1.shape[1]
    NK = TP // L
    ND = D // L
    scale = D ** -0.5
    pad = K // 2
    cfg = CFG
    hh32 = hh.bitcast(_U32)

    def w_copy(src, dst, k):
        return pltpu.make_async_copy(src, dst, wsem.at[k])

    def col_copies(src, dst, k0):
        return [pltpu.make_async_copy(src.at[:, pl.ds(n * L, L)], dst.at[n], wsem.at[k0 + n])
                for n in range(dst.shape[0])]

    NF = F // FC
    c_wa1 = [w_copy(wa1_h.at[:, pl.ds(c * FC, FC)], wa1.at[:, pl.ds(c * FC, FC)], c) for c in range(NF)]
    c_wb1 = [w_copy(wb1_h.at[pl.ds(c * FC, FC), :], wb1.at[pl.ds(c * FC, FC), :], NF + c)
             for c in range(NF)]
    k0 = 2 * NF
    c_rest = [w_copy(src, dst, k0 + n) for n, (src, dst) in enumerate(
        [(wq_h, wq), (wk_h, wk), (wv_h, wv), (wo_h, wo), (dw_h, dwv), (wp2_h, wp2),
         (wa2_h, wa2), (wb2_h, wb2)])] + col_copies(wp1_h, wp1, k0 + 8)

    def rows(i):
        return i * R if isinstance(i, int) else pl.multiple_of(i * R, 16)

    def x_copy(i):
        return pltpu.make_async_copy(x_hbm.at[pl.ds(rows(i), R), :], xall.at[pl.ds(rows(i), R), :],
                                     xsem.at[i])

    def o_copy(i):
        return pltpu.make_async_copy(xall.at[pl.ds(rows(i), R), :], o_hbm.at[pl.ds(rows(i), R), :],
                                     xsem.at[i])

    def tile(i):
        if isinstance(i, int):
            return i // TPB, (i % TPB) * R
        b = i // TPB
        return b, pl.multiple_of((i - b * TPB) * R, 16)

    def ld_x(i):
        b, r0 = tile(i)
        return _cat([x1[b, n, pl.ds(r0, R), :] for n in range(ND)])

    def st_cols(ref, i, v):
        b, r0 = tile(i)
        for n in range(ND):
            ref[b, n, pl.ds(r0, R), :] = v[:, n * L:(n + 1) * L]

    x_copy(0).start()
    c_wa1[0].start()
    for c in range(NF):
        if c + 1 < NF:
            c_wa1[c + 1].start()
        c_wb1[c].start()
    for t in range(1, NT):
        x_copy(t).start()
    for c in c_rest:
        c.start()

    for b in range(B):
        for n in range(ND):
            hh[b, n, T:TP, :] = jnp.zeros((TP - T, L), _BF16)
            g[b, n, 0:2 * HALO, :] = jnp.zeros((2 * HALO, L), _F32)
            g[b, n, 2 * HALO + T:, :] = jnp.zeros((2 * HALO, L), _F32)
        dc[b, 0:HALO, :] = jnp.zeros((HALO, D), _F32)

    def ff(wa, wb, mid=None, first=False):
        hid = {}

        def up(c):
            if first and c < 3:
                for w in ([c_wa1[0]], [c_wa1[1], c_wb1[0]], c_wa1[2:] + [c_wb1[1]])[c]:
                    w.wait()
            u = jnp.dot(hb[...], wa[:, c * FC:(c + 1) * FC], preferred_element_type=_F32)
            hid[c] = (u + u * jnp.tanh(u)).astype(_BF16)

        def down(c):
            if first and c == 2:
                for w in c_wb1[2:] + [x_copy(1)]:
                    w.wait()
            d = jnp.dot(hid.pop(c), wb[c * FC:(c + 1) * FC, :], preferred_element_type=_F32)
            if c == 0:
                acc[...] = d
            else:
                acc[...] += d

        up(0)
        for c in range(NF):
            if c + 1 < NF:
                up(c + 1)
            if c == NF - 2 and mid is not None:
                mid()
            down(c)

    def ln1(i):
        hb[...] = _ln(xall[pl.ds(rows(i), R), :].astype(_F32), 0.5).astype(_BF16)

    def post_a(i):
        xr = xall[pl.ds(rows(i), R), :].astype(_F32) + 0.5 * acc[...]
        st_cols(x1, i, xr)
        st_cols(hh, i, _ln(xr).astype(_BF16))

    x_copy(0).wait()
    ln1(0)
    ff(wa1, wb1, first=True)
    ln1(1)

    def phase_a(i, carry):
        x_copy(i + 1).wait()
        post_a(i - 1)
        ff(wa1, wb1)
        ln1(i + 1)
        return carry

    jax.lax.fori_loop(1, NT - 1, phase_a, 0)
    for c in c_rest:
        c.wait()
    post_a(NT - 2)
    ff(wa1, wb1)
    for n in range(ND):
        wm[n] = (jax.lax.dot_general(wq[...], wk[n * L:(n + 1) * L, :], _NT,
                                     preferred_element_type=_F32)
                 * (scale * _LOG2E)).astype(_BF16)
        wvo[n] = jnp.dot(wv[...], wo[:, n * L:(n + 1) * L],
                         preferred_element_type=_F32).astype(_BF16)
    dwf[...] = dwv[...].astype(_F32)
    post_a(NT - 1)

    CP = cfg['CP']
    CW = R + HALO
    piece_rows = [(p * CP, CP) for p in range(R // CP)] + [(R, HALO)]

    def q_proj(i, lo=0, hi=ND, after_pass=lambda d: None):
        b, r0 = tile(i)
        r = r0 // 2 if isinstance(r0, int) else pl.multiple_of(r0 // 2, 8)
        h = _cat([_bf(hh32[b, j, pl.ds(r, R // 2), :]) for j in range(ND)])
        for n in range(lo, hi):
            d = jnp.dot(h, wm[n], preferred_element_type=_F32)
            qbuf[n] = d.astype(_BF16)
            after_pass(d)

    def step_b(i, stats, prev=True, conv=True):
        z0 = zero_ref[0]
        nz = [0]

        def fresh(ref):
            nz[0] += 1
            z = pl.multiple_of(z0 * nz[0], 8)
            r32 = ref.bitcast(_U32)
            return _cat([ref[j] for j in range(ND)])

        st = dict(psum=None, stats=stats)
        k = i - 1

        def edge_mask(w0, a):
            _, r0 = tile(k)
            n = a.shape[0]
            parts = [a]
            if w0 == 0:
                parts = [jnp.where(r0 > 0, a[:HALO], 0.0), a[HALO:]]
            if w0 + n > R:
                h = parts[-1]
                cut = h.shape[0] - HALO
                parts[-1:] = [h[:cut], jnp.where(r0 == T - R, h[cut:], 0.0)]
            parts = [q for q in parts if q.shape[0]]
            return parts[0] if len(parts) == 1 else _cat(parts, 0)

        def conv_piece(p):
            b, r0 = tile(k)
            w0, n = piece_rows[p]
            cols = []
            for j in range(ND):
                win = g[b, j, pl.ds(r0 + w0, n + 2 * HALO), :]
                a = None
                for t in range(K):
                    o = HALO - pad + t
                    v = win[o:o + n, :] * dwf[t:t + 1, j * L:(j + 1) * L]
                    a = v if a is None else a + v
                cols.append(a)
            a = _cat(cols)
            dc[b, pl.ds(r0 + w0, n), :] = a
            ps = jnp.sum(edge_mask(w0, a).reshape(n // 8, 8, D), axis=0)
            st['psum'] = ps if st['psum'] is None else st['psum'] + ps

        def conv_finish(part):
            b, r0 = tile(k)
            nparts = cfg['nfin']
            if part == 0:
                cnt = (R - HALO * jnp.asarray(r0 == 0, jnp.int32)
                       + HALO * jnp.asarray(r0 == T - R, jnp.int32)).astype(_F32)
                st['mu'] = jnp.sum(st['psum'], axis=0, keepdims=True) / cnt
                tmean[pl.ds(k, 1), :] = st['mu']
            lo = (CW // 8 * part // nparts) * 8
            hi = (CW // 8 * (part + 1) // nparts) * 8
            dd = dc[b, pl.ds(r0 + lo, hi - lo), :] - st['mu']
            m2 = jnp.sum(edge_mask(lo, dd * dd).reshape((hi - lo) // 8, 8, D), axis=0)
            s = st['stats']
            st['stats'] = (s[0] + st['psum'] if part == 0 else s[0], s[1] + m2)

        def ln3_part(part):
            b, r0 = tile(i - 1)
            rs = R // cfg['lnp']
            x2 = _cat([x1[b, n, pl.ds(pl.multiple_of(r0 + part * rs + z0, 8), rs), :]
                       for n in range(ND)])
            h = _ln(x2, 0.5).astype(_BF16)
            for n in range(ND):
                h3b[n, part * rs:(part + 1) * rs, :] = h[:, n * L:(n + 1) * L]

        def exp_chunk(c):
            ps = []
            for n in range(ND * c, ND * c + ND):
                p = jnp.exp2(sbuf[n] - st['m'])
                ps.append(p.astype(_BF16))
                st['l'] = p if n == 0 else st['l'] + p
            return _cat(ps)

        def gate_g(d):
            g[z0, 0, pl.ds(T + 3 * HALO, 8), :] = d[0:8, :]

        def gate_x(d):
            x1[z0, 0, pl.ds(T, 8), :] = d[0:8, :]

        def gate_s(d):
            r = cfg['egr'] * 8
            sbuf[z0 + NK, 0:8, :] = d[r:r + 8, :]

        def gate_l(d):
            lbuf[pl.ds(pl.multiple_of(R + z0, 8), 8), :] = d[0:8, :]

        def inv_l():
            rbuf[...] = jnp.broadcast_to(1.0 / jnp.sum(lbuf[0:R, :], axis=-1, keepdims=True), (R, L))

        def gate_dc(d):
            dc[z0, pl.ds(T + HALO, 8), 0:L] = d[0:8, :]

        order = cfg['order']
        size = dict(S=NK, A=cfg['ssplit'], B=NK - cfg['ssplit'], W=ND, O=NK, P=2 * ND,
                    Q=cfg['qsplit'], R=ND - cfg['qsplit'])
        start = {}
        for name in order:
            start[name] = sum(size[o] for o in order[:order.index(name)])
        jobs = {}

        def add(seg, t, gate, fn):
            jobs.setdefault(start[seg] + t, []).append((gate, fn))

        if conv:
            for p in range(len(piece_rows)):
                add(cfg['cseg'], cfg['cstart'] + p * cfg['cevery'], gate_g,
                    functools.partial(conv_piece, p))
            for p in range(cfg['nfin']):
                add(cfg['fseg'], cfg['fin'] + p * cfg['fevery'], gate_dc,
                    functools.partial(conv_finish, p))
        if cfg['rseg']:
            add(cfg['rseg'], cfg['rpos'], gate_l, inv_l)
        if prev:
            for p in range(cfg['lnp']):
                add(cfg['lseg'], cfg['lstart'] + p * cfg['levery'], gate_x,
                    functools.partial(ln3_part, p))

        def span(fn):
            at = [t for t, js in jobs.items() for _, j in js if getattr(j, 'func', j) is fn]
            return min(at), max(at)

        if prev:
            assert start['W'] + ND - 1 <= span(ln3_part)[0] and span(ln3_part)[1] < start['P']
        if conv:
            assert start['P'] + 2 * ND - 1 <= span(conv_piece)[0]
            assert span(conv_piece)[1] <= span(conv_finish)[0]
        assert start['O'] + NK - 1 <= span(inv_l)[0]

        def after_pass(t, d):
            for gate, fn in jobs.pop(t, []):
                gate(d)
                fn()

        b, _ = tile(i)

        def seg_s(lo, hi, t0):
            for n in range(lo, hi):
                keys = _cat([_bf(hh32[b, j, pl.ds(n * L // 2, L // 2), :]) for j in range(ND)])
                s = jax.lax.dot_general(fresh(qbuf), keys, _NT, preferred_element_type=_F32)
                if (n + 1) * L > T:
                    if isinstance(i, int):
                        s = s + kbias[n - T // L]
                    else:
                        col = jax.lax.broadcasted_iota(jnp.int32, (1, L), 1) + n * L
                        s = jnp.where(col < T, s, -1e30)
                sbuf[n] = s
                st['mm'] = s if n == 0 else jnp.maximum(st['mm'], s)
                after_pass(t0 + n - lo, s)
            if hi == NK:
                st['m'] = jnp.max(st['mm'], axis=-1, keepdims=True)

        def seg_w(t0):
            b1, r1 = tile(i - 1)
            for n in range(ND):
                d = jnp.dot(fresh(o16), wvo[n], preferred_element_type=_F32)
                x1[b1, n, pl.ds(r1, R), :] += d * rbuf[...]
                after_pass(t0 + n, d)

        def seg_o(t0):
            NC = NK // ND
            p = exp_chunk(0)
            o = [None] * ND
            for c in range(NC):
                pn = None
                for n in range(ND):
                    v = _bf(hh32[b, n, pl.ds(c * ND * L // 2, ND * L // 2), :])
                    d = jnp.dot(p, v, preferred_element_type=_F32)
                    o[n] = d if c == 0 else o[n] + d
                    if c + 1 == NC:
                        o16[n] = o[n].astype(_BF16)
                    if n == cfg['egn'] and c + 1 < NC:
                        gate_s(d)
                        pn = exp_chunk(c + 1)
                    after_pass(t0 + c * ND + n, d)
                p = pn
            if cfg['rseg']:
                lbuf[0:R, :] = st['l']
            else:
                rbuf[...] = jnp.broadcast_to(1.0 / jnp.sum(st['l'], axis=-1, keepdims=True), (R, L))

        def seg_q(lo, hi, t0):
            cnt = [t0]

            def ap(d):
                after_pass(cnt[0], d)
                cnt[0] += 1
            q_proj(i + 1 if isinstance(i, int) else jnp.minimum(i + 1, NT - 1), lo, hi, ap)

        def seg_p(t0):
            b1, r1 = tile(i - 1)
            for n in range(ND):
                a = jnp.dot(fresh(h3b), wp1[n], preferred_element_type=_F32)
                after_pass(t0 + 2 * n, a)
                bb = jnp.dot(fresh(h3b), wp1[ND + n], preferred_element_type=_F32)
                g[b1, n, pl.ds(r1 + 2 * HALO, R), :] = a + a * jnp.tanh(bb)
                after_pass(t0 + 2 * n + 1, bb)

        segs = dict(S=(True, functools.partial(seg_s, 0, NK)),
                    A=(True, functools.partial(seg_s, 0, cfg['ssplit'])),
                    B=(True, functools.partial(seg_s, cfg['ssplit'], NK)), W=(prev, seg_w), O=(True, seg_o), Q=(True, functools.partial(seg_q, 0, cfg['qsplit'])),
                    R=(True, functools.partial(seg_q, cfg['qsplit'], ND)),
                    P=(prev, seg_p))
        for name in order:
            on, fn = segs[name]
            if on:
                fn(start[name])
            for t in range(start[name], start[name] + size[name]):
                for _, job in jobs.pop(t, []):
                    job()
        assert not jobs
        return st['stats']

    stats = (jnp.zeros((8, D), _F32), jnp.zeros((8, D), _F32))
    q_proj(0)
    stats = step_b(0, stats, prev=False, conv=False)
    stats = jax.lax.fori_loop(1, NT, step_b, stats)

    last = NT - 1
    b1, r1 = tile(last)
    RH = (R // 32) * 16
    for lo, hi in ((0, RH), (RH, R)):
        o = _cat([o16[c, lo:hi, :] for c in range(ND)])
        for n in range(ND):
            d = jnp.dot(o, wvo[n], preferred_element_type=_F32)
            x1[b1, n, r1 + lo:r1 + hi, :] += d * rbuf[lo:hi, :]
    for lo, hi in ((0, RH), (RH, R)):
        h = _ln(_cat([x1[b1, n, r1 + lo:r1 + hi, :] for n in range(ND)]), 0.5).astype(_BF16)
        for j in range(ND):
            a = jnp.dot(h, wp1[j], preferred_element_type=_F32)
            bb = jnp.dot(h, wp1[ND + j], preferred_element_type=_F32)
            g[b1, j, r1 + 2 * HALO + lo:r1 + 2 * HALO + hi, :] = a + a * jnp.tanh(bb)

    TPR = cfg['TP']
    shift = tmean[last - 1:last, :]

    def tail_conv(p, carry):
        w0 = pl.multiple_of(p * TPR, 8)
        c1, c2 = [], []
        for j in range(ND):
            a = None
            for t in range(K):
                v = (g[b1, j, pl.ds(r1 + w0 + HALO - pad + t, TPR), :]
                     * dwf[t:t + 1, j * L:(j + 1) * L])
                a = v if a is None else a + v
            dc[b1, pl.ds(r1 + w0, TPR), j * L:(j + 1) * L] = a
            dd = (a - shift[:, j * L:(j + 1) * L]).reshape(TPR // 8, 8, L)
            c1.append(jnp.sum(dd, axis=0))
            c2.append(jnp.sum(dd * dd, axis=0))
        return carry[0] + _cat(c1), carry[1] + _cat(c2)

    t1, t2 = jax.lax.fori_loop(0, CW // TPR, tail_conv,
                               (jnp.zeros((8, D), _F32), jnp.zeros((8, D), _F32)))
    t1 = jnp.sum(t1, axis=0, keepdims=True)
    t2 = jnp.sum(t2, axis=0, keepdims=True)
    tmean[last:NT, :] = shift + t1 * (1.0 / CW)

    trow = jax.lax.broadcasted_iota(jnp.int32, (NT, 1), 0) % TPB
    tcnt = (R - HALO * (trow == 0).astype(jnp.int32)
            + HALO * (trow == TPB - 1).astype(jnp.int32)).astype(_F32)
    mu = (jnp.sum(stats[0], axis=0, keepdims=True) + (t1 + CW * shift)) * (1.0 / N)
    dm = tmean[...] - mu
    var = (jnp.sum(stats[1], axis=0, keepdims=True) + (t2 - t1 * t1 * (1.0 / CW))
           + jnp.sum(dm * dm * tcnt, axis=0, keepdims=True)) * (1.0 / N)
    rstd = jax.lax.rsqrt(var + _EPS) * 0.5

    def pw2(i):
        b, r0 = tile(i)
        u = (dc[b, pl.ds(r0 + HALO, R), :] - mu) * rstd
        a = (u + u * jnp.tanh(u)).astype(_BF16)
        st_cols(x1, i, ld_x(i) + jnp.dot(a, wp2[...], preferred_element_type=_F32))

    def ln4(i):
        hb[...] = _ln(ld_x(i), 0.5).astype(_BF16)

    def post_d(i):
        xall[pl.ds(rows(i), R), :] = _ln(ld_x(i) + 0.5 * acc[...]).astype(_BF16)
        o_copy(i).start()

    pw2(0)
    pw2(1)
    ln4(0)
    ff(wa2, wb2)
    ln4(1)

    def phase_d(i, carry):
        post_d(i - 1)
        ff(wa2, wb2, mid=lambda: pw2(i + 1))
        ln4(i + 1)
        return carry

    jax.lax.fori_loop(1, NT - 1, phase_d, 0)
    post_d(NT - 2)
    ff(wa2, wb2)
    bl, rl = tile(NT - 1)
    RQ = R // cfg['oparts']
    tails = []
    for q in range(cfg['oparts']):
        lo = (NT - 1) * R + q * RQ
        x4 = (_cat([x1[bl, n, rl + q * RQ:rl + (q + 1) * RQ, :] for n in range(ND)])
              + 0.5 * acc[q * RQ:(q + 1) * RQ, :])
        xall[lo:lo + RQ, :] = _ln(x4).astype(_BF16)
        tails.append(pltpu.make_async_copy(xall.at[pl.ds(lo, RQ), :], o_hbm.at[pl.ds(lo, RQ), :],
                                           wsem.at[q]))
        tails[-1].start()
    for t in range(NT - 1):
        o_copy(t).wait()
    for c in tails:
        c.wait()


@jax.jit
def pallas_standalone__conformer_family_conformer__speech_kernel(
    x: jax.Array,
    w_ff1_a: jax.Array,
    w_ff1_b: jax.Array,
    w_q: jax.Array,
    w_k: jax.Array,
    w_v: jax.Array,
    w_o: jax.Array,
    w_pw1: jax.Array,
    dw: jax.Array,
    w_pw2: jax.Array,
    w_ff2_a: jax.Array,
    w_ff2_b: jax.Array,
):
    B, T, D = x.shape
    K = dw.shape[0]
    N = B * T
    TP = -(-T // D) * D
    ND = D // L
    assert T % R == 0 and K // 2 <= HALO and K - 1 - K // 2 <= HALO and D % L == 0

    weights = (w_ff1_a, w_ff1_b, w_q, w_k, w_v, w_o, w_pw1, dw, w_pw2, w_ff2_a, w_ff2_b)
    V = pltpu.VMEM
    scratch = [V(w.shape, w.dtype) for w in weights[:6]]
    scratch += [V((2 * ND, D, L), _BF16)]
    scratch += [V(w.shape, w.dtype) for w in weights[7:]]
    scratch += [
        V((ND, D, L), _BF16),
        V((ND, D, L), _BF16),
        V((N, D), x.dtype),
        V((B, ND, T + 8, L), _F32),
        V((B, ND, TP, L), _BF16),
        V((B, ND, T + 4 * HALO, L), _F32),
        V((B, T + 2 * HALO, D), _F32),
        V((TP // L + 1, R, L), _F32),
        V((R, D), _BF16),
        V((R, D), _F32),
        V((ND, R, L), _BF16),
        V((ND, R, L), _BF16),
        V((ND, R, L), _BF16),
        V((R, L), _F32),
        V((R + 8, L), _F32),
        V((K, D), _F32),
        V((N // R, D), _F32),
        pltpu.SemaphoreType.DMA((8 + 2 * (w_ff1_a.shape[1] // FC) + 2 * ND,)),
        pltpu.SemaphoreType.DMA((N // R,)),
    ]
    col = np.arange(T // L * L, TP).reshape(-1, 1, L)
    kbias = np.where(col < T, 0.0, -1e30).astype(np.float32)
    out = pl.pallas_call(
        functools.partial(_kernel, B=B, T=T, D=D, K=K),
        out_shape=jax.ShapeDtypeStruct((N, D), x.dtype),
        in_specs=([pl.BlockSpec(memory_space=pltpu.SMEM), pl.BlockSpec(memory_space=pltpu.VMEM)]
                  + [pl.BlockSpec(memory_space=pl.ANY)] * (1 + len(weights))),
        out_specs=pl.BlockSpec(memory_space=pl.ANY),
        scratch_shapes=scratch,
        compiler_params=pltpu.CompilerParams(
            vmem_limit_bytes=120 * 2**20,
            flags={"XLA_TPU_EVENLY_DISTRIBUTE_CRITICAL_NODES": True},
        ),
        name="conformer",
    )(np.zeros((1,), np.int32), kbias, x.reshape(N, D), *weights)
    return out.reshape(B, T, D)
```

```python
import functools

import jax
import jax.numpy as jnp
import numpy as np
import jax.experimental.pallas as pl
import jax.experimental.pallas.tpu as pltpu

_EPS = 1e-05
_LOG2E = 1.4426950408889634

R = 400
FC = 512
HALO = 8
L = 128

CFG = dict(order='WAPBQOR', ssplit=6, qsplit=2, CP=40, cseg='B', cstart=1, cevery=1, lseg='A', lnp=5, lstart=0, levery=1,
           egn=1, egr=5, fseg='O', fin=3, nfin=3, fevery=4, rseg='R', rpos=0, TB=80)

_NT = (((1,), (1,)), ((), ()))
_F32 = jnp.float32
_BF16 = jnp.bfloat16
_U32 = jnp.uint32


def _cat(xs, axis=1):
    return jnp.concatenate(xs, axis=axis)


def _bf(x):
    return pltpu.bitcast(x, _BF16)


def _ln(x, scale=None):
    d = x.shape[-1]
    m = jnp.sum(x, axis=-1, keepdims=True) * (1.0 / d)
    xc = x - m
    v = jnp.sum(xc * xc, axis=-1, keepdims=True) * (1.0 / d)
    r = jax.lax.rsqrt(v + _EPS)
    if scale is not None:
        r = r * scale
    return xc * r


def _kernel(zero_ref, kbias,
            x_hbm, wa1_h, wb1_h, wq_h, wk_h, wv_h, wo_h, wp1_h, dw_h, wp2_h, wa2_h, wb2_h,
            o_hbm,
            wa1, wb1, wq, wk, wv, wo, wp1, dwv, wp2, wa2, wb2, wm, wvo,
            xall, x1, hh, g, dc, sbuf, hb, acc, qbuf, o16, h3b, rbuf, lbuf, dwf, tmean,
            wsem, xsem,
            *, B, T, D, K):
    N = B * T
    NT = N // R
    TPB = T // R
    TP = hh.shape[2]
    F = wa1.shape[1]
    NK = TP // L
    ND = D // L
    scale = D ** -0.5
    pad = K // 2
    cfg = CFG
    hh32 = hh.bitcast(_U32)

    def w_copy(src, dst, k):
        return pltpu.make_async_copy(src, dst, wsem.at[k])

    def col_copies(src, dst, k0):
        return [pltpu.make_async_copy(src.at[:, pl.ds(n * L, L)], dst.at[n], wsem.at[k0 + n])
                for n in range(dst.shape[0])]

    NF = F // FC
    c_wa1 = [w_copy(wa1_h.at[:, pl.ds(c * FC, FC)], wa1.at[:, pl.ds(c * FC, FC)], c) for c in range(NF)]
    c_wb1 = [w_copy(wb1_h.at[pl.ds(c * FC, FC), :], wb1.at[pl.ds(c * FC, FC), :], NF + c)
             for c in range(NF)]
    k0 = 2 * NF
    c_rest = [w_copy(src, dst, k0 + n) for n, (src, dst) in enumerate(
        [(wq_h, wq), (wk_h, wk), (wv_h, wv), (wo_h, wo), (dw_h, dwv), (wp2_h, wp2),
         (wa2_h, wa2), (wb2_h, wb2)])] + col_copies(wp1_h, wp1, k0 + 8)

    def rows(i):
        return i * R if isinstance(i, int) else pl.multiple_of(i * R, 16)

    def x_copy(i):
        return pltpu.make_async_copy(x_hbm.at[pl.ds(rows(i), R), :], xall.at[pl.ds(rows(i), R), :],
                                     xsem.at[i])

    def o_copy(i):
        return pltpu.make_async_copy(xall.at[pl.ds(rows(i), R), :], o_hbm.at[pl.ds(rows(i), R), :],
                                     xsem.at[i])

    def tile(i):
        if isinstance(i, int):
            return i // TPB, (i % TPB) * R
        b = i // TPB
        return b, pl.multiple_of((i - b * TPB) * R, 16)

    def ld_x(i):
        b, r0 = tile(i)
        return _cat([x1[b, n, pl.ds(r0, R), :] for n in range(ND)])

    def st_cols(ref, i, v):
        b, r0 = tile(i)
        for n in range(ND):
            ref[b, n, pl.ds(r0, R), :] = v[:, n * L:(n + 1) * L]

    x_copy(0).start()
    c_wa1[0].start()
    for c in range(NF):
        if c + 1 < NF:
            c_wa1[c + 1].start()
        c_wb1[c].start()
    for t in range(1, NT):
        x_copy(t).start()
    for c in c_rest:
        c.start()

    for b in range(B):
        for n in range(ND):
            hh[b, n, T:TP, :] = jnp.zeros((TP - T, L), _BF16)
            g[b, n, 0:2 * HALO, :] = jnp.zeros((2 * HALO, L), _F32)
            g[b, n, 2 * HALO + T:, :] = jnp.zeros((2 * HALO, L), _F32)
        dc[b, 0:HALO, :] = jnp.zeros((HALO, D), _F32)

    def ff(wa, wb, mid=None, first=False, finish=None):
        hid = {}

        def up(c):
            if first and c < 3:
                for w in ([c_wa1[0]], [c_wa1[1], c_wb1[0]], c_wa1[2:] + [c_wb1[1]])[c]:
                    w.wait()
            u = jnp.dot(hb[...], wa[:, c * FC:(c + 1) * FC], preferred_element_type=_F32)
            hid[c] = (u + u * jnp.tanh(u)).astype(_BF16)

        def down(c):
            if first and c == 2:
                for w in c_wb1[2:] + [x_copy(1)]:
                    w.wait()
            if finish is not None and c == NF - 1:
                h = hid.pop(c)
                for lo in range(0, R, cfg['TB']):
                    hi = lo + cfg['TB']
                    d = jnp.dot(h[lo:hi], wb[c * FC:(c + 1) * FC, :], preferred_element_type=_F32)
                    finish(lo, hi, acc[lo:hi, :] + d)
                return
            d = jnp.dot(hid.pop(c), wb[c * FC:(c + 1) * FC, :], preferred_element_type=_F32)
            if c == 0:
                acc[...] = d
            else:
                acc[...] += d

        up(0)
        for c in range(NF):
            if c + 1 < NF:
                up(c + 1)
            if c == NF - 2 and mid is not None:
                mid()
            down(c)

    def ln1(i):
        hb[...] = _ln(xall[pl.ds(rows(i), R), :].astype(_F32), 0.5).astype(_BF16)

    def post_a(i):
        xr = xall[pl.ds(rows(i), R), :].astype(_F32) + 0.5 * acc[...]
        st_cols(x1, i, xr)
        st_cols(hh, i, _ln(xr).astype(_BF16))

    x_copy(0).wait()
    ln1(0)
    ff(wa1, wb1, first=True)
    ln1(1)

    def phase_a(i, carry):
        x_copy(i + 1).wait()
        post_a(i - 1)
        ff(wa1, wb1)
        ln1(i + 1)
        return carry

    jax.lax.fori_loop(1, NT - 1, phase_a, 0)
    for c in c_rest:
        c.wait()
    post_a(NT - 2)
    ff(wa1, wb1)
    for n in range(ND):
        wm[n] = (jax.lax.dot_general(wq[...], wk[n * L:(n + 1) * L, :], _NT,
                                     preferred_element_type=_F32)
                 * (scale * _LOG2E)).astype(_BF16)
        wvo[n] = jnp.dot(wv[...], wo[:, n * L:(n + 1) * L],
                         preferred_element_type=_F32).astype(_BF16)
    dwf[...] = dwv[...].astype(_F32)
    post_a(NT - 1)

    CP = cfg['CP']
    CW = R + HALO
    piece_rows = [(p * CP, CP) for p in range(R // CP)] + [(R, HALO)]

    def q_proj(i, lo=0, hi=ND, after_pass=lambda d: None):
        b, r0 = tile(i)
        r = r0 // 2 if isinstance(r0, int) else pl.multiple_of(r0 // 2, 8)
        h = _cat([_bf(hh32[b, j, pl.ds(r, R // 2), :]) for j in range(ND)])
        for n in range(lo, hi):
            d = jnp.dot(h, wm[n], preferred_element_type=_F32)
            qbuf[n] = d.astype(_BF16)
            after_pass(d)

    def step_b(i, stats, prev=True, conv=True, early=False):
        z0 = zero_ref[0]
        nz = [0]

        def fresh(ref):
            nz[0] += 1
            z = pl.multiple_of(z0 * nz[0], 8)
            r32 = ref.bitcast(_U32)
            return _cat([ref[j] for j in range(ND)])

        st = dict(psum=None, stats=stats)
        k = i - 1

        def edge_mask(w0, a):
            _, r0 = tile(k)
            n = a.shape[0]
            parts = [a]
            if w0 == 0:
                parts = [jnp.where(r0 > 0, a[:HALO], 0.0), a[HALO:]]
            if w0 + n > R:
                h = parts[-1]
                cut = h.shape[0] - HALO
                parts[-1:] = [h[:cut], jnp.where(r0 == T - R, h[cut:], 0.0)]
            parts = [q for q in parts if q.shape[0]]
            return parts[0] if len(parts) == 1 else _cat(parts, 0)

        def conv_piece(p):
            b, r0 = tile(k)
            w0, n = piece_rows[p]
            cols = []
            for j in range(ND):
                win = g[b, j, pl.ds(r0 + w0, n + 2 * HALO), :]
                a = None
                for t in range(K):
                    o = HALO - pad + t
                    v = win[o:o + n, :] * dwf[t:t + 1, j * L:(j + 1) * L]
                    a = v if a is None else a + v
                cols.append(a)
            a = _cat(cols)
            dc[b, pl.ds(r0 + w0, n), :] = a
            ps = jnp.sum(edge_mask(w0, a).reshape(n // 8, 8, D), axis=0)
            st['psum'] = ps if st['psum'] is None else st['psum'] + ps

        def conv_finish(part):
            b, r0 = tile(k)
            nparts = cfg['nfin']
            if part == 0:
                cnt = (R - HALO * jnp.asarray(r0 == 0, jnp.int32)
                       + HALO * jnp.asarray(r0 == T - R, jnp.int32)).astype(_F32)
                st['mu'] = jnp.sum(st['psum'], axis=0, keepdims=True) / cnt
                tmean[pl.ds(k, 1), :] = st['mu']
            lo = (CW // 8 * part // nparts) * 8
            hi = (CW // 8 * (part + 1) // nparts) * 8
            dd = dc[b, pl.ds(r0 + lo, hi - lo), :] - st['mu']
            m2 = jnp.sum(edge_mask(lo, dd * dd).reshape((hi - lo) // 8, 8, D), axis=0)
            s = st['stats']
            st['stats'] = (s[0] + st['psum'] if part == 0 else s[0], s[1] + m2)

        def ln3_part(part):
            b, r0 = tile(i - 1)
            rs = R // cfg['lnp']
            x2 = _cat([x1[b, n, pl.ds(pl.multiple_of(r0 + part * rs + z0, 8), rs), :]
                       for n in range(ND)])
            h = _ln(x2, 0.5).astype(_BF16)
            for n in range(ND):
                h3b[n, part * rs:(part + 1) * rs, :] = h[:, n * L:(n + 1) * L]

        def exp_chunk(c):
            ps = []
            for n in range(ND * c, ND * c + ND):
                p = jnp.exp2(sbuf[n] - st['m'])
                ps.append(p.astype(_BF16))
                st['l'] = p if n == 0 else st['l'] + p
            return _cat(ps)

        def gate_g(d):
            g[z0, 0, pl.ds(T + 3 * HALO, 8), :] = d[0:8, :]

        def gate_x(d):
            x1[z0, 0, pl.ds(T, 8), :] = d[0:8, :]

        def gate_s(d):
            r = cfg['egr'] * 8
            sbuf[z0 + NK, 0:8, :] = d[r:r + 8, :]

        def gate_l(d):
            lbuf[pl.ds(pl.multiple_of(R + z0, 8), 8), :] = d[0:8, :]

        def inv_l():
            rbuf[...] = jnp.broadcast_to(1.0 / jnp.sum(lbuf[0:R, :], axis=-1, keepdims=True), (R, L))

        def gate_dc(d):
            dc[z0, pl.ds(T + HALO, 8), 0:L] = d[0:8, :]

        order = cfg['order']
        size = dict(S=NK, A=cfg['ssplit'], B=NK - cfg['ssplit'], W=ND, O=NK, P=2 * ND,
                    Q=cfg['qsplit'], R=ND - cfg['qsplit'])
        start = {}
        for name in order:
            start[name] = sum(size[o] for o in order[:order.index(name)])
        jobs = {}

        def add(seg, t, gate, fn):
            jobs.setdefault(start[seg] + t, []).append((gate, fn))

        if conv:
            for p in range(len(piece_rows)):
                add(cfg['cseg'], cfg['cstart'] + p * cfg['cevery'], gate_g,
                    functools.partial(conv_piece, p))
            for p in range(cfg['nfin']):
                add(cfg['fseg'], cfg['fin'] + p * cfg['fevery'], gate_dc,
                    functools.partial(conv_finish, p))
        if cfg['rseg']:
            add(cfg['rseg'], cfg['rpos'], gate_l, inv_l)
        if prev:
            for p in range(cfg['lnp']):
                add(cfg['lseg'], cfg['lstart'] + p * cfg['levery'], gate_x,
                    functools.partial(ln3_part, p))

        def span(fn):
            at = [t for t, js in jobs.items() for _, j in js if getattr(j, 'func', j) is fn]
            return min(at), max(at)

        if prev:
            assert start['W'] + ND - 1 <= span(ln3_part)[0] and span(ln3_part)[1] < start['P']
        if conv:
            assert start['P'] + 2 * ND - 1 <= span(conv_piece)[0]
            assert span(conv_piece)[1] <= span(conv_finish)[0]
        assert start['O'] + NK - 1 <= span(inv_l)[0]

        def after_pass(t, d):
            for gate, fn in jobs.pop(t, []):
                gate(d)
                fn()

        b, _ = tile(i)

        def seg_s(lo, hi, t0):
            for n in range(lo, hi):
                keys = _cat([_bf(hh32[b, j, pl.ds(n * L // 2, L // 2), :]) for j in range(ND)])
                s = jax.lax.dot_general(fresh(qbuf), keys, _NT, preferred_element_type=_F32)
                if (n + 1) * L > T:
                    if early:
                        s = s + kbias[n - T // L]
                    else:
                        col = jax.lax.broadcasted_iota(jnp.int32, (1, L), 1) + n * L
                        s = jnp.where(col < T, s, -1e30)
                sbuf[n] = s
                st['mm'] = s if n == 0 else jnp.maximum(st['mm'], s)
                after_pass(t0 + n - lo, s)
            if hi == NK:
                st['m'] = jnp.max(st['mm'], axis=-1, keepdims=True)

        def seg_w(t0):
            b1, r1 = tile(i - 1)
            for n in range(ND):
                d = jnp.dot(fresh(o16), wvo[n], preferred_element_type=_F32)
                x1[b1, n, pl.ds(r1, R), :] += d * rbuf[...]
                after_pass(t0 + n, d)

        def seg_o(t0):
            NC = NK // ND
            p = exp_chunk(0)
            o = [None] * ND
            for c in range(NC):
                pn = None
                for n in range(ND):
                    v = _bf(hh32[b, n, pl.ds(c * ND * L // 2, ND * L // 2), :])
                    d = jnp.dot(p, v, preferred_element_type=_F32)
                    o[n] = d if c == 0 else o[n] + d
                    if c + 1 == NC:
                        o16[n] = o[n].astype(_BF16)
                    if n == cfg['egn'] and c + 1 < NC:
                        gate_s(d)
                        pn = exp_chunk(c + 1)
                    after_pass(t0 + c * ND + n, d)
                p = pn
            if cfg['rseg']:
                lbuf[0:R, :] = st['l']
            else:
                rbuf[...] = jnp.broadcast_to(1.0 / jnp.sum(st['l'], axis=-1, keepdims=True), (R, L))

        def seg_q(lo, hi, t0):
            cnt = [t0]

            def ap(d):
                after_pass(cnt[0], d)
                cnt[0] += 1
            q_proj(i + 1 if isinstance(i, int) else jnp.minimum(i + 1, NT - 1), lo, hi, ap)

        def seg_p(t0):
            b1, r1 = tile(i - 1)
            for n in range(ND):
                a = jnp.dot(fresh(h3b), wp1[n], preferred_element_type=_F32)
                after_pass(t0 + 2 * n, a)
                bb = jnp.dot(fresh(h3b), wp1[ND + n], preferred_element_type=_F32)
                g[b1, n, pl.ds(r1 + 2 * HALO, R), :] = a + a * jnp.tanh(bb)
                after_pass(t0 + 2 * n + 1, bb)

        segs = dict(S=(True, functools.partial(seg_s, 0, NK)),
                    A=(True, functools.partial(seg_s, 0, cfg['ssplit'])),
                    B=(True, functools.partial(seg_s, cfg['ssplit'], NK)), W=(prev, seg_w), O=(True, seg_o), Q=(True, functools.partial(seg_q, 0, cfg['qsplit'])),
                    R=(True, functools.partial(seg_q, cfg['qsplit'], ND)),
                    P=(prev, seg_p))
        for name in order:
            on, fn = segs[name]
            if on:
                fn(start[name])
            for t in range(start[name], start[name] + size[name]):
                for _, job in jobs.pop(t, []):
                    job()
        assert not jobs
        return st['stats']

    stats = (jnp.zeros((8, D), _F32), jnp.zeros((8, D), _F32))
    q_proj(0)
    stats = step_b(zero_ref[0], stats, prev=False, conv=False, early=True)
    stats = jax.lax.fori_loop(1, NT, step_b, stats)

    last = NT - 1
    b1, r1 = tile(last)
    RB = cfg['TB']
    blocks = [(lo, lo + RB) for lo in range(0, R, RB)]
    for lo, hi in blocks:
        o = _cat([o16[c, lo:hi, :] for c in range(ND)])
        for n in range(ND):
            d = jnp.dot(o, wvo[n], preferred_element_type=_F32)
            x1[b1, n, r1 + lo:r1 + hi, :] += d * rbuf[lo:hi, :]
    shift = tmean[last - 1:last, :]
    t1 = jnp.zeros((8, D), _F32)
    t2 = jnp.zeros((8, D), _F32)

    def conv_rows(lo, hi):
        c1, c2 = [], []
        for j in range(ND):
            a = None
            for t in range(K):
                v = (g[b1, j, r1 + lo + HALO - pad + t:r1 + hi + HALO - pad + t, :]
                     * dwf[t:t + 1, j * L:(j + 1) * L])
                a = v if a is None else a + v
            dc[b1, r1 + lo:r1 + hi, j * L:(j + 1) * L] = a
            dd = (a - shift[:, j * L:(j + 1) * L]).reshape((hi - lo) // 8, 8, L)
            c1.append(jnp.sum(dd, axis=0))
            c2.append(jnp.sum(dd * dd, axis=0))
        return _cat(c1), _cat(c2)

    for lo, hi in blocks:
        h = _ln(_cat([x1[b1, n, r1 + lo:r1 + hi, :] for n in range(ND)]), 0.5).astype(_BF16)
        for j in range(ND):
            a = jnp.dot(h, wp1[j], preferred_element_type=_F32)
            bb = jnp.dot(h, wp1[ND + j], preferred_element_type=_F32)
            g[b1, j, r1 + 2 * HALO + lo:r1 + 2 * HALO + hi, :] = a + a * jnp.tanh(bb)
        c1, c2 = conv_rows(lo, hi if hi < R else CW)
        t1, t2 = t1 + c1, t2 + c2
    t1 = jnp.sum(t1, axis=0, keepdims=True)
    t2 = jnp.sum(t2, axis=0, keepdims=True)
    tmean[last:NT, :] = shift + t1 * (1.0 / CW)

    trow = jax.lax.broadcasted_iota(jnp.int32, (NT, 1), 0) % TPB
    tcnt = (R - HALO * (trow == 0).astype(jnp.int32)
            + HALO * (trow == TPB - 1).astype(jnp.int32)).astype(_F32)
    mu = (jnp.sum(stats[0], axis=0, keepdims=True) + (t1 + CW * shift)) * (1.0 / N)
    dm = tmean[...] - mu
    var = (jnp.sum(stats[1], axis=0, keepdims=True) + (t2 - t1 * t1 * (1.0 / CW))
           + jnp.sum(dm * dm * tcnt, axis=0, keepdims=True)) * (1.0 / N)
    rstd = jax.lax.rsqrt(var + _EPS) * 0.5

    def pw2(i):
        b, r0 = tile(i)
        u = (dc[b, pl.ds(r0 + HALO, R), :] - mu) * rstd
        a = (u + u * jnp.tanh(u)).astype(_BF16)
        st_cols(x1, i, ld_x(i) + jnp.dot(a, wp2[...], preferred_element_type=_F32))

    def ln4(i):
        hb[...] = _ln(ld_x(i), 0.5).astype(_BF16)

    def post_d(i):
        xall[pl.ds(rows(i), R), :] = _ln(ld_x(i) + 0.5 * acc[...]).astype(_BF16)
        o_copy(i).start()

    pw2(0)
    pw2(1)
    ln4(0)
    ff(wa2, wb2)
    ln4(1)

    def phase_d(i, carry):
        post_d(i - 1)
        ff(wa2, wb2, mid=lambda: pw2(i + 1))
        ln4(i + 1)
        return carry

    jax.lax.fori_loop(1, NT - 1, phase_d, 0)
    post_d(NT - 2)
    bl, rl = tile(NT - 1)
    tails = []

    def leave(lo, hi, f):
        x4 = _cat([x1[bl, n, rl + lo:rl + hi, :] for n in range(ND)]) + 0.5 * f
        o0 = (NT - 1) * R + lo
        xall[o0:o0 + hi - lo, :] = _ln(x4).astype(_BF16)
        tails.append(pltpu.make_async_copy(xall.at[pl.ds(o0, hi - lo), :],
                                           o_hbm.at[pl.ds(o0, hi - lo), :], wsem.at[len(tails)]))
        tails[-1].start()

    ff(wa2, wb2, finish=leave)
    for t in range(NT - 1):
        o_copy(t).wait()
    for c in tails:
        c.wait()


@jax.jit
def pallas_standalone__conformer_family_conformer__speech_kernel(
    x: jax.Array,
    w_ff1_a: jax.Array,
    w_ff1_b: jax.Array,
    w_q: jax.Array,
    w_k: jax.Array,
    w_v: jax.Array,
    w_o: jax.Array,
    w_pw1: jax.Array,
    dw: jax.Array,
    w_pw2: jax.Array,
    w_ff2_a: jax.Array,
    w_ff2_b: jax.Array,
):
    B, T, D = x.shape
    K = dw.shape[0]
    N = B * T
    TP = -(-T // D) * D
    ND = D // L
    assert T % R == 0 and K // 2 <= HALO and K - 1 - K // 2 <= HALO and D % L == 0

    weights = (w_ff1_a, w_ff1_b, w_q, w_k, w_v, w_o, w_pw1, dw, w_pw2, w_ff2_a, w_ff2_b)
    V = pltpu.VMEM
    scratch = [V(w.shape, w.dtype) for w in weights[:6]]
    scratch += [V((2 * ND, D, L), _BF16)]
    scratch += [V(w.shape, w.dtype) for w in weights[7:]]
    scratch += [
        V((ND, D, L), _BF16),
        V((ND, D, L), _BF16),
        V((N, D), x.dtype),
        V((B, ND, T + 8, L), _F32),
        V((B, ND, TP, L), _BF16),
        V((B, ND, T + 4 * HALO, L), _F32),
        V((B, T + 2 * HALO, D), _F32),
        V((TP // L + 1, R, L), _F32),
        V((R, D), _BF16),
        V((R, D), _F32),
        V((ND, R, L), _BF16),
        V((ND, R, L), _BF16),
        V((ND, R, L), _BF16),
        V((R, L), _F32),
        V((R + 8, L), _F32),
        V((K, D), _F32),
        V((N // R, D), _F32),
        pltpu.SemaphoreType.DMA((8 + 2 * (w_ff1_a.shape[1] // FC) + 2 * ND,)),
        pltpu.SemaphoreType.DMA((N // R,)),
    ]
    col = np.arange(T // L * L, TP).reshape(-1, 1, L)
    kbias = np.where(col < T, 0.0, -1e30).astype(np.float32)
    out = pl.pallas_call(
        functools.partial(_kernel, B=B, T=T, D=D, K=K),
        out_shape=jax.ShapeDtypeStruct((N, D), x.dtype),
        in_specs=([pl.BlockSpec(memory_space=pltpu.SMEM), pl.BlockSpec(memory_space=pltpu.VMEM)]
                  + [pl.BlockSpec(memory_space=pl.ANY)] * (1 + len(weights))),
        out_specs=pl.BlockSpec(memory_space=pl.ANY),
        scratch_shapes=scratch,
        compiler_params=pltpu.CompilerParams(
            vmem_limit_bytes=120 * 2**20,
            flags={"XLA_TPU_EVENLY_DISTRIBUTE_CRITICAL_NODES": True},
        ),
        name="conformer",
    )(np.zeros((1,), np.int32), kbias, x.reshape(N, D), *weights)
    return out.reshape(B, T, D)
```

```python
import functools

import jax
import jax.numpy as jnp
import numpy as np
import jax.experimental.pallas as pl
import jax.experimental.pallas.tpu as pltpu

_EPS = 1e-05
_LOG2E = 1.4426950408889634

R = 400
FC = 512
HALO = 8
L = 128

CFG = dict(order='WAPBQOR', ssplit=6, qsplit=2, CP=40, cseg='B', cstart=1, cevery=1, lseg='A', lnp=5, lstart=0, levery=1,
           egn=1, egr=5, fseg='O', fin=3, nfin=3, fevery=4, rseg='R', rpos=0, TB=80)

_NT = (((1,), (1,)), ((), ()))
_F32 = jnp.float32
_BF16 = jnp.bfloat16
_U32 = jnp.uint32


def _cat(xs, axis=1):
    return jnp.concatenate(xs, axis=axis)


def _bf(x):
    return pltpu.bitcast(x, _BF16)


def _ln(x, scale=None):
    d = x.shape[-1]
    m = jnp.sum(x, axis=-1, keepdims=True) * (1.0 / d)
    xc = x - m
    v = jnp.sum(xc * xc, axis=-1, keepdims=True) * (1.0 / d)
    r = jax.lax.rsqrt(v + _EPS)
    if scale is not None:
        r = r * scale
    return xc * r


def _kernel(zero_ref, kbias,
            x_hbm, wa1_h, wb1_h, wq_h, wk_h, wv_h, wo_h, wp1_h, dw_h, wp2_h, wa2_h, wb2_h,
            o_hbm,
            wa1, wb1, wq, wk, wv, wo, wp1, dwv, wp2, wa2, wb2, wa0, wm, wvo,
            xall, x1, hh, g, dc, sbuf, hb, acc, qbuf, o16, h3b, rbuf, lbuf, dwf, tmean,
            wsem, xsem,
            *, B, T, D, K):
    N = B * T
    NT = N // R
    TPB = T // R
    TP = hh.shape[2]
    F = wb1.shape[0]
    NK = TP // L
    ND = D // L
    scale = D ** -0.5
    pad = K // 2
    cfg = CFG
    hh32 = hh.bitcast(_U32)

    def w_copy(src, dst, k):
        return pltpu.make_async_copy(src, dst, wsem.at[k])

    NF = F // FC
    CT = FC // L

    def up_copies(src, dst, c, k):
        return [pltpu.make_async_copy(src.at[:, pl.ds(n * L, L)], dst.at[n], wsem.at[k])
                for n in range(c * CT, (c + 1) * CT)]

    def down_copies(src, dst, c, k):
        return [pltpu.make_async_copy(src.at[pl.ds(c * FC, FC), :], dst.at[pl.ds(c * FC, FC), :], wsem.at[k])]

    c_wa0 = [w_copy(wa1_h.at[:, pl.ds(c * FC, FC)], wa0.at[:, pl.ds(c * FC, FC)], c) for c in range(NF)]
    c_wb1 = [down_copies(wb1_h, wb1, c, NF + c) for c in range(NF)]
    k0 = 2 * NF
    c_rest = [w_copy(src, dst, k0 + n) for n, (src, dst) in enumerate(
        [(wq_h, wq), (wk_h, wk), (wv_h, wv), (wo_h, wo), (dw_h, dwv), (wp2_h, wp2)])]
    c_rest += sum([up_copies(wp1_h, wp1, c, k0 + 6) for c in range(2 * ND // CT)], [])
    c_rest += sum([up_copies(wa2_h, wa2, c, k0 + 7) for c in range(NF)], [])
    c_rest += [w_copy(wb2_h, wb2, k0 + 8)]

    def rows(i):
        return i * R if isinstance(i, int) else pl.multiple_of(i * R, 16)

    def x_copy(i):
        return pltpu.make_async_copy(x_hbm.at[pl.ds(rows(i), R), :], xall.at[pl.ds(rows(i), R), :],
                                     xsem.at[i])

    def o_copy(i):
        return pltpu.make_async_copy(xall.at[pl.ds(rows(i), R), :], o_hbm.at[pl.ds(rows(i), R), :],
                                     xsem.at[i])

    def tile(i):
        if isinstance(i, int):
            return i // TPB, (i % TPB) * R
        b = i // TPB
        return b, pl.multiple_of((i - b * TPB) * R, 16)

    def ld_x(i):
        b, r0 = tile(i)
        return _cat([x1[b, n, pl.ds(r0, R), :] for n in range(ND)])

    def st_cols(ref, i, v):
        b, r0 = tile(i)
        for n in range(ND):
            ref[b, n, pl.ds(r0, R), :] = v[:, n * L:(n + 1) * L]

    x_copy(0).start()
    c_wa0[0].start()
    for c in range(NF):
        for w in c_wa0[c + 1:c + 2] + c_wb1[c]:
            w.start()
    x_copy(1).start()
    for t in range(2, NT):
        x_copy(t).start()
    for c in c_rest:
        c.start()

    for b in range(B):
        for n in range(ND):
            hh[b, n, T:TP, :] = jnp.zeros((TP - T, L), _BF16)
            g[b, n, 0:2 * HALO, :] = jnp.zeros((2 * HALO, L), _F32)
            g[b, n, 2 * HALO + T:, :] = jnp.zeros((2 * HALO, L), _F32)
        dc[b, 0:HALO, :] = jnp.zeros((HALO, D), _F32)

    def ff(wa, wb, mid=None, first=False, finish=None):
        hid = {}

        def up(c):
            if first and c < 3:
                for w in (c_wa0[:1], c_wa0[1:2] + c_wb1[0], c_wa0[2:] + c_wb1[1])[c]:
                    w.wait()
            w = wa0[:, c * FC:(c + 1) * FC] if first else _cat([wa[c * CT + n] for n in range(CT)])
            u = jnp.dot(hb[...], w, preferred_element_type=_F32)
            hid[c] = (u + u * jnp.tanh(u)).astype(_BF16)

        def down(c):
            if first and c == 2:
                for w in sum(c_wb1[2:], [x_copy(1)]):
                    w.wait()
            if first and c >= 1:
                cut = [(F // L) * q // (NF - 1) for q in range(NF)]
                for n in range(cut[c - 1], cut[c]):
                    wa1[n] = wa0[:, n * L:(n + 1) * L]
            w = wb[c * FC:(c + 1) * FC, :]
            if finish is not None and c == NF - 1:
                h = hid.pop(c)
                for lo in range(0, R, cfg['TB']):
                    hi = lo + cfg['TB']
                    d = jnp.dot(h[lo:hi], w, preferred_element_type=_F32)
                    finish(lo, hi, acc[lo:hi, :] + d)
                return
            d = jnp.dot(hid.pop(c), w, preferred_element_type=_F32)
            if c == 0:
                acc[...] = d
            else:
                acc[...] += d

        up(0)
        for c in range(NF):
            if c + 1 < NF:
                up(c + 1)
            if c == NF - 2 and mid is not None:
                mid()
            down(c)

    def ln1(i):
        hb[...] = _ln(xall[pl.ds(rows(i), R), :].astype(_F32), 0.5).astype(_BF16)

    def post_a(i):
        xr = xall[pl.ds(rows(i), R), :].astype(_F32) + 0.5 * acc[...]
        st_cols(x1, i, xr)
        st_cols(hh, i, _ln(xr).astype(_BF16))

    x_copy(0).wait()
    ln1(0)
    ff(wa1, wb1, first=True)
    ln1(1)

    def phase_a(i, carry):
        x_copy(i + 1).wait()
        post_a(i - 1)
        ff(wa1, wb1)
        ln1(i + 1)
        return carry

    jax.lax.fori_loop(1, NT - 1, phase_a, 0)
    for c in c_rest:
        c.wait()
    post_a(NT - 2)
    ff(wa1, wb1)
    for n in range(ND):
        wm[n] = (jax.lax.dot_general(wq[...], wk[n * L:(n + 1) * L, :], _NT,
                                     preferred_element_type=_F32)
                 * (scale * _LOG2E)).astype(_BF16)
        wvo[n] = jnp.dot(wv[...], wo[:, n * L:(n + 1) * L],
                         preferred_element_type=_F32).astype(_BF16)
    dwf[...] = dwv[...].astype(_F32)
    post_a(NT - 1)

    CP = cfg['CP']
    CW = R + HALO
    piece_rows = [(p * CP, CP) for p in range(R // CP)] + [(R, HALO)]

    def q_proj(i, lo=0, hi=ND, after_pass=lambda d: None):
        b, r0 = tile(i)
        r = r0 // 2 if isinstance(r0, int) else pl.multiple_of(r0 // 2, 8)
        h = _cat([_bf(hh32[b, j, pl.ds(r, R // 2), :]) for j in range(ND)])
        for n in range(lo, hi):
            d = jnp.dot(h, wm[n], preferred_element_type=_F32)
            qbuf[n] = d.astype(_BF16)
            after_pass(d)

    def step_b(i, stats, prev=True, conv=True, early=False):
        z0 = zero_ref[0]
        nz = [0]

        def fresh(ref):
            nz[0] += 1
            z = pl.multiple_of(z0 * nz[0], 8)
            r32 = ref.bitcast(_U32)
            return _cat([ref[j] for j in range(ND)])

        st = dict(psum=None, stats=stats)
        k = i - 1

        def edge_mask(w0, a):
            _, r0 = tile(k)
            n = a.shape[0]
            parts = [a]
            if w0 == 0:
                parts = [jnp.where(r0 > 0, a[:HALO], 0.0), a[HALO:]]
            if w0 + n > R:
                h = parts[-1]
                cut = h.shape[0] - HALO
                parts[-1:] = [h[:cut], jnp.where(r0 == T - R, h[cut:], 0.0)]
            parts = [q for q in parts if q.shape[0]]
            return parts[0] if len(parts) == 1 else _cat(parts, 0)

        def conv_piece(p):
            b, r0 = tile(k)
            w0, n = piece_rows[p]
            cols = []
            for j in range(ND):
                win = g[b, j, pl.ds(r0 + w0, n + 2 * HALO), :]
                a = None
                for t in range(K):
                    o = HALO - pad + t
                    v = win[o:o + n, :] * dwf[t:t + 1, j * L:(j + 1) * L]
                    a = v if a is None else a + v
                cols.append(a)
            a = _cat(cols)
            dc[b, pl.ds(r0 + w0, n), :] = a
            ps = jnp.sum(edge_mask(w0, a).reshape(n // 8, 8, D), axis=0)
            st['psum'] = ps if st['psum'] is None else st['psum'] + ps

        def conv_finish(part):
            b, r0 = tile(k)
            nparts = cfg['nfin']
            if part == 0:
                cnt = (R - HALO * jnp.asarray(r0 == 0, jnp.int32)
                       + HALO * jnp.asarray(r0 == T - R, jnp.int32)).astype(_F32)
                st['mu'] = jnp.sum(st['psum'], axis=0, keepdims=True) / cnt
                tmean[pl.ds(k, 1), :] = st['mu']
            lo = (CW // 8 * part // nparts) * 8
            hi = (CW // 8 * (part + 1) // nparts) * 8
            dd = dc[b, pl.ds(r0 + lo, hi - lo), :] - st['mu']
            m2 = jnp.sum(edge_mask(lo, dd * dd).reshape((hi - lo) // 8, 8, D), axis=0)
            s = st['stats']
            st['stats'] = (s[0] + st['psum'] if part == 0 else s[0], s[1] + m2)

        def ln3_part(part):
            b, r0 = tile(i - 1)
            rs = R // cfg['lnp']
            x2 = _cat([x1[b, n, pl.ds(pl.multiple_of(r0 + part * rs + z0, 8), rs), :]
                       for n in range(ND)])
            h = _ln(x2, 0.5).astype(_BF16)
            for n in range(ND):
                h3b[n, part * rs:(part + 1) * rs, :] = h[:, n * L:(n + 1) * L]

        def exp_chunk(c):
            ps = []
            for n in range(ND * c, ND * c + ND):
                p = jnp.exp2(sbuf[n] - st['m'])
                ps.append(p.astype(_BF16))
                st['l'] = p if n == 0 else st['l'] + p
            return _cat(ps)

        def gate_g(d):
            g[z0, 0, pl.ds(T + 3 * HALO, 8), :] = d[0:8, :]

        def gate_x(d):
            x1[z0, 0, pl.ds(T, 8), :] = d[0:8, :]

        def gate_s(d):
            r = cfg['egr'] * 8
            sbuf[z0 + NK, 0:8, :] = d[r:r + 8, :]

        def gate_l(d):
            lbuf[pl.ds(pl.multiple_of(R + z0, 8), 8), :] = d[0:8, :]

        def inv_l():
            rbuf[...] = jnp.broadcast_to(1.0 / jnp.sum(lbuf[0:R, :], axis=-1, keepdims=True), (R, L))

        def gate_dc(d):
            dc[z0, pl.ds(T + HALO, 8), 0:L] = d[0:8, :]

        order = cfg['order']
        size = dict(S=NK, A=cfg['ssplit'], B=NK - cfg['ssplit'], W=ND, O=NK, P=2 * ND,
                    Q=cfg['qsplit'], R=ND - cfg['qsplit'])
        start = {}
        for name in order:
            start[name] = sum(size[o] for o in order[:order.index(name)])
        jobs = {}

        def add(seg, t, gate, fn):
            jobs.setdefault(start[seg] + t, []).append((gate, fn))

        if conv:
            for p in range(len(piece_rows)):
                add(cfg['cseg'], cfg['cstart'] + p * cfg['cevery'], gate_g,
                    functools.partial(conv_piece, p))
            for p in range(cfg['nfin']):
                add(cfg['fseg'], cfg['fin'] + p * cfg['fevery'], gate_dc,
                    functools.partial(conv_finish, p))
        if cfg['rseg']:
            add(cfg['rseg'], cfg['rpos'], gate_l, inv_l)
        if prev:
            for p in range(cfg['lnp']):
                add(cfg['lseg'], cfg['lstart'] + p * cfg['levery'], gate_x,
                    functools.partial(ln3_part, p))

        def span(fn):
            at = [t for t, js in jobs.items() for _, j in js if getattr(j, 'func', j) is fn]
            return min(at), max(at)

        if prev:
            assert start['W'] + ND - 1 <= span(ln3_part)[0] and span(ln3_part)[1] < start['P']
        if conv:
            assert start['P'] + 2 * ND - 1 <= span(conv_piece)[0]
            assert span(conv_piece)[1] <= span(conv_finish)[0]
        assert start['O'] + NK - 1 <= span(inv_l)[0]

        def after_pass(t, d):
            for gate, fn in jobs.pop(t, []):
                gate(d)
                fn()

        b, _ = tile(i)

        def seg_s(lo, hi, t0):
            for n in range(lo, hi):
                keys = _cat([_bf(hh32[b, j, pl.ds(n * L // 2, L // 2), :]) for j in range(ND)])
                s = jax.lax.dot_general(fresh(qbuf), keys, _NT, preferred_element_type=_F32)
                if (n + 1) * L > T:
                    if early:
                        s = s + kbias[n - T // L]
                    else:
                        col = jax.lax.broadcasted_iota(jnp.int32, (1, L), 1) + n * L
                        s = jnp.where(col < T, s, -1e30)
                sbuf[n] = s
                st['mm'] = s if n == 0 else jnp.maximum(st['mm'], s)
                after_pass(t0 + n - lo, s)
            if hi == NK:
                st['m'] = jnp.max(st['mm'], axis=-1, keepdims=True)

        def seg_w(t0):
            b1, r1 = tile(i - 1)
            for n in range(ND):
                d = jnp.dot(fresh(o16), wvo[n], preferred_element_type=_F32)
                x1[b1, n, pl.ds(r1, R), :] += d * rbuf[...]
                after_pass(t0 + n, d)

        def seg_o(t0):
            NC = NK // ND
            p = exp_chunk(0)
            o = [None] * ND
            for c in range(NC):
                pn = None
                for n in range(ND):
                    v = _bf(hh32[b, n, pl.ds(c * ND * L // 2, ND * L // 2), :])
                    d = jnp.dot(p, v, preferred_element_type=_F32)
                    o[n] = d if c == 0 else o[n] + d
                    if c + 1 == NC:
                        o16[n] = o[n].astype(_BF16)
                    if n == cfg['egn'] and c + 1 < NC:
                        gate_s(d)
                        pn = exp_chunk(c + 1)
                    after_pass(t0 + c * ND + n, d)
                p = pn
            if cfg['rseg']:
                lbuf[0:R, :] = st['l']
            else:
                rbuf[...] = jnp.broadcast_to(1.0 / jnp.sum(st['l'], axis=-1, keepdims=True), (R, L))

        def seg_q(lo, hi, t0):
            cnt = [t0]

            def ap(d):
                after_pass(cnt[0], d)
                cnt[0] += 1
            q_proj(i + 1 if isinstance(i, int) else jnp.minimum(i + 1, NT - 1), lo, hi, ap)

        def seg_p(t0):
            b1, r1 = tile(i - 1)
            for n in range(ND):
                a = jnp.dot(fresh(h3b), wp1[n], preferred_element_type=_F32)
                after_pass(t0 + 2 * n, a)
                bb = jnp.dot(fresh(h3b), wp1[ND + n], preferred_element_type=_F32)
                g[b1, n, pl.ds(r1 + 2 * HALO, R), :] = a + a * jnp.tanh(bb)
                after_pass(t0 + 2 * n + 1, bb)

        segs = dict(S=(True, functools.partial(seg_s, 0, NK)),
                    A=(True, functools.partial(seg_s, 0, cfg['ssplit'])),
                    B=(True, functools.partial(seg_s, cfg['ssplit'], NK)), W=(prev, seg_w), O=(True, seg_o), Q=(True, functools.partial(seg_q, 0, cfg['qsplit'])),
                    R=(True, functools.partial(seg_q, cfg['qsplit'], ND)),
                    P=(prev, seg_p))
        for name in order:
            on, fn = segs[name]
            if on:
                fn(start[name])
            for t in range(start[name], start[name] + size[name]):
                for _, job in jobs.pop(t, []):
                    job()
        assert not jobs
        return st['stats']

    stats = (jnp.zeros((8, D), _F32), jnp.zeros((8, D), _F32))
    q_proj(0)
    stats = step_b(zero_ref[0], stats, prev=False, conv=False, early=True)
    stats = jax.lax.fori_loop(1, NT, step_b, stats)

    last = NT - 1
    b1, r1 = tile(last)
    RB = cfg['TB']
    blocks = [(lo, lo + RB) for lo in range(0, R, RB)]
    for lo, hi in blocks:
        o = _cat([o16[c, lo:hi, :] for c in range(ND)])
        for n in range(ND):
            d = jnp.dot(o, wvo[n], preferred_element_type=_F32)
            x1[b1, n, r1 + lo:r1 + hi, :] += d * rbuf[lo:hi, :]
    shift = tmean[last - 1:last, :]
    t1 = jnp.zeros((8, D), _F32)
    t2 = jnp.zeros((8, D), _F32)

    def conv_rows(lo, hi):
        c1, c2 = [], []
        for j in range(ND):
            a = None
            for t in range(K):
                v = (g[b1, j, r1 + lo + HALO - pad + t:r1 + hi + HALO - pad + t, :]
                     * dwf[t:t + 1, j * L:(j + 1) * L])
                a = v if a is None else a + v
            dc[b1, r1 + lo:r1 + hi, j * L:(j + 1) * L] = a
            dd = (a - shift[:, j * L:(j + 1) * L]).reshape((hi - lo) // 8, 8, L)
            c1.append(jnp.sum(dd, axis=0))
            c2.append(jnp.sum(dd * dd, axis=0))
        return _cat(c1), _cat(c2)

    for lo, hi in blocks:
        h = _ln(_cat([x1[b1, n, r1 + lo:r1 + hi, :] for n in range(ND)]), 0.5).astype(_BF16)
        for j in range(ND):
            a = jnp.dot(h, wp1[j], preferred_element_type=_F32)
            bb = jnp.dot(h, wp1[ND + j], preferred_element_type=_F32)
            g[b1, j, r1 + 2 * HALO + lo:r1 + 2 * HALO + hi, :] = a + a * jnp.tanh(bb)
        c1, c2 = conv_rows(lo, hi if hi < R else CW)
        t1, t2 = t1 + c1, t2 + c2
    t1 = jnp.sum(t1, axis=0, keepdims=True)
    t2 = jnp.sum(t2, axis=0, keepdims=True)
    tmean[last:NT, :] = shift + t1 * (1.0 / CW)

    trow = jax.lax.broadcasted_iota(jnp.int32, (NT, 1), 0) % TPB
    tcnt = (R - HALO * (trow == 0).astype(jnp.int32)
            + HALO * (trow == TPB - 1).astype(jnp.int32)).astype(_F32)
    mu = (jnp.sum(stats[0], axis=0, keepdims=True) + (t1 + CW * shift)) * (1.0 / N)
    dm = tmean[...] - mu
    var = (jnp.sum(stats[1], axis=0, keepdims=True) + (t2 - t1 * t1 * (1.0 / CW))
           + jnp.sum(dm * dm * tcnt, axis=0, keepdims=True)) * (1.0 / N)
    rstd = jax.lax.rsqrt(var + _EPS) * 0.5

    def pw2(i):
        b, r0 = tile(i)
        u = (dc[b, pl.ds(r0 + HALO, R), :] - mu) * rstd
        a = (u + u * jnp.tanh(u)).astype(_BF16)
        st_cols(x1, i, ld_x(i) + jnp.dot(a, wp2[...], preferred_element_type=_F32))

    def ln4(i):
        hb[...] = _ln(ld_x(i), 0.5).astype(_BF16)

    def post_d(i):
        xall[pl.ds(rows(i), R), :] = _ln(ld_x(i) + 0.5 * acc[...]).astype(_BF16)
        o_copy(i).start()

    pw2(0)
    pw2(1)
    ln4(0)
    ff(wa2, wb2)
    ln4(1)

    def phase_d(i, carry):
        post_d(i - 1)
        ff(wa2, wb2, mid=lambda: pw2(i + 1))
        ln4(i + 1)
        return carry

    jax.lax.fori_loop(1, NT - 1, phase_d, 0)
    post_d(NT - 2)
    bl, rl = tile(NT - 1)
    tails = []

    def leave(lo, hi, f):
        x4 = _cat([x1[bl, n, rl + lo:rl + hi, :] for n in range(ND)]) + 0.5 * f
        o0 = (NT - 1) * R + lo
        xall[o0:o0 + hi - lo, :] = _ln(x4).astype(_BF16)
        tails.append(pltpu.make_async_copy(xall.at[pl.ds(o0, hi - lo), :],
                                           o_hbm.at[pl.ds(o0, hi - lo), :], wsem.at[len(tails)]))
        tails[-1].start()

    ff(wa2, wb2, finish=leave)
    for t in range(NT - 1):
        o_copy(t).wait()
    for c in tails:
        c.wait()


@jax.jit
def pallas_standalone__conformer_family_conformer__speech_kernel(
    x: jax.Array,
    w_ff1_a: jax.Array,
    w_ff1_b: jax.Array,
    w_q: jax.Array,
    w_k: jax.Array,
    w_v: jax.Array,
    w_o: jax.Array,
    w_pw1: jax.Array,
    dw: jax.Array,
    w_pw2: jax.Array,
    w_ff2_a: jax.Array,
    w_ff2_b: jax.Array,
):
    B, T, D = x.shape
    K = dw.shape[0]
    N = B * T
    TP = -(-T // D) * D
    ND = D // L
    assert T % R == 0 and K // 2 <= HALO and K - 1 - K // 2 <= HALO and D % L == 0

    weights = (w_ff1_a, w_ff1_b, w_q, w_k, w_v, w_o, w_pw1, dw, w_pw2, w_ff2_a, w_ff2_b)
    V = pltpu.VMEM
    F = w_ff1_a.shape[1]
    tiled = lambda w: V((w.shape[1] // L, w.shape[0], L), w.dtype)
    scratch = [tiled(w_ff1_a), V(w_ff1_b.shape, w_ff1_b.dtype)] + [V(w.shape, w.dtype) for w in weights[2:6]]
    scratch += [tiled(w_pw1), V(dw.shape, dw.dtype), V(w_pw2.shape, w_pw2.dtype),
                tiled(w_ff2_a), V(w_ff2_b.shape, w_ff2_b.dtype)]
    scratch += [
        V(w_ff1_a.shape, w_ff1_a.dtype),
        V((ND, D, L), _BF16),
        V((ND, D, L), _BF16),
        V((N, D), x.dtype),
        V((B, ND, T + 8, L), _F32),
        V((B, ND, TP, L), _BF16),
        V((B, ND, T + 4 * HALO, L), _F32),
        V((B, T + 2 * HALO, D), _F32),
        V((TP // L + 1, R, L), _F32),
        V((R, D), _BF16),
        V((R, D), _F32),
        V((ND, R, L), _BF16),
        V((ND, R, L), _BF16),
        V((ND, R, L), _BF16),
        V((R, L), _F32),
        V((R + 8, L), _F32),
        V((K, D), _F32),
        V((N // R, D), _F32),
        pltpu.SemaphoreType.DMA((max(9 + 2 * (F // FC), R // CFG['TB']),)),
        pltpu.SemaphoreType.DMA((N // R,)),
    ]
    col = np.arange(T // L * L, TP).reshape(-1, 1, L)
    kbias = np.where(col < T, 0.0, -1e30).astype(np.float32)
    out = pl.pallas_call(
        functools.partial(_kernel, B=B, T=T, D=D, K=K),
        out_shape=jax.ShapeDtypeStruct((N, D), x.dtype),
        in_specs=([pl.BlockSpec(memory_space=pltpu.SMEM), pl.BlockSpec(memory_space=pltpu.VMEM)]
                  + [pl.BlockSpec(memory_space=pl.ANY)] * (1 + len(weights))),
        out_specs=pl.BlockSpec(memory_space=pl.ANY),
        scratch_shapes=scratch,
        compiler_params=pltpu.CompilerParams(
            vmem_limit_bytes=120 * 2**20,
            flags={"XLA_TPU_EVENLY_DISTRIBUTE_CRITICAL_NODES": True},
        ),
        name="conformer",
    )(np.zeros((1,), np.int32), kbias, x.reshape(N, D), *weights)
    return out.reshape(B, T, D)
```

```python
import functools

import jax
import jax.numpy as jnp
import numpy as np
import jax.experimental.pallas as pl
import jax.experimental.pallas.tpu as pltpu

_EPS = 1e-05
_LOG2E = 1.4426950408889634

R = 400
FC = 512
HALO = 8
L = 128

CFG = dict(
    order='WAPBQOR',
    ssplit=6,
    qsplit=2,
    CP=40, cseg='B', cstart=1, cevery=1,
    lnp=5, lseg='A', lstart=0, levery=1,
    nfin=3, fseg='O', fin=3, fevery=4,
    egn=1, egr=5,
    rseg='R', rpos=0,
    TB=80,
)

_NT = (((1,), (1,)), ((), ()))
_F32 = jnp.float32
_BF16 = jnp.bfloat16
_U32 = jnp.uint32


def _cat(xs, axis=1):
    return jnp.concatenate(xs, axis=axis)


def _bf(x):
    return pltpu.bitcast(x, _BF16)


def _ln(x, scale=None):
    d = x.shape[-1]
    m = jnp.sum(x, axis=-1, keepdims=True) * (1.0 / d)
    xc = x - m
    v = jnp.sum(xc * xc, axis=-1, keepdims=True) * (1.0 / d)
    r = jax.lax.rsqrt(v + _EPS)
    if scale is not None:
        r = r * scale
    return xc * r


def _kernel(zero_ref, kbias,
            x_hbm, wa1_h, wb1_h, wq_h, wk_h, wv_h, wo_h, wp1_h, dw_h, wp2_h, wa2_h, wb2_h,
            o_hbm,
            wa1, wb1, wq, wk, wv, wo, wp1, dwv, wp2, wa2, wb2, wa0, wm, wvo,
            xall, x1, hh, g, dc, sbuf, hb, acc, qbuf, o16, h3b, rbuf, lbuf, dwf, tmean,
            wsem, xsem,
            *, B, T, D, K):
    N = B * T
    NT = N // R
    TPB = T // R
    TP = hh.shape[2]
    F = wb1.shape[0]
    NK = TP // L
    ND = D // L
    scale = D ** -0.5
    pad = K // 2
    cfg = CFG
    hh32 = hh.bitcast(_U32)

    def w_copy(src, dst, k):
        return pltpu.make_async_copy(src, dst, wsem.at[k])

    NF = F // FC
    CT = FC // L

    def up_copies(src, dst, c, k):
        return [pltpu.make_async_copy(src.at[:, pl.ds(n * L, L)], dst.at[n], wsem.at[k])
                for n in range(c * CT, (c + 1) * CT)]

    def down_copies(src, dst, c, k):
        return [w_copy(src.at[pl.ds(c * FC, FC), :], dst.at[pl.ds(c * FC, FC), :], k)]

    c_wa0 = [w_copy(wa1_h.at[:, pl.ds(c * FC, FC)], wa0.at[:, pl.ds(c * FC, FC)], c) for c in range(NF)]
    c_wb1 = [down_copies(wb1_h, wb1, c, NF + c) for c in range(NF)]
    k0 = 2 * NF
    c_rest = [w_copy(src, dst, k0 + n) for n, (src, dst) in enumerate(
        [(wq_h, wq), (wk_h, wk), (wv_h, wv), (wo_h, wo), (dw_h, dwv), (wp2_h, wp2)])]
    c_rest += sum([up_copies(wp1_h, wp1, c, k0 + 6) for c in range(2 * ND // CT)], [])
    c_rest += sum([up_copies(wa2_h, wa2, c, k0 + 7) for c in range(NF)], [])
    c_rest += [w_copy(wb2_h, wb2, k0 + 8)]

    def rows(i):
        return i * R if isinstance(i, int) else pl.multiple_of(i * R, 16)

    def x_copy(i):
        return pltpu.make_async_copy(x_hbm.at[pl.ds(rows(i), R), :], xall.at[pl.ds(rows(i), R), :],
                                     xsem.at[i])

    def o_copy(i):
        return pltpu.make_async_copy(xall.at[pl.ds(rows(i), R), :], o_hbm.at[pl.ds(rows(i), R), :],
                                     xsem.at[i])

    def tile(i):
        if isinstance(i, int):
            return i // TPB, (i % TPB) * R
        b = i // TPB
        return b, pl.multiple_of((i - b * TPB) * R, 16)

    def ld_x(i):
        b, r0 = tile(i)
        return _cat([x1[b, n, pl.ds(r0, R), :] for n in range(ND)])

    def st_cols(ref, i, v):
        b, r0 = tile(i)
        for n in range(ND):
            ref[b, n, pl.ds(r0, R), :] = v[:, n * L:(n + 1) * L]

    x_copy(0).start()
    c_wa0[0].start()
    for c in range(NF):
        for w in c_wa0[c + 1:c + 2] + c_wb1[c]:
            w.start()
    for t in range(1, NT):
        x_copy(t).start()
    for c in c_rest:
        c.start()

    for b in range(B):
        for n in range(ND):
            hh[b, n, T:TP, :] = jnp.zeros((TP - T, L), _BF16)
            g[b, n, 0:2 * HALO, :] = jnp.zeros((2 * HALO, L), _F32)
            g[b, n, 2 * HALO + T:, :] = jnp.zeros((2 * HALO, L), _F32)
        dc[b, 0:HALO, :] = jnp.zeros((HALO, D), _F32)

    def ff(wa, wb, mid=None, first=False, finish=None):
        hid = {}

        def up(c):
            if first and c < 3:
                for w in (c_wa0[:1], c_wa0[1:2] + c_wb1[0], c_wa0[2:] + c_wb1[1])[c]:
                    w.wait()
            w = wa0[:, c * FC:(c + 1) * FC] if first else _cat([wa[c * CT + n] for n in range(CT)])
            u = jnp.dot(hb[...], w, preferred_element_type=_F32)
            hid[c] = (u + u * jnp.tanh(u)).astype(_BF16)

        def down(c):
            if first and c == 2:
                for w in sum(c_wb1[2:], [x_copy(1)]):
                    w.wait()
            if first and c >= 1:
                cut = [(F // L) * q // (NF - 1) for q in range(NF)]
                for n in range(cut[c - 1], cut[c]):
                    wa1[n] = wa0[:, n * L:(n + 1) * L]
            w = wb[c * FC:(c + 1) * FC, :]
            if finish is not None and c == NF - 1:
                h = hid.pop(c)
                for lo in range(0, R, cfg['TB']):
                    hi = lo + cfg['TB']
                    d = jnp.dot(h[lo:hi], w, preferred_element_type=_F32)
                    finish(lo, hi, acc[lo:hi, :] + d)
                return
            d = jnp.dot(hid.pop(c), w, preferred_element_type=_F32)
            if c == 0:
                acc[...] = d
            else:
                acc[...] += d

        up(0)
        for c in range(NF):
            if c + 1 < NF:
                up(c + 1)
            if c == NF - 2 and mid is not None:
                mid()
            down(c)

    def ln1(i):
        hb[...] = _ln(xall[pl.ds(rows(i), R), :].astype(_F32), 0.5).astype(_BF16)

    def post_a(i):
        xr = xall[pl.ds(rows(i), R), :].astype(_F32) + 0.5 * acc[...]
        st_cols(x1, i, xr)
        st_cols(hh, i, _ln(xr).astype(_BF16))

    x_copy(0).wait()
    ln1(0)
    ff(wa1, wb1, first=True)
    ln1(1)

    def phase_a(i, carry):
        x_copy(i + 1).wait()
        post_a(i - 1)
        ff(wa1, wb1)
        ln1(i + 1)
        return carry

    jax.lax.fori_loop(1, NT - 1, phase_a, 0)
    for c in c_rest:
        c.wait()
    post_a(NT - 2)
    ff(wa1, wb1)
    for n in range(ND):
        wm[n] = (jax.lax.dot_general(wq[...], wk[n * L:(n + 1) * L, :], _NT,
                                     preferred_element_type=_F32)
                 * (scale * _LOG2E)).astype(_BF16)
        wvo[n] = jnp.dot(wv[...], wo[:, n * L:(n + 1) * L],
                         preferred_element_type=_F32).astype(_BF16)
    dwf[...] = dwv[...].astype(_F32)
    post_a(NT - 1)

    CP = cfg['CP']
    CW = R + HALO
    piece_rows = [(p * CP, CP) for p in range(R // CP)] + [(R, HALO)]

    def q_proj(i, lo=0, hi=ND, after_pass=lambda d: None):
        b, r0 = tile(i)
        r = r0 // 2 if isinstance(r0, int) else pl.multiple_of(r0 // 2, 8)
        h = _cat([_bf(hh32[b, j, pl.ds(r, R // 2), :]) for j in range(ND)])
        for n in range(lo, hi):
            d = jnp.dot(h, wm[n], preferred_element_type=_F32)
            qbuf[n] = d.astype(_BF16)
            after_pass(d)

    def step_b(i, stats, prev=True, conv=True, early=False):
        z0 = zero_ref[0]

        def operand(ref):
            return _cat([ref[j] for j in range(ND)])

        st = dict(psum=None, stats=stats)
        k = i - 1

        def edge_mask(w0, a):
            _, r0 = tile(k)
            n = a.shape[0]
            parts = [a]
            if w0 == 0:
                parts = [jnp.where(r0 > 0, a[:HALO], 0.0), a[HALO:]]
            if w0 + n > R:
                h = parts[-1]
                cut = h.shape[0] - HALO
                parts[-1:] = [h[:cut], jnp.where(r0 == T - R, h[cut:], 0.0)]
            parts = [q for q in parts if q.shape[0]]
            return parts[0] if len(parts) == 1 else _cat(parts, 0)

        def conv_piece(p):
            b, r0 = tile(k)
            w0, n = piece_rows[p]
            cols = []
            for j in range(ND):
                win = g[b, j, pl.ds(r0 + w0, n + 2 * HALO), :]
                a = None
                for t in range(K):
                    o = HALO - pad + t
                    v = win[o:o + n, :] * dwf[t:t + 1, j * L:(j + 1) * L]
                    a = v if a is None else a + v
                cols.append(a)
            a = _cat(cols)
            dc[b, pl.ds(r0 + w0, n), :] = a
            ps = jnp.sum(edge_mask(w0, a).reshape(n // 8, 8, D), axis=0)
            st['psum'] = ps if st['psum'] is None else st['psum'] + ps

        def conv_finish(part):
            b, r0 = tile(k)
            nparts = cfg['nfin']
            if part == 0:
                cnt = (R - HALO * jnp.asarray(r0 == 0, jnp.int32)
                       + HALO * jnp.asarray(r0 == T - R, jnp.int32)).astype(_F32)
                st['mu'] = jnp.sum(st['psum'], axis=0, keepdims=True) / cnt
                tmean[pl.ds(k, 1), :] = st['mu']
            lo = (CW // 8 * part // nparts) * 8
            hi = (CW // 8 * (part + 1) // nparts) * 8
            dd = dc[b, pl.ds(r0 + lo, hi - lo), :] - st['mu']
            m2 = jnp.sum(edge_mask(lo, dd * dd).reshape((hi - lo) // 8, 8, D), axis=0)
            s = st['stats']
            st['stats'] = (s[0] + st['psum'] if part == 0 else s[0], s[1] + m2)

        def ln3_part(part):
            b, r0 = tile(i - 1)
            rs = R // cfg['lnp']
            x2 = _cat([x1[b, n, pl.ds(pl.multiple_of(r0 + part * rs + z0, 8), rs), :]
                       for n in range(ND)])
            h = _ln(x2, 0.5).astype(_BF16)
            for n in range(ND):
                h3b[n, part * rs:(part + 1) * rs, :] = h[:, n * L:(n + 1) * L]

        def exp_chunk(c):
            ps = []
            for n in range(ND * c, ND * c + ND):
                p = jnp.exp2(sbuf[n] - st['m'])
                ps.append(p.astype(_BF16))
                st['l'] = p if n == 0 else st['l'] + p
            return _cat(ps)

        def gate_g(d):
            g[z0, 0, pl.ds(T + 3 * HALO, 8), :] = d[0:8, :]

        def gate_x(d):
            x1[z0, 0, pl.ds(T, 8), :] = d[0:8, :]

        def gate_s(d):
            r = cfg['egr'] * 8
            sbuf[z0 + NK, 0:8, :] = d[r:r + 8, :]

        def gate_l(d):
            lbuf[pl.ds(pl.multiple_of(R + z0, 8), 8), :] = d[0:8, :]

        def inv_l():
            rbuf[...] = jnp.broadcast_to(1.0 / jnp.sum(lbuf[0:R, :], axis=-1, keepdims=True), (R, L))

        def gate_dc(d):
            dc[z0, pl.ds(T + HALO, 8), 0:L] = d[0:8, :]

        order = cfg['order']
        size = dict(A=cfg['ssplit'], B=NK - cfg['ssplit'], W=ND, O=NK, P=2 * ND,
                    Q=cfg['qsplit'], R=ND - cfg['qsplit'])
        start = {}
        for name in order:
            start[name] = sum(size[o] for o in order[:order.index(name)])
        jobs = {}

        def add(seg, t, gate, fn):
            jobs.setdefault(start[seg] + t, []).append((gate, fn))

        if conv:
            for p in range(len(piece_rows)):
                add(cfg['cseg'], cfg['cstart'] + p * cfg['cevery'], gate_g,
                    functools.partial(conv_piece, p))
            for p in range(cfg['nfin']):
                add(cfg['fseg'], cfg['fin'] + p * cfg['fevery'], gate_dc,
                    functools.partial(conv_finish, p))
        add(cfg['rseg'], cfg['rpos'], gate_l, inv_l)
        if prev:
            for p in range(cfg['lnp']):
                add(cfg['lseg'], cfg['lstart'] + p * cfg['levery'], gate_x,
                    functools.partial(ln3_part, p))

        def span(fn):
            at = [t for t, js in jobs.items() for _, j in js if getattr(j, 'func', j) is fn]
            return min(at), max(at)

        if prev:
            assert start['W'] + ND - 1 <= span(ln3_part)[0] and span(ln3_part)[1] < start['P']
        if conv:
            assert start['P'] + 2 * ND - 1 <= span(conv_piece)[0]
            assert span(conv_piece)[1] <= span(conv_finish)[0]
        assert start['O'] + NK - 1 <= span(inv_l)[0]

        def after_pass(t, d):
            for gate, fn in jobs.pop(t, []):
                gate(d)
                fn()

        b, _ = tile(i)

        def seg_s(lo, hi, t0):
            for n in range(lo, hi):
                keys = _cat([_bf(hh32[b, j, pl.ds(n * L // 2, L // 2), :]) for j in range(ND)])
                s = jax.lax.dot_general(operand(qbuf), keys, _NT, preferred_element_type=_F32)
                if (n + 1) * L > T:
                    if early:
                        s = s + kbias[n - T // L]
                    else:
                        col = jax.lax.broadcasted_iota(jnp.int32, (1, L), 1) + n * L
                        s = jnp.where(col < T, s, -1e30)
                sbuf[n] = s
                st['mm'] = s if n == 0 else jnp.maximum(st['mm'], s)
                after_pass(t0 + n - lo, s)
            if hi == NK:
                st['m'] = jnp.max(st['mm'], axis=-1, keepdims=True)

        def seg_w(t0):
            b1, r1 = tile(i - 1)
            for n in range(ND):
                d = jnp.dot(operand(o16), wvo[n], preferred_element_type=_F32)
                x1[b1, n, pl.ds(r1, R), :] += d * rbuf[...]
                after_pass(t0 + n, d)

        def seg_o(t0):
            NC = NK // ND
            p = exp_chunk(0)
            o = [None] * ND
            for c in range(NC):
                pn = None
                for n in range(ND):
                    v = _bf(hh32[b, n, pl.ds(c * ND * L // 2, ND * L // 2), :])
                    d = jnp.dot(p, v, preferred_element_type=_F32)
                    o[n] = d if c == 0 else o[n] + d
                    if c + 1 == NC:
                        o16[n] = o[n].astype(_BF16)
                    if n == cfg['egn'] and c + 1 < NC:
                        gate_s(d)
                        pn = exp_chunk(c + 1)
                    after_pass(t0 + c * ND + n, d)
                p = pn
            lbuf[0:R, :] = st['l']

        def seg_q(lo, hi, t0):
            cnt = [t0]

            def ap(d):
                after_pass(cnt[0], d)
                cnt[0] += 1
            q_proj(i + 1 if isinstance(i, int) else jnp.minimum(i + 1, NT - 1), lo, hi, ap)

        def seg_p(t0):
            b1, r1 = tile(i - 1)
            for n in range(ND):
                a = jnp.dot(operand(h3b), wp1[n], preferred_element_type=_F32)
                after_pass(t0 + 2 * n, a)
                bb = jnp.dot(operand(h3b), wp1[ND + n], preferred_element_type=_F32)
                g[b1, n, pl.ds(r1 + 2 * HALO, R), :] = a + a * jnp.tanh(bb)
                after_pass(t0 + 2 * n + 1, bb)

        segs = dict(A=(True, functools.partial(seg_s, 0, cfg['ssplit'])),
                    B=(True, functools.partial(seg_s, cfg['ssplit'], NK)),
                    Q=(True, functools.partial(seg_q, 0, cfg['qsplit'])),
                    R=(True, functools.partial(seg_q, cfg['qsplit'], ND)),
                    O=(True, seg_o), W=(prev, seg_w), P=(prev, seg_p))
        for name in order:
            on, fn = segs[name]
            if on:
                fn(start[name])
            for t in range(start[name], start[name] + size[name]):
                for _, job in jobs.pop(t, []):
                    job()
        assert not jobs
        return st['stats']

    stats = (jnp.zeros((8, D), _F32), jnp.zeros((8, D), _F32))
    q_proj(0)
    stats = step_b(zero_ref[0], stats, prev=False, conv=False, early=True)
    stats = jax.lax.fori_loop(1, NT, step_b, stats)

    last = NT - 1
    b1, r1 = tile(last)
    RB = cfg['TB']
    blocks = [(lo, lo + RB) for lo in range(0, R, RB)]
    for lo, hi in blocks:
        o = _cat([o16[c, lo:hi, :] for c in range(ND)])
        for n in range(ND):
            d = jnp.dot(o, wvo[n], preferred_element_type=_F32)
            x1[b1, n, r1 + lo:r1 + hi, :] += d * rbuf[lo:hi, :]
    shift = tmean[last - 1:last, :]
    t1 = jnp.zeros((8, D), _F32)
    t2 = jnp.zeros((8, D), _F32)

    def conv_rows(lo, hi):
        c1, c2 = [], []
        for j in range(ND):
            a = None
            for t in range(K):
                v = (g[b1, j, r1 + lo + HALO - pad + t:r1 + hi + HALO - pad + t, :]
                     * dwf[t:t + 1, j * L:(j + 1) * L])
                a = v if a is None else a + v
            dc[b1, r1 + lo:r1 + hi, j * L:(j + 1) * L] = a
            dd = (a - shift[:, j * L:(j + 1) * L]).reshape((hi - lo) // 8, 8, L)
            c1.append(jnp.sum(dd, axis=0))
            c2.append(jnp.sum(dd * dd, axis=0))
        return _cat(c1), _cat(c2)

    for lo, hi in blocks:
        h = _ln(_cat([x1[b1, n, r1 + lo:r1 + hi, :] for n in range(ND)]), 0.5).astype(_BF16)
        for j in range(ND):
            a = jnp.dot(h, wp1[j], preferred_element_type=_F32)
            bb = jnp.dot(h, wp1[ND + j], preferred_element_type=_F32)
            g[b1, j, r1 + 2 * HALO + lo:r1 + 2 * HALO + hi, :] = a + a * jnp.tanh(bb)
        c1, c2 = conv_rows(lo, hi if hi < R else CW)
        t1, t2 = t1 + c1, t2 + c2
    t1 = jnp.sum(t1, axis=0, keepdims=True)
    t2 = jnp.sum(t2, axis=0, keepdims=True)
    tmean[last:NT, :] = shift + t1 * (1.0 / CW)

    trow = jax.lax.broadcasted_iota(jnp.int32, (NT, 1), 0) % TPB
    tcnt = (R - HALO * (trow == 0).astype(jnp.int32)
            + HALO * (trow == TPB - 1).astype(jnp.int32)).astype(_F32)
    mu = (jnp.sum(stats[0], axis=0, keepdims=True) + (t1 + CW * shift)) * (1.0 / N)
    dm = tmean[...] - mu
    var = (jnp.sum(stats[1], axis=0, keepdims=True) + (t2 - t1 * t1 * (1.0 / CW))
           + jnp.sum(dm * dm * tcnt, axis=0, keepdims=True)) * (1.0 / N)
    rstd = jax.lax.rsqrt(var + _EPS) * 0.5

    def pw2(i):
        b, r0 = tile(i)
        u = (dc[b, pl.ds(r0 + HALO, R), :] - mu) * rstd
        a = (u + u * jnp.tanh(u)).astype(_BF16)
        st_cols(x1, i, ld_x(i) + jnp.dot(a, wp2[...], preferred_element_type=_F32))

    def ln4(i):
        hb[...] = _ln(ld_x(i), 0.5).astype(_BF16)

    def post_d(i):
        xall[pl.ds(rows(i), R), :] = _ln(ld_x(i) + 0.5 * acc[...]).astype(_BF16)
        o_copy(i).start()

    pw2(0)
    pw2(1)
    ln4(0)
    ff(wa2, wb2)
    ln4(1)

    def phase_d(i, carry):
        post_d(i - 1)
        ff(wa2, wb2, mid=lambda: pw2(i + 1))
        ln4(i + 1)
        return carry

    jax.lax.fori_loop(1, NT - 1, phase_d, 0)
    post_d(NT - 2)
    bl, rl = tile(NT - 1)
    tails = []

    def leave(lo, hi, f):
        x4 = _cat([x1[bl, n, rl + lo:rl + hi, :] for n in range(ND)]) + 0.5 * f
        o0 = (NT - 1) * R + lo
        xall[o0:o0 + hi - lo, :] = _ln(x4).astype(_BF16)
        tails.append(pltpu.make_async_copy(xall.at[pl.ds(o0, hi - lo), :],
                                           o_hbm.at[pl.ds(o0, hi - lo), :], wsem.at[len(tails)]))
        tails[-1].start()

    ff(wa2, wb2, finish=leave)
    for t in range(NT - 1):
        o_copy(t).wait()
    for c in tails:
        c.wait()


@jax.jit
def pallas_standalone__conformer_family_conformer__speech_kernel(
    x: jax.Array,
    w_ff1_a: jax.Array,
    w_ff1_b: jax.Array,
    w_q: jax.Array,
    w_k: jax.Array,
    w_v: jax.Array,
    w_o: jax.Array,
    w_pw1: jax.Array,
    dw: jax.Array,
    w_pw2: jax.Array,
    w_ff2_a: jax.Array,
    w_ff2_b: jax.Array,
):
    B, T, D = x.shape
    K = dw.shape[0]
    N = B * T
    TP = -(-T // D) * D
    ND = D // L
    assert T % R == 0 and K // 2 <= HALO and K - 1 - K // 2 <= HALO and D % L == 0

    weights = (w_ff1_a, w_ff1_b, w_q, w_k, w_v, w_o, w_pw1, dw, w_pw2, w_ff2_a, w_ff2_b)
    V = pltpu.VMEM
    F = w_ff1_a.shape[1]
    tiled = lambda w: V((w.shape[1] // L, w.shape[0], L), w.dtype)
    scratch = [tiled(w_ff1_a), V(w_ff1_b.shape, w_ff1_b.dtype)] + [V(w.shape, w.dtype) for w in weights[2:6]]
    scratch += [tiled(w_pw1), V(dw.shape, dw.dtype), V(w_pw2.shape, w_pw2.dtype),
                tiled(w_ff2_a), V(w_ff2_b.shape, w_ff2_b.dtype)]
    scratch += [
        V(w_ff1_a.shape, w_ff1_a.dtype),
        V((ND, D, L), _BF16),
        V((ND, D, L), _BF16),
        V((N, D), x.dtype),
        V((B, ND, T + 8, L), _F32),
        V((B, ND, TP, L), _BF16),
        V((B, ND, T + 4 * HALO, L), _F32),
        V((B, T + 2 * HALO, D), _F32),
        V((TP // L + 1, R, L), _F32),
        V((R, D), _BF16),
        V((R, D), _F32),
        V((ND, R, L), _BF16),
        V((ND, R, L), _BF16),
        V((ND, R, L), _BF16),
        V((R, L), _F32),
        V((R + 8, L), _F32),
        V((K, D), _F32),
        V((N // R, D), _F32),
        pltpu.SemaphoreType.DMA((max(9 + 2 * (F // FC), R // CFG['TB']),)),
        pltpu.SemaphoreType.DMA((N // R,)),
    ]
    col = np.arange(T // L * L, TP).reshape(-1, 1, L)
    kbias = np.where(col < T, 0.0, -1e30).astype(np.float32)
    out = pl.pallas_call(
        functools.partial(_kernel, B=B, T=T, D=D, K=K),
        out_shape=jax.ShapeDtypeStruct((N, D), x.dtype),
        in_specs=([pl.BlockSpec(memory_space=pltpu.SMEM), pl.BlockSpec(memory_space=pltpu.VMEM)]
                  + [pl.BlockSpec(memory_space=pl.ANY)] * (1 + len(weights))),
        out_specs=pl.BlockSpec(memory_space=pl.ANY),
        scratch_shapes=scratch,
        compiler_params=pltpu.CompilerParams(
            vmem_limit_bytes=120 * 2**20,
            flags={"XLA_TPU_EVENLY_DISTRIBUTE_CRITICAL_NODES": True},
        ),
        name="conformer",
    )(np.zeros((1,), np.int32), kbias, x.reshape(N, D), *weights)
    return out.reshape(B, T, D)
```

```python
import functools

import jax
import jax.numpy as jnp
import numpy as np
import jax.experimental.pallas as pl
import jax.experimental.pallas.tpu as pltpu

_EPS = 1e-05
_LOG2E = 1.4426950408889634

R = 400
FC = 512
HALO = 8
L = 128

CFG = dict(
    order='WAPBQOR',
    ssplit=6,
    qsplit=2,
    CP=40, cseg='B', cstart=1, cevery=1,
    lnp=5, lseg='A', lstart=0, levery=1,
    nfin=3, fseg='O', fin=3, fevery=4,
    egn=1, egr=5,
    rseg='R', rpos=0,
    ahead=1,
    TB=80,
)

_NT = (((1,), (1,)), ((), ()))
_F32 = jnp.float32
_BF16 = jnp.bfloat16
_U32 = jnp.uint32


def _cat(xs, axis=1):
    return jnp.concatenate(xs, axis=axis)


def _bf(x):
    return pltpu.bitcast(x, _BF16)


def _ln(x, scale=None):
    d = x.shape[-1]
    m = jnp.sum(x, axis=-1, keepdims=True) * (1.0 / d)
    xc = x - m
    v = jnp.sum(xc * xc, axis=-1, keepdims=True) * (1.0 / d)
    r = jax.lax.rsqrt(v + _EPS)
    if scale is not None:
        r = r * scale
    return xc * r


def _kernel(zero_ref, kbias,
            x_hbm, wa1_h, wb1_h, wq_h, wk_h, wv_h, wo_h, wp1_h, dw_h, wp2_h, wa2_h, wb2_h,
            o_hbm,
            wa1, wb1, wq, wk, wv, wo, wp1, dwv, wp2, wa2, wb2, wa0, wm, wvo,
            xall, x1, hh, g, dc, sbuf, hb, acc, qbuf, o16, h3b, rbuf, lbuf, dwf, tmean,
            wsem, xsem,
            *, B, T, D, K):
    N = B * T
    NT = N // R
    TPB = T // R
    TP = hh.shape[2]
    F = wb1.shape[0]
    NK = TP // L
    ND = D // L
    scale = D ** -0.5
    pad = K // 2
    cfg = CFG
    hh32 = hh.bitcast(_U32)

    def w_copy(src, dst, k):
        return pltpu.make_async_copy(src, dst, wsem.at[k])

    NF = F // FC
    CT = FC // L

    def up_copies(src, dst, c, k):
        return [pltpu.make_async_copy(src.at[:, pl.ds(n * L, L)], dst.at[n], wsem.at[k])
                for n in range(c * CT, (c + 1) * CT)]

    def down_copies(src, dst, c, k):
        return [w_copy(src.at[pl.ds(c * FC, FC), :], dst.at[pl.ds(c * FC, FC), :], k)]

    c_wa0 = [w_copy(wa1_h.at[:, pl.ds(c * FC, FC)], wa0.at[:, pl.ds(c * FC, FC)], c) for c in range(NF)]
    c_wb1 = [down_copies(wb1_h, wb1, c, NF + c) for c in range(NF)]
    k0 = 2 * NF
    c_rest = [w_copy(src, dst, k0 + n) for n, (src, dst) in enumerate(
        [(wq_h, wq), (wk_h, wk), (wv_h, wv), (wo_h, wo), (dw_h, dwv), (wp2_h, wp2)])]
    c_rest += sum([up_copies(wp1_h, wp1, c, k0 + 6) for c in range(2 * ND // CT)], [])
    c_rest += sum([up_copies(wa2_h, wa2, c, k0 + 7) for c in range(NF)], [])
    c_rest += [w_copy(wb2_h, wb2, k0 + 8)]

    def rows(i):
        return i * R if isinstance(i, int) else pl.multiple_of(i * R, 16)

    def x_copy(i):
        return pltpu.make_async_copy(x_hbm.at[pl.ds(rows(i), R), :], xall.at[pl.ds(rows(i), R), :],
                                     xsem.at[i])

    def o_copy(i):
        return pltpu.make_async_copy(xall.at[pl.ds(rows(i), R), :], o_hbm.at[pl.ds(rows(i), R), :],
                                     xsem.at[i])

    def tile(i):
        if isinstance(i, int):
            return i // TPB, (i % TPB) * R
        b = i // TPB
        return b, pl.multiple_of((i - b * TPB) * R, 16)

    def ld_x(i):
        b, r0 = tile(i)
        return _cat([x1[b, n, pl.ds(r0, R), :] for n in range(ND)])

    def st_cols(ref, i, v):
        b, r0 = tile(i)
        for n in range(ND):
            ref[b, n, pl.ds(r0, R), :] = v[:, n * L:(n + 1) * L]

    groups = [c_wa0[:1], c_wa0[1:2] + c_wb1[0], c_wa0[2:] + c_wb1[1],
              sum(c_wb1[2:], [x_copy(1)]), [x_copy(t) for t in range(2, NT)] + c_rest]
    AH = cfg['ahead']

    def arrive(k):
        for w in groups[k]:
            w.wait()
        for w in sum(groups[k + AH:k + AH + 1], []):
            w.start()

    x_copy(0).start()
    for w in sum(groups[:AH], []):
        w.start()

    for b in range(B):
        for n in range(ND):
            hh[b, n, T:TP, :] = jnp.zeros((TP - T, L), _BF16)
            g[b, n, 0:2 * HALO, :] = jnp.zeros((2 * HALO, L), _F32)
            g[b, n, 2 * HALO + T:, :] = jnp.zeros((2 * HALO, L), _F32)
        dc[b, 0:HALO, :] = jnp.zeros((HALO, D), _F32)

    def ff(wa, wb, mid=None, first=False, finish=None):
        hid = {}

        def up(c):
            if first and c < 3:
                arrive(c)
            w = wa0[:, c * FC:(c + 1) * FC] if first else _cat([wa[c * CT + n] for n in range(CT)])
            u = jnp.dot(hb[...], w, preferred_element_type=_F32)
            hid[c] = (u + u * jnp.tanh(u)).astype(_BF16)

        def down(c):
            if first and c == 2:
                arrive(3)
            if first and c >= 1:
                cut = [(F // L) * q // (NF - 1) for q in range(NF)]
                for n in range(cut[c - 1], cut[c]):
                    wa1[n] = wa0[:, n * L:(n + 1) * L]
            w = wb[c * FC:(c + 1) * FC, :]
            if finish is not None and c == NF - 1:
                h = hid.pop(c)
                for lo in range(0, R, cfg['TB']):
                    hi = lo + cfg['TB']
                    d = jnp.dot(h[lo:hi], w, preferred_element_type=_F32)
                    finish(lo, hi, acc[lo:hi, :] + d)
                return
            d = jnp.dot(hid.pop(c), w, preferred_element_type=_F32)
            if c == 0:
                acc[...] = d
            else:
                acc[...] += d

        up(0)
        for c in range(NF):
            if c + 1 < NF:
                up(c + 1)
            if c == NF - 2 and mid is not None:
                mid()
            down(c)

    def ln1(i):
        hb[...] = _ln(xall[pl.ds(rows(i), R), :].astype(_F32), 0.5).astype(_BF16)

    def post_a(i):
        xr = xall[pl.ds(rows(i), R), :].astype(_F32) + 0.5 * acc[...]
        st_cols(x1, i, xr)
        st_cols(hh, i, _ln(xr).astype(_BF16))

    x_copy(0).wait()
    ln1(0)
    ff(wa1, wb1, first=True)
    ln1(1)

    def phase_a(i, carry):
        x_copy(i + 1).wait()
        post_a(i - 1)
        ff(wa1, wb1)
        ln1(i + 1)
        return carry

    jax.lax.fori_loop(1, NT - 1, phase_a, 0)
    for c in c_rest:
        c.wait()
    post_a(NT - 2)
    ff(wa1, wb1)
    for n in range(ND):
        wm[n] = (jax.lax.dot_general(wq[...], wk[n * L:(n + 1) * L, :], _NT,
                                     preferred_element_type=_F32)
                 * (scale * _LOG2E)).astype(_BF16)
        wvo[n] = jnp.dot(wv[...], wo[:, n * L:(n + 1) * L],
                         preferred_element_type=_F32).astype(_BF16)
    dwf[...] = dwv[...].astype(_F32)
    post_a(NT - 1)

    CP = cfg['CP']
    CW = R + HALO
    piece_rows = [(p * CP, CP) for p in range(R // CP)] + [(R, HALO)]

    def q_proj(i, lo=0, hi=ND, after_pass=lambda d: None):
        b, r0 = tile(i)
        r = r0 // 2 if isinstance(r0, int) else pl.multiple_of(r0 // 2, 8)
        h = _cat([_bf(hh32[b, j, pl.ds(r, R // 2), :]) for j in range(ND)])
        for n in range(lo, hi):
            d = jnp.dot(h, wm[n], preferred_element_type=_F32)
            qbuf[n] = d.astype(_BF16)
            after_pass(d)

    def step_b(i, stats, prev=True, conv=True, early=False):
        z0 = zero_ref[0]

        def operand(ref):
            return _cat([ref[j] for j in range(ND)])

        st = dict(psum=None, stats=stats)
        k = i - 1

        def edge_mask(w0, a):
            _, r0 = tile(k)
            n = a.shape[0]
            parts = [a]
            if w0 == 0:
                parts = [jnp.where(r0 > 0, a[:HALO], 0.0), a[HALO:]]
            if w0 + n > R:
                h = parts[-1]
                cut = h.shape[0] - HALO
                parts[-1:] = [h[:cut], jnp.where(r0 == T - R, h[cut:], 0.0)]
            parts = [q for q in parts if q.shape[0]]
            return parts[0] if len(parts) == 1 else _cat(parts, 0)

        def conv_piece(p):
            b, r0 = tile(k)
            w0, n = piece_rows[p]
            cols = []
            for j in range(ND):
                win = g[b, j, pl.ds(r0 + w0, n + 2 * HALO), :]
                a = None
                for t in range(K):
                    o = HALO - pad + t
                    v = win[o:o + n, :] * dwf[t:t + 1, j * L:(j + 1) * L]
                    a = v if a is None else a + v
                cols.append(a)
            a = _cat(cols)
            dc[b, pl.ds(r0 + w0, n), :] = a
            ps = jnp.sum(edge_mask(w0, a).reshape(n // 8, 8, D), axis=0)
            st['psum'] = ps if st['psum'] is None else st['psum'] + ps

        def conv_finish(part):
            b, r0 = tile(k)
            nparts = cfg['nfin']
            if part == 0:
                cnt = (R - HALO * jnp.asarray(r0 == 0, jnp.int32)
                       + HALO * jnp.asarray(r0 == T - R, jnp.int32)).astype(_F32)
                st['mu'] = jnp.sum(st['psum'], axis=0, keepdims=True) / cnt
                tmean[pl.ds(k, 1), :] = st['mu']
            lo = (CW // 8 * part // nparts) * 8
            hi = (CW // 8 * (part + 1) // nparts) * 8
            dd = dc[b, pl.ds(r0 + lo, hi - lo), :] - st['mu']
            m2 = jnp.sum(edge_mask(lo, dd * dd).reshape((hi - lo) // 8, 8, D), axis=0)
            s = st['stats']
            st['stats'] = (s[0] + st['psum'] if part == 0 else s[0], s[1] + m2)

        def ln3_part(part):
            b, r0 = tile(i - 1)
            rs = R // cfg['lnp']
            x2 = _cat([x1[b, n, pl.ds(pl.multiple_of(r0 + part * rs + z0, 8), rs), :]
                       for n in range(ND)])
            h = _ln(x2, 0.5).astype(_BF16)
            for n in range(ND):
                h3b[n, part * rs:(part + 1) * rs, :] = h[:, n * L:(n + 1) * L]

        def exp_chunk(c):
            ps = []
            for n in range(ND * c, ND * c + ND):
                p = jnp.exp2(sbuf[n] - st['m'])
                ps.append(p.astype(_BF16))
                st['l'] = p if n == 0 else st['l'] + p
            return _cat(ps)

        def gate_g(d):
            g[z0, 0, pl.ds(T + 3 * HALO, 8), :] = d[0:8, :]

        def gate_x(d):
            x1[z0, 0, pl.ds(T, 8), :] = d[0:8, :]

        def gate_s(d):
            r = cfg['egr'] * 8
            sbuf[z0 + NK, 0:8, :] = d[r:r + 8, :]

        def gate_l(d):
            lbuf[pl.ds(pl.multiple_of(R + z0, 8), 8), :] = d[0:8, :]

        def inv_l():
            rbuf[...] = jnp.broadcast_to(1.0 / jnp.sum(lbuf[0:R, :], axis=-1, keepdims=True), (R, L))

        def gate_dc(d):
            dc[z0, pl.ds(T + HALO, 8), 0:L] = d[0:8, :]

        order = cfg['order']
        size = dict(A=cfg['ssplit'], B=NK - cfg['ssplit'], W=ND, O=NK, P=2 * ND,
                    Q=cfg['qsplit'], R=ND - cfg['qsplit'])
        start = {}
        for name in order:
            start[name] = sum(size[o] for o in order[:order.index(name)])
        jobs = {}

        def add(seg, t, gate, fn):
            jobs.setdefault(start[seg] + t, []).append((gate, fn))

        if conv:
            for p in range(len(piece_rows)):
                add(cfg['cseg'], cfg['cstart'] + p * cfg['cevery'], gate_g,
                    functools.partial(conv_piece, p))
            for p in range(cfg['nfin']):
                add(cfg['fseg'], cfg['fin'] + p * cfg['fevery'], gate_dc,
                    functools.partial(conv_finish, p))
        add(cfg['rseg'], cfg['rpos'], gate_l, inv_l)
        if prev:
            for p in range(cfg['lnp']):
                add(cfg['lseg'], cfg['lstart'] + p * cfg['levery'], gate_x,
                    functools.partial(ln3_part, p))

        def span(fn):
            at = [t for t, js in jobs.items() for _, j in js if getattr(j, 'func', j) is fn]
            return min(at), max(at)

        if prev:
            assert start['W'] + ND - 1 <= span(ln3_part)[0] and span(ln3_part)[1] < start['P']
        if conv:
            assert start['P'] + 2 * ND - 1 <= span(conv_piece)[0]
            assert span(conv_piece)[1] <= span(conv_finish)[0]
        assert start['O'] + NK - 1 <= span(inv_l)[0]

        def after_pass(t, d):
            for gate, fn in jobs.pop(t, []):
                gate(d)
                fn()

        b, _ = tile(i)

        def seg_s(lo, hi, t0):
            for n in range(lo, hi):
                keys = _cat([_bf(hh32[b, j, pl.ds(n * L // 2, L // 2), :]) for j in range(ND)])
                s = jax.lax.dot_general(operand(qbuf), keys, _NT, preferred_element_type=_F32)
                if (n + 1) * L > T:
                    if early:
                        s = s + kbias[n - T // L]
                    else:
                        col = jax.lax.broadcasted_iota(jnp.int32, (1, L), 1) + n * L
                        s = jnp.where(col < T, s, -1e30)
                sbuf[n] = s
                st['mm'] = s if n == 0 else jnp.maximum(st['mm'], s)
                after_pass(t0 + n - lo, s)
            if hi == NK:
                st['m'] = jnp.max(st['mm'], axis=-1, keepdims=True)

        def seg_w(t0):
            b1, r1 = tile(i - 1)
            for n in range(ND):
                d = jnp.dot(operand(o16), wvo[n], preferred_element_type=_F32)
                x1[b1, n, pl.ds(r1, R), :] += d * rbuf[...]
                after_pass(t0 + n, d)

        def seg_o(t0):
            NC = NK // ND
            p = exp_chunk(0)
            o = [None] * ND
            for c in range(NC):
                pn = None
                for n in range(ND):
                    v = _bf(hh32[b, n, pl.ds(c * ND * L // 2, ND * L // 2), :])
                    d = jnp.dot(p, v, preferred_element_type=_F32)
                    o[n] = d if c == 0 else o[n] + d
                    if c + 1 == NC:
                        o16[n] = o[n].astype(_BF16)
                    if n == cfg['egn'] and c + 1 < NC:
                        gate_s(d)
                        pn = exp_chunk(c + 1)
                    after_pass(t0 + c * ND + n, d)
                p = pn
            lbuf[0:R, :] = st['l']

        def seg_q(lo, hi, t0):
            cnt = [t0]

            def ap(d):
                after_pass(cnt[0], d)
                cnt[0] += 1
            q_proj(i + 1 if isinstance(i, int) else jnp.minimum(i + 1, NT - 1), lo, hi, ap)

        def seg_p(t0):
            b1, r1 = tile(i - 1)
            for n in range(ND):
                a = jnp.dot(operand(h3b), wp1[n], preferred_element_type=_F32)
                after_pass(t0 + 2 * n, a)
                bb = jnp.dot(operand(h3b), wp1[ND + n], preferred_element_type=_F32)
                g[b1, n, pl.ds(r1 + 2 * HALO, R), :] = a + a * jnp.tanh(bb)
                after_pass(t0 + 2 * n + 1, bb)

        segs = dict(A=(True, functools.partial(seg_s, 0, cfg['ssplit'])),
                    B=(True, functools.partial(seg_s, cfg['ssplit'], NK)),
                    Q=(True, functools.partial(seg_q, 0, cfg['qsplit'])),
                    R=(True, functools.partial(seg_q, cfg['qsplit'], ND)),
                    O=(True, seg_o), W=(prev, seg_w), P=(prev, seg_p))
        for name in order:
            on, fn = segs[name]
            if on:
                fn(start[name])
            for t in range(start[name], start[name] + size[name]):
                for _, job in jobs.pop(t, []):
                    job()
        assert not jobs
        return st['stats']

    stats = (jnp.zeros((8, D), _F32), jnp.zeros((8, D), _F32))
    q_proj(0)
    stats = step_b(zero_ref[0], stats, prev=False, conv=False, early=True)
    stats = jax.lax.fori_loop(1, NT, step_b, stats)

    last = NT - 1
    b1, r1 = tile(last)
    RB = cfg['TB']
    blocks = [(lo, lo + RB) for lo in range(0, R, RB)]
    for lo, hi in blocks:
        o = _cat([o16[c, lo:hi, :] for c in range(ND)])
        for n in range(ND):
            d = jnp.dot(o, wvo[n], preferred_element_type=_F32)
            x1[b1, n, r1 + lo:r1 + hi, :] += d * rbuf[lo:hi, :]
    shift = tmean[last - 1:last, :]
    t1 = jnp.zeros((8, D), _F32)
    t2 = jnp.zeros((8, D), _F32)

    def conv_rows(lo, hi):
        c1, c2 = [], []
        for j in range(ND):
            a = None
            for t in range(K):
                v = (g[b1, j, r1 + lo + HALO - pad + t:r1 + hi + HALO - pad + t, :]
                     * dwf[t:t + 1, j * L:(j + 1) * L])
                a = v if a is None else a + v
            dc[b1, r1 + lo:r1 + hi, j * L:(j + 1) * L] = a
            dd = (a - shift[:, j * L:(j + 1) * L]).reshape((hi - lo) // 8, 8, L)
            c1.append(jnp.sum(dd, axis=0))
            c2.append(jnp.sum(dd * dd, axis=0))
        return _cat(c1), _cat(c2)

    for lo, hi in blocks:
        h = _ln(_cat([x1[b1, n, r1 + lo:r1 + hi, :] for n in range(ND)]), 0.5).astype(_BF16)
        for j in range(ND):
            a = jnp.dot(h, wp1[j], preferred_element_type=_F32)
            bb = jnp.dot(h, wp1[ND + j], preferred_element_type=_F32)
            g[b1, j, r1 + 2 * HALO + lo:r1 + 2 * HALO + hi, :] = a + a * jnp.tanh(bb)
        c1, c2 = conv_rows(lo, hi if hi < R else CW)
        t1, t2 = t1 + c1, t2 + c2
    t1 = jnp.sum(t1, axis=0, keepdims=True)
    t2 = jnp.sum(t2, axis=0, keepdims=True)
    tmean[last:NT, :] = shift + t1 * (1.0 / CW)

    trow = jax.lax.broadcasted_iota(jnp.int32, (NT, 1), 0) % TPB
    tcnt = (R - HALO * (trow == 0).astype(jnp.int32)
            + HALO * (trow == TPB - 1).astype(jnp.int32)).astype(_F32)
    mu = (jnp.sum(stats[0], axis=0, keepdims=True) + (t1 + CW * shift)) * (1.0 / N)
    dm = tmean[...] - mu
    var = (jnp.sum(stats[1], axis=0, keepdims=True) + (t2 - t1 * t1 * (1.0 / CW))
           + jnp.sum(dm * dm * tcnt, axis=0, keepdims=True)) * (1.0 / N)
    rstd = jax.lax.rsqrt(var + _EPS) * 0.5

    def pw2(i):
        b, r0 = tile(i)
        u = (dc[b, pl.ds(r0 + HALO, R), :] - mu) * rstd
        a = (u + u * jnp.tanh(u)).astype(_BF16)
        st_cols(x1, i, ld_x(i) + jnp.dot(a, wp2[...], preferred_element_type=_F32))

    def ln4(i):
        hb[...] = _ln(ld_x(i), 0.5).astype(_BF16)

    def post_d(i):
        xall[pl.ds(rows(i), R), :] = _ln(ld_x(i) + 0.5 * acc[...]).astype(_BF16)
        o_copy(i).start()

    pw2(0)
    pw2(1)
    ln4(0)
    ff(wa2, wb2)
    ln4(1)

    def phase_d(i, carry):
        post_d(i - 1)
        ff(wa2, wb2, mid=lambda: pw2(i + 1))
        ln4(i + 1)
        return carry

    jax.lax.fori_loop(1, NT - 1, phase_d, 0)
    post_d(NT - 2)
    bl, rl = tile(NT - 1)
    tails = []

    def leave(lo, hi, f):
        x4 = _cat([x1[bl, n, rl + lo:rl + hi, :] for n in range(ND)]) + 0.5 * f
        o0 = (NT - 1) * R + lo
        xall[o0:o0 + hi - lo, :] = _ln(x4).astype(_BF16)
        tails.append(pltpu.make_async_copy(xall.at[pl.ds(o0, hi - lo), :],
                                           o_hbm.at[pl.ds(o0, hi - lo), :], wsem.at[len(tails)]))
        tails[-1].start()

    ff(wa2, wb2, finish=leave)
    for t in range(NT - 1):
        o_copy(t).wait()
    for c in tails:
        c.wait()


@jax.jit
def pallas_standalone__conformer_family_conformer__speech_kernel(
    x: jax.Array,
    w_ff1_a: jax.Array,
    w_ff1_b: jax.Array,
    w_q: jax.Array,
    w_k: jax.Array,
    w_v: jax.Array,
    w_o: jax.Array,
    w_pw1: jax.Array,
    dw: jax.Array,
    w_pw2: jax.Array,
    w_ff2_a: jax.Array,
    w_ff2_b: jax.Array,
):
    B, T, D = x.shape
    K = dw.shape[0]
    N = B * T
    TP = -(-T // D) * D
    ND = D // L
    assert T % R == 0 and K // 2 <= HALO and K - 1 - K // 2 <= HALO and D % L == 0

    weights = (w_ff1_a, w_ff1_b, w_q, w_k, w_v, w_o, w_pw1, dw, w_pw2, w_ff2_a, w_ff2_b)
    V = pltpu.VMEM
    F = w_ff1_a.shape[1]
    tiled = lambda w: V((w.shape[1] // L, w.shape[0], L), w.dtype)
    scratch = [tiled(w_ff1_a), V(w_ff1_b.shape, w_ff1_b.dtype)] + [V(w.shape, w.dtype) for w in weights[2:6]]
    scratch += [tiled(w_pw1), V(dw.shape, dw.dtype), V(w_pw2.shape, w_pw2.dtype),
                tiled(w_ff2_a), V(w_ff2_b.shape, w_ff2_b.dtype)]
    scratch += [
        V(w_ff1_a.shape, w_ff1_a.dtype),
        V((ND, D, L), _BF16),
        V((ND, D, L), _BF16),
        V((N, D), x.dtype),
        V((B, ND, T + 8, L), _F32),
        V((B, ND, TP, L), _BF16),
        V((B, ND, T + 4 * HALO, L), _F32),
        V((B, T + 2 * HALO, D), _F32),
        V((TP // L + 1, R, L), _F32),
        V((R, D), _BF16),
        V((R, D), _F32),
        V((ND, R, L), _BF16),
        V((ND, R, L), _BF16),
        V((ND, R, L), _BF16),
        V((R, L), _F32),
        V((R + 8, L), _F32),
        V((K, D), _F32),
        V((N // R, D), _F32),
        pltpu.SemaphoreType.DMA((max(9 + 2 * (F // FC), R // CFG['TB']),)),
        pltpu.SemaphoreType.DMA((N // R,)),
    ]
    col = np.arange(T // L * L, TP).reshape(-1, 1, L)
    kbias = np.where(col < T, 0.0, -1e30).astype(np.float32)
    out = pl.pallas_call(
        functools.partial(_kernel, B=B, T=T, D=D, K=K),
        out_shape=jax.ShapeDtypeStruct((N, D), x.dtype),
        in_specs=([pl.BlockSpec(memory_space=pltpu.SMEM), pl.BlockSpec(memory_space=pltpu.VMEM)]
                  + [pl.BlockSpec(memory_space=pl.ANY)] * (1 + len(weights))),
        out_specs=pl.BlockSpec(memory_space=pl.ANY),
        scratch_shapes=scratch,
        compiler_params=pltpu.CompilerParams(
            vmem_limit_bytes=120 * 2**20,
            flags={"XLA_TPU_EVENLY_DISTRIBUTE_CRITICAL_NODES": True},
        ),
        name="conformer",
    )(np.zeros((1,), np.int32), kbias, x.reshape(N, D), *weights)
    return out.reshape(B, T, D)
```
